```python
import os as _os
_os.environ.setdefault("JAX_PLATFORMS", "cpu")
import jax
import jax.numpy as jnp

def _softmax(x, axis=-1):
    return jax.nn.softmax(x, axis=axis)
def _gelu(x):
    return jax.nn.gelu(x, approximate=True)
def _silu(x):
    return jax.nn.silu(x)
def _sigmoid(x):
    return jax.nn.sigmoid(x)
def _layernorm(x, axis=-1, eps=1e-5):
    m = jnp.mean(x, axis=axis, keepdims=True)
    v = jnp.var(x, axis=axis, keepdims=True)
    return (x - m) / jnp.sqrt(v + eps)
def _scatter_add(tgt, idx, src, axis=0):
    return tgt.at[idx].add(src)
def _segment_sum(src, seg, n):
    return jax.ops.segment_sum(src, seg, n)
class _Rng:
    def __init__(self, key):
        self._k = key
    def _next(self):
        self._k, sub = jax.random.split(self._k)
        return sub
    def normal(self, shape):
        return jax.random.normal(self._next(), shape, dtype=jnp.bfloat16)
    def randint(self, lo, hi, shape):
        return jax.random.randint(self._next(), shape, lo, hi, dtype=jnp.int32)
    def uniform(self, shape, lo=0.0, hi=1.0):
        return jax.random.uniform(self._next(), shape, jnp.bfloat16, lo, hi)
    def permutation(self, n):
        return jax.random.permutation(self._next(), n)


kernel_name = 'interleave_layers__spectral_gfnet__mixer_token_mlp__prompt'

def setup_inputs():
    _rng = _Rng(jax.random.key(int.from_bytes(__import__("os").urandom(4), "little")))
    _w = (lambda a: (lambda t: t.astype(jnp.bfloat16) if jnp.issubdtype(t.dtype, jnp.floating) else t)(jnp.asarray(a)))
    def _A_setup():
        B, S, D = 1, 2048, 640
        Df = D // 2 + 1
        return {
            "x": _w((lambda *s: _rng.normal(s) * 0.05)(B, S, D)),
            "w_r": _w((lambda *s: _rng.normal(s) * 0.2)(S, Df) * 0.02),
            "w_i": _w((lambda *s: _rng.normal(s) * 0.2)(S, Df) * 0.02),
        }
    _A_in = _A_setup()

    def _B_setup():
        B, S, D, F = 1, 2048, 640, 1728
        return {
            "x": _w((lambda *s: _rng.normal(s) * 0.05)(B, S, D)),
            "w1": _w((lambda *s: _rng.normal(s) * 0.1)(S, F) * (S ** -0.5)),
            "b1": _w((lambda *s: _rng.normal(s) * 0.1)(F) * 0.02),
            "w2": _w((lambda *s: _rng.normal(s) * 0.1)(F, S) * (F ** -0.5)),
            "b2": _w((lambda *s: _rng.normal(s) * 0.1)(S) * 0.02),
        }
    _B_in = _B_setup()

    return {
        "A_x": _A_in["x"],
        "A_w_r": _A_in["w_r"],
        "A_w_i": _A_in["w_i"],
        "B_x": _B_in["x"],
        "B_w1": _B_in["w1"],
        "B_b1": _B_in["b1"],
        "B_w2": _B_in["w2"],
        "B_b2": _B_in["b2"],
    }

def reference(A_x, A_w_r, A_w_i, B_x, B_w1, B_b1, B_w2, B_b2):
    def _A_ref(x, w_r, w_i):
        B, S, D = x.shape
        X = (lambda x, axes=(-2,-1): jnp.fft.rfft2(x.astype(jnp.float32), axes=axes))(x, axes=(-2, -1))
        W = w_r + 1j * w_i
        X = X * W
        y = (lambda x, s, axes=(-2,-1): jnp.fft.irfft2(x, s=s, axes=axes).astype(jnp.bfloat16))(X, (S, D), axes=(-2, -1))
        return y

    def _B_ref(x, w1, b1, w2, b2):
        B, S, D = x.shape
        h = _layernorm(x, axis=-1)
        u = jnp.einsum("bsd,sf->bdf", h, w1) + b1
        u = _gelu(u)
        y = jnp.einsum("bdf,fs->bds", u, w2) + b2
        return (lambda x, *d: x.transpose(*d))(y, 0, 2, 1)

    x = A_x
    x = x + _A_ref(_layernorm(x, axis=-1), A_w_r, A_w_i)
    x = x + _B_ref(_layernorm(x, axis=-1), B_w1, B_b1, B_w2, B_b2)
    x = x + _A_ref(_layernorm(x, axis=-1), A_w_r, A_w_i)
    x = x + _B_ref(_layernorm(x, axis=-1), B_w1, B_b1, B_w2, B_b2)
    return x
```

```python
import numpy as np
import jax
import jax.numpy as jnp
from jax import lax
import jax.experimental.pallas as pl
import jax.experimental.pallas.tpu as pltpu
import ml_dtypes


S, D, F = 2048, 640, 1728
FP = 1792
EPS = 1e-5
f32, bf16, u32 = jnp.float32, jnp.bfloat16, jnp.uint32

TILE_CLASSES = ((0, 5), (2, 8), (4, 6), (7, 3), (9, 1))
SN1, SN2 = np.sin(2 * np.pi / 5), np.sin(4 * np.pi / 5)
C5 = float(np.sqrt(5) / 4)
R5 = float(SN2 / SN1)
GR = 336


def _d_mats():
    d3, j = np.arange(64), np.arange(32)
    i = np.arange(128)
    mix = (i // 8 % 2) * 64 + (i // 16) * 8 + i % 8
    cols = (i // 64) * 64 + (i // 8 % 2) * 32 + (i // 16 % 4) * 8 + i % 8
    fwd, inv = [], []
    z = np.zeros((32, 64))
    for p, (ka, kb) in enumerate(TILE_CLASSES):
        ea = np.exp(-2j * np.pi * np.outer(ka + 10 * j, d3) / D)
        eb = np.exp(-2j * np.pi * np.outer(kb + 10 * j, d3) / D)
        c = np.full(128, 2.0)
        if p == 0:
            m = np.block([[ea.real, z], [z, eb.real], [ea.imag, z], [z, eb.imag]])
            m[64, :64] = (-1.0) ** d3
            c[0] = c[64] = 1.0
        else:
            m = np.block([[ea.real, SN1 * ea.imag], [eb.real, -SN1 * eb.imag],
                          [ea.imag, -SN1 * ea.real], [eb.imag, SN1 * eb.real]])
        fwd.append(m[mix])
        inv.append(((m * c[:, None]).T / (S * D))[mix][:, cols])
    b = np.concatenate(fwd + inv, axis=1).astype(ml_dtypes.bfloat16).view(np.uint16).astype(np.uint32)
    return b[0::2] | (b[1::2] << 16)


_DM = _d_mats()


def L(t, n=1):
    return slice(128 * t, 128 * (t + n))


def add(a, b):
    return b if a is None else a if b is None else lax.add(a, b)


def sub(a, b):
    return a if b is None else lax.neg(b) if a is None else lax.sub(a, b)


def mul(a, b):
    if isinstance(b, float):
        return lax.mul(a, lax.full(a.shape, b, f32))
    return lax.mul(a, b)


def tree(xs):
    return xs[0] if len(xs) == 1 else add(tree(xs[:len(xs) // 2]), tree(xs[len(xs) // 2:]))


def cast(a, dt):
    return lax.convert_element_type(a, dt)


def cat(*xs):
    return lax.concatenate(xs, 0)


def rows(x, lo, n):
    return lax.slice_in_dim(x, lo, lo + n, axis=0)


def bcast(x, n):
    return lax.broadcast_in_dim(x, (n, 128), (0, 1))


def iota(axis):
    return lax.broadcasted_iota(jnp.int32, (8, 128), axis)


def cmul(u, v):
    return sub(mul(u[0], v[0]), mul(u[1], v[1])), add(mul(u[0], v[1]), mul(u[1], v[0]))


def unit(turns):
    angle = turns * float(-2 * np.pi)
    return jnp.cos(angle), jnp.sin(angle)


def _radix5(x0, x1, x2, x3, x4):
    s1, d1, s2, d2 = add(x1, x4), sub(x1, x4), add(x2, x3), sub(x2, x3)
    t = add(s1, s2)
    m = sub(x0, mul(t, 0.25))
    q = mul(sub(s1, s2), C5)
    return add(x0, t), add(m, q), add(d1, mul(d2, R5)), sub(m, q), sub(mul(d1, R5), d2)


def _radix5_t(t0, a1, b1, a2, b2):
    m = add(a1, a2)
    q = mul(sub(a1, a2), C5)
    t = sub(t0, mul(m, 0.25))
    s1, s2 = add(t, q), sub(t, q)
    d1, d2 = add(b1, mul(b2, R5)), sub(mul(b1, R5), b2)
    return add(t0, m), add(s1, d1), add(s2, d2), sub(s2, d2), sub(s1, d1)


def _half4(u, v):
    return add(u[0], v[0]), add(u[1], v[1]), sub(u[0], v[0]), sub(u[1], v[1])


def _finish4(e, o, sign):
    pr, pi, mr, mi = e
    sr, si, tr, ti = o
    o0, o2 = (add(pr, sr), add(pi, si)), (sub(pr, sr), sub(pi, si))
    oa, ob = (add(mr, ti), sub(mi, tr)), (sub(mr, ti), add(mi, tr))
    return (o0, oa, o2, ob) if sign < 0 else (o0, ob, o2, oa)


def _radix4(v, sign):
    return _finish4(_half4(v[0], v[2]), _half4(v[1], v[3]), sign)


def _twiddle(v, e):
    r, i = v
    e %= 16
    if e == 0:
        return r, i
    if e == 4:
        return lax.neg(i), r
    if e == 12:
        return i, lax.neg(r)
    c, s = float(np.cos(np.pi * e / 8)), float(np.sin(np.pi * e / 8))
    if e % 4 == 2:
        if c * s > 0:
            return mul(sub(r, i), c), mul(add(r, i), c)
        return mul(add(r, i), c), mul(sub(i, r), c)
    return sub(mul(r, c), mul(i, s)), add(mul(r, s), mul(i, c))


def _lhs7(i, a):
    if i == 0: return add(a(0, 0), a(1, 1))
    if i == 1: return add(a(1, 0), a(1, 1))
    if i == 2: return a(0, 0)
    if i == 3: return a(1, 1)
    if i == 4: return add(a(0, 0), a(0, 1))
    if i == 5: return sub(a(1, 0), a(0, 0))
    return sub(a(0, 1), a(1, 1))


def _rhs7(i, b):
    if i == 0: return add(b(0, 0), b(1, 1))
    if i == 1: return b(0, 0)
    if i == 2: return sub(b(0, 1), b(1, 1))
    if i == 3: return sub(b(1, 0), b(0, 0))
    if i == 4: return b(1, 1)
    if i == 5: return add(b(0, 0), b(0, 1))
    return add(b(1, 0), b(1, 1))


def _fold7(j, m, get, put, done):
    if j < 3:
        put(j, m)
    elif j == 3:
        done(1, 0, add(get(1), m))
        put(3, add(get(0), m))
    elif j == 4:
        done(0, 1, add(get(2), m))
        put(4, sub(get(3), m))
    elif j == 5:
        done(1, 1, add(add(sub(get(0, 2), get(1, 2)), get(2, 2)), m))
    else:
        done(0, 0, add(get(4), m))


LG = ((2, 3, 0), (1, 5), (4, 6))
ACT = 0
RG = ((1, 4, 0), (2, 5), (3, 6))
_FIRST = [7 * i + j for group in LG for i in group for j in range(7)]
_N = np.cumsum([0, 12, 16, 8, 12])
EARLY = [(k, _FIRST[lo:hi]) for k, lo, hi in zip((1, 1, 2, 2), _N, _N[1:])]
DONE = {ij: k for k, part in EARLY for ij in part}


def _nt(a, b):
    return lax.dot_general(a, b, (((1,), (1,)), ((), ())), preferred_element_type=f32)


def _nn(a, b):
    return lax.dot_general(a, b, (((1,), (0,)), ((), ())), preferred_element_type=f32)


def _merge(*streams):
    order = []
    for si, st in enumerate(streams):
        st, t0, t1 = st if isinstance(st, tuple) else (st, 0.0, 1.0)
        tot, acc = float(sum(t[0] for t in st)) or 1.0, 0.0
        for t in st:
            order.append((t0 + (t1 - t0) * (acc + (0.5 * t[0] if si else 0.0)) / tot, si, len(order), t))
            acc += t[0]
    for _, _, _, t in sorted(order, key=lambda o: o[:3]):
        t[1](*t[2:])


class Bank:
    def __init__(self, refs, offsets, cols, nrows, packed=0, chained=0):
        self.refs, self.offsets, self.nrows, self.packed, self.chained = refs, offsets, nrows, packed, chained
        self.cache, self.count = {}, 0

    @staticmethod
    def shapes(count, cols, nrows, packed=0, chained=0):
        n = (cols + 2) // 3 * nrows // 2 if packed else cols * nrows
        shape = ((n + 8 + 31) // 32 * 32, 384 if packed else 128)
        return [pltpu.VMEM(shape, u32 if packed else f32) for _ in range(count)]

    def view(self, k, via):
        if (k, via) not in self.cache:
            r = self.refs[k]
            r = r.at[pl.ds(self.offsets[via], r.shape[0])] if via else r
            self.cache[k, via] = r.bitcast(bf16) if self.packed else r
        return self.cache[k, via]

    def where(self, col, lo, n):
        blk, lane = divmod(col, 3 if self.packed else 1)
        return slice(blk * self.nrows + lo, blk * self.nrows + lo + n), L(lane)

    def get(self, k, col, lo=0, n=None, via=1):
        return self.view(k, via)[self.where(col, lo, n or self.nrows)]

    def wide(self, k, cols, lo=0, n=None, via=1):
        return lax.concatenate([self.get(k, c, lo, n, via) for c in cols], 1)

    def put(self, k, col, lo, val):
        for c in range(val.shape[1] // 128):
            self.count += 1
            part = lax.slice_in_dim(val, 128 * c, 128 * c + 128, axis=1)
            self.view(k, (0, 6 + self.count % 2, 6)[self.chained])[self.where(col + c, lo, val.shape[0])] = part

    def clear_tokens(self):
        for r in self.refs:
            r[r.shape[0] - 8:r.shape[0], 0:128] = jnp.zeros((8, 128), r.dtype)

    def token(self, k):
        n = self.refs[k].shape[0]
        return (id(self), k), self.refs[k][n - 8:n, 0:128]

    def mark(self, k, val):
        n = self.refs[k].shape[0]
        self.refs[k][n - 8:n, :] = val


class Table(Bank):
    def __init__(self, refs, offsets, size, groups, per, chained):
        super().__init__(refs, offsets, None, size, 1, chained)
        self.per = per
        self.slot = {i: (g, per * k) for g, group in enumerate(groups) for k, i in enumerate(group)}

    @staticmethod
    def shapes(tiles, size, groups, per, chained):
        return [s for _ in range(tiles) for g in groups for s in Bank.shapes(1, per * len(g), size, 1)]

    def load(self, k, i, j, via, lo=0, n=None):
        g, s = self.slot[i]
        return self.get(3 * k + g, s + j, lo, n, via)

    def store(self, k, i, j, lo, val):
        g, s = self.slot[i]
        self.put(3 * k + g, s + j, lo, cast(val, bf16))
        if j == self.per - 1 and (self.chained == 1 or 0):
            self.pending.append(self.token(3 * k + g))

    def tiles(self, ij, ks, via, axis=1):
        return lax.concatenate([self.load(k, ij // 7, ij % 7, via) for k in ks], axis)


BANKS = dict(x0=(Bank, 4, 4, D), x1=(Bank, 4, 4, D), va=(Bank, 8, 4, GR), vb=(Bank, 16, 4, 168), mr2=(Bank, 14, 4, GR),
             br2=(Bank, 4, 14, 128, 1, 1), tb=(Bank, 4, 20, 128, 1, 1),
             a1=(Table, 4, 160, LG, 7, 2), hp=(Bank, 4, 15, 160, 1, 2), bt=(Bank, 1, 2, 128), gt=(Bank, 1, 2, D), a2=(Table, 3, 160, LG, 7, 1), ar2=(Bank, 1, 7, 320, 1, 1),
             b1=(Table, 12, 128, RG, 7, 1), b2=(Table, 12, 128, RG, 7, 1),
             lo=(Bank, 10, 1, 160), hi=(Bank, 10, 4, 160), zb=(Bank, 4, 12, GR, 1, 1), mean=(Bank, 4, 16, 8, 0, 2), sums=(Bank, 4, 4, 64))


def _kernel(zero_ref, x_hbm, wr_hbm, wi_hbm, w1_hbm, b1_hbm, w2_hbm, b2_hbm, dm_hbm, o_hbm,
            b1_ref, b2_ref, wrb, wib, w1b, w2b, dm_ref, smb, wp, wt, small, sems, kept):
    zs = [None] + [pl.multiple_of(zero_ref[k], 16) for k in range(7)]
    m = {name: spec[0](kept[name], zs, *spec[2:]) for name, spec in BANKS.items()}
    pool, a1, a2 = kept["mr2"], kept["a1"], kept["a2"]
    m.update(k1=Bank(pool[:8], zs, 4, GR), hb=Bank(pool[8:12], zs, 4, GR), part=Bank(pool[:6] + pool[8:9], zs, 8, 160),
             mr1=Bank(pool[6:8], zs, 5, F - 1536), d0=Bank(pool[10:], zs, 4, 128),
             yb=Bank(a1, zs, 4, GR, 1))


    dm = dm_ref.bitcast(bf16)
    sm = [r.at[pl.ds(z, r.shape[0])].bitcast(bf16) for r in (smb,) for z in zs[1:5]]
    wpr = [r.at[pl.ds(zs[1], 2)] for r in wp]
    w_rd = [[r.at[pl.ds(zs[1 + g], F)] for g in range(3)] for r in (w1b, w2b)]
    tokens, used, ready = [], [], set()
    for bank in m.values():
        bank.pending = tokens

    def row(i, n):
        return bcast(small[i:i + 1, :], n)

    def paced(a):
        if not tokens:
            return a
        n, gates = a.shape[0] // 16, {}
        for i, (key, tok) in enumerate(tokens):
            at = (max(((i + 1) * n) // len(tokens) - 1, 0), 0, n - 1, i * n // len(tokens))[0]
            gates.setdefault(at, {})[key] = tok
        tokens.clear()
        parts, lo = [], 0
        for r in sorted(gates):
            if r > lo:
                parts.append(lax.slice(a, (16 * lo, 0), (16 * r, 128)))
            w = pltpu.bitcast(lax.slice(a, (16 * r, 0), (16 * r + 16, 128)), u32)
            for tok in gates[r].values():
                w = lax.bitwise_or(w, lax.bitcast_convert_type(tok, u32))
            parts.append(pltpu.bitcast(w, bf16))
            lo = r + 1
        if lo < n:
            parts.append(lax.slice(a, (16 * lo, 0), (16 * n, 128)))
        left = cat(*parts)
        return left if a.shape[1] == 128 else lax.concatenate([left, lax.slice(a, (0, 128), a.shape)], 1)

    def copy(src, dst):
        used.append(None)
        return pltpu.make_async_copy(src, dst, sems.at[len(used) - 1])

    order = [a + 4 * b for a in range(4) for b in range(4)]
    x_cp = {t: copy(x_hbm.at[L(t), :], w2b.at[L(t // 3), L(5 * (t % 3), 5)]) for t in order}
    o_cp = {t: copy(w1b.at[L(t // 3), L(5 * (t % 3), 5)], o_hbm.at[L(t), :]) for t in order}
    fence = copy(b2_hbm, b2_ref.at[16:32, :])
    w_cp = {(k, n): copy(src.at[lo:hi, :], dst.at[lo:hi, :]) for k, (src, dst) in enumerate(((w1_hbm, w1b), (w2_hbm, w2b)))
            for n, (lo, hi) in enumerate(((0, 512), (512, 1024), (1024, 1536), (1536, F)))}
    w_cp[0, 0] = [copy(w1_hbm.at[0:512, L(t)], w1b.at[0:512, L(t)]) for t in order]

    def get_v(name, a, q, lo, n):
        return m[name].get(2 * a, q, lo, n), m[name].get(2 * a + 1, q, lo, n)

    def put_v(name, a, q, lo, val):
        m[name].put(2 * a, q, lo, val[0])
        m[name].put(2 * a + 1, q, lo, val[1])

    def gather(acc, t, *xs):
        acc[t, 0] = add(acc.get((t, 0)), tree(xs))
        acc[t, 1] = add(acc.get((t, 1)), tree([mul(x, x) for x in xs]))

    def moments(acc, t):
        mean = jnp.sum(acc[t, 0], axis=0, keepdims=True) * (1.0 / D)
        return mean, jnp.maximum(jnp.sum(acc[t, 1], axis=0, keepdims=True) * (1.0 / D) - mean * mean, 0.0)

    def norm_once(acc, t):
        mean, var = moments(acc, t)
        small[32 + t:33 + t, :] = mean
        small[48 + t:49 + t, :] = lax.rsqrt(var + EPS)

    def load_x(t):
        eye = (lax.broadcasted_iota(jnp.int32, (128, 128), 0) == lax.broadcasted_iota(jnp.int32, (128, 128), 1)).astype(bf16)
        xt = _nt(paced(eye), jnp.concatenate([w2b[L(t // 3), L(5 * (t % 3) + j)] for j in range(5)], axis=0))
        acc = {}
        for c in range(16):
            x = [lax.slice(xt, (8 * c, 128 * j), (8 * c + 8, 128 * j + 128)) for j in range(5)]
            for j in range(5):
                m["x0"].put(t % 4, t // 4, 128 * j + 8 * c, x[j])
            gather(acc, t, *x)
        norm_once(acc, t)

    def fwd10(src, t, c):
        halves = []
        m10, r = mul(row(32 + t, 8), 10.0), row(48 + t, 8)
        for h in range(2):
            x = [m[src].get(t % 4, t // 4, 64 * i + 16 * c + 8 * h, 8) for i in range(10)]
            e = _radix5(*[add(x[i], x[i + 5]) for i in range(5)])
            o = _radix5(*[sub(x[i], x[i + 5]) if i % 2 == 0 else sub(x[i + 5], x[i]) for i in range(5)])
            halves.append([mul(v, r) for v in (sub(e[0], m10), o[0], e[1], e[2], e[3], e[4], o[1], o[2], o[3], o[4])])
        for i in range(10):
            m["tb"].put(t % 4, 4 * (i // 2) + t // 4, 64 * (i % 2) + 16 * c, cast(cat(halves[0][i], halves[1][i]), bf16))
        tokens.append(m["tb"].token(t % 4))

    def fwd_d(a, p):
        g = _nn(paced(dm[:, L(p)]), m["tb"].wide(a, range(4 * p, 4 * p + 4)))
        for c in range(8):
            v = [(lax.slice(g, (16 * c, 128 * b), (16 * c + 8, 128 * b + 128)),
                  lax.slice(g, (16 * c + 8, 128 * b), (16 * c + 16, 128 * b + 128))) for b in range(4)]
            if p == 0 and c == 0:
                for q, w in enumerate(_radix4([(i, jnp.zeros((8, 128), f32)) for (_, i) in v], -1)):
                    w = _twiddle(w, -q * a)
                    put_v("va", a, q, 320, (cat(w[0], w[0]), cat(w[1], w[1])))
                v = [(r, jnp.where(iota(0) == 0, 0.0, i)) for (r, i) in v]
            for q, w in enumerate(_radix4(v, -1)):
                put_v("va", a, q, 80 * (c % 4) + 16 * p + 8 * (c // 4), _twiddle(w, -q * a))

    def permute_w(get, put):
        cur = [get((-k) % 16) for k in range(16)]
        cur = [pltpu.roll(c, (-k) % 16, 1) if k else c for k, c in enumerate(cur)]
        for bit in (1, 2, 4, 8):
            msk = (iota(1) & bit) != 0
            cur = [lax.select(msk, cur[(k - bit) % 16], cur[k]) for k in range(16)]
        for k in range(16):
            put(k, cur[k])

    def prep_w(src, ri, part, c):
        if c < 20:
            def put(k, v):
                wp[part][ri, k, 8 * (c - 5 * part):8 * (c - 5 * part) + 8, :] = v
            permute_w(lambda t: pltpu.bitcast(src[16 * c:16 * c + 16, L(t)], u32), put)
        else:
            def put(k, v):
                wt[ri, k] = v
            permute_w(lambda t: bcast(cast(src[320:321, L(t)], f32), 8), put)

    def w_rows(ri, k1, c):
        if c == 20:
            v = wt[ri, k1]
            return cat(v, v)
        out = []
        for k in TILE_CLASSES[c % 5]:
            v = wpr[min(c // 5, 2)][ri, k1, pl.ds(k // 2 + 40 * (c // 15), 8, stride=5), :]
            out.append(lax.bitwise_and(v, lax.full(v.shape, 0xFFFF0000, u32)) if k % 2 else lax.shift_left(v, lax.full(v.shape, 16, u32)))
        return pltpu.bitcast(cat(*out), f32)

    def spectral(extra):
        units = [(h, q) for h in range(2) for q in range(4)]

        def s_in(q, c):
            z = _radix4([get_v("va", a, q, 16 * c, 16) for a in range(4)], -1)
            for p in range(4):
                for j, val in enumerate((add(z[p][0], z[p][1]), z[p][0], z[p][1])):
                    m["zb"].put(q, 3 * p + j, 16 * c, cast(val, bf16))
            tokens.append(m["zb"].token(q))

        def s_dot(h, q, p, j, inverse):
            lo, n = 160 * h, 160 + 16 * h
            lhs = paced(m["yb"].get(3 * q + j, p, lo, n) if inverse else m["zb"].get(q, 3 * p + j, lo, n))
            return (_nt if inverse else _nn)(lhs, sm[2 * h + inverse][L(q + 4 * p), L(j)])

        def s_fwd(h, q, ps):
            prod = {(p, j): s_dot(h, q, p, j, 0) for p in ps for j in (1, 2)}
            for k in range(10 + h):
                c = 10 * h + k
                for p in ps:
                    both = m["k1"].get(2 * q, p, 16 * c, 16)
                    x = sub(both, rows(prod[p, 2], 16 * k, 16)), add(both, rows(prod[p, 1], 16 * k, 16))
                    yr, yi = cmul(x, (w_rows(0, q + 4 * p, c), w_rows(1, q + 4 * p, c)))
                    for j, val in enumerate((add(yr, yi), yi, yr)):
                        m["yb"].put(3 * q + j, p, 16 * c, cast(val, bf16))

        def s_inv(h, q, odd):
            ps = (odd, odd + 2)
            prod = {(p, j): s_dot(h, q, p, j, 1) for p in ps for j in (1, 2)}
            for k in range(20 + h):
                lo, z = 160 * h + 8 * k, []
                for p in ps:
                    both = m["k1"].get(2 * q + 1, p, lo, 8)
                    z.append((add(both, rows(prod[p, 1], 8 * k, 8)), sub(both, rows(prod[p, 2], 8 * k, 8))))
                half = _half4(*z)
                if not odd:
                    for j in range(4):
                        m["hb"].put(q, j, lo, half[j])
                else:
                    for a, w in enumerate(_finish4([m["hb"].get(q, j, lo, 8) for j in range(4)], half, 1)):
                        put_v("vb", 4 * h + a, q, 8 * k, _twiddle(w, q * a))

        for c in range(10):
            s_in(0, c)
        tokens.clear()
        for u in range(9):
            now, before = units[u] if u < 8 else None, units[u - 1] if u else None
            common = ([now + (0,)] if now else []) + ([before + (1,)] if before else [])
            side = list(extra[u])
            if u < 7:
                h, q = units[u + 1]
                side += [(1, s_in, q, 10 * h + k) for k in range(10 + h)]
            early = [(1, inv4, a, p, c) for a in range(4) for p in range(5) for c in range(2)][u - 5::4] if u > 4 else []
            for k, (h, q, inverse) in enumerate(common):
                _merge(side[k * len(side) // len(common):(k + 1) * len(side) // len(common)])
                for p in range(4):
                    m["k1"].put(2 * q + inverse, p, 160 * h, s_dot(h, q, p, 0, inverse))
            for odd in range(2):
                if now:
                    s_fwd(*now, (odd, odd + 2))
                if before:
                    _merge(early[5 * odd:5 * odd + 5])
                    s_inv(*before, odd)

    def inv4(a, p, c):
        g = _radix4([get_v("vb", 4 * (c // 2) + a, q, 80 * (c % 2) + 16 * p, 16) for q in range(4)], 1)
        if (p, c) == (0, 0):
            for b in range(4):
                m["mean"].put(a, 4 + 2 * b, 0, rows(g[b][0], 0, 8))
                m["mean"].put(a, 5 + 2 * b, 0, rows(g[b][1], 8, 8))
                m["mean"].put(a, 12 + b, 0, rows(g[b][1], 0, 8))
        for b in range(4):
            for j in range(1 if (p, c) == (0, 0) else 2):
                m["tb"].put(a, 4 * p + b, 64 * j + 16 * c, cast(g[b][j], bf16))
        tokens.append(m["tb"].token(a))

    def real_bins(a):
        ny = _radix4([get_v("vb", 4 + a, q, 160, 8) for q in range(4)], 1)
        for b in range(4):
            t = a + 4 * b
            m["tb"].put(a, b, 64, cast(cat(lax.select(iota(0) == 0, ny[b][0], m["mean"].get(a, 12 + b)), m["mean"].get(a, 5 + 2 * b)), bf16))
            mean = small[32 + t:33 + t, :] + m["mean"].get(a, 4 + 2 * b, 0, 1) * (1.0 / (S * D))
            small[64 + t:65 + t, :] = small[16 + t:17 + t, :] + mean
            m["mean"].put(a, b, 0, bcast(mean, 8))
        tokens.append(m["mean"].token(a))

    def inv_d0(a):
        m["d0"].put(a, 0, 0, _nn(paced(dm[:, L(5)]), m["tb"].wide(a, range(4))))

    def inv_d(src, a, b):
        t = a + 4 * b
        tt = [_nn(dm[:, L(5 + p)], m["tb"].get(a, 4 * p + b)) for p in range(1, 5)]
        mean, sq = m["mean"].get(a, b), None
        for c in range(8):
            v = [rows(tt[i // 2], 16 * c + 8 * (i % 2), 8) for i in range(8)]
            e = _radix5_t(sub(m["d0"].get(a, b, 16 * c, 8), mean), *v[0:4])
            o = _radix5_t(m["d0"].get(a, b, 16 * c + 8, 8), *v[4:8])
            part = []
            for i in range(5):
                for j, sg in ((i, i % 2), (i + 5, 1 - i % 2)):
                    x = add(m[src].get(a, b, 64 * j + 8 * c, 8, 2), (sub if sg else add)(e[i], o[i]))
                    m["x1"].put(a, b, 64 * j + 8 * c, x)
                    part.append(mul(x, x))
            sq = add(sq, tree(part))
        var = jnp.sum(sq, axis=0, keepdims=True) * (1.0 / D)
        r = lax.rsqrt(var + EPS)
        small[48 + t:49 + t, :] = r * lax.rsqrt(var * r * r + EPS) * 0.5

    def split2(load, pick, put, group):
        seen = {}

        def blk(i, j):
            if (i, j) not in seen:
                seen[i, j] = load(i, j)
            return seen[i, j]
        for i in group:
            h = {(r, k): pick(i, lambda r1, k1: blk(2 * r1 + r, 2 * k1 + k)) for r in range(2) for k in range(2)}
            for j in range(7):
                put(i, j, pick(j, lambda r, k: h[r, k]))

    def lhs1(a, v, g):
        def load(r, k):
            t = a + 4 * k
            h = mul(m["x1"].get(a, k, 160 * r + 16 * v, 16, 3 + g), row(48 + t, 16))
            if r != k and (0, 2, 1, 0)[r // 2 * 2 + k // 2] == g:
                m["hp"].put(a, 4 * r + k, 16 * v, cast(h, bf16))
            return h

        def put(i, j, val):
            m["a1"].store(a, i, j, 16 * v, val)
        split2(load, _lhs7, put, LG[g])
        tokens.append(m["hp"].token(a))
        tokens.append(m["a1"].token(3 * a + g))

    def weights(which, g, lo, t):
        return cast(w_rd[which][g][lo:lo + 16, L(t)], f32)

    def rhs_main(which, n, a, v, g):
        def raw(f, s):
            lo = 128 * (4 * n + f) + 16 * v
            return weights(which, g, lo, a + 4 * s)
        tab = m[("b1", "b2")[which]]
        split2(raw if which else lambda s, f: raw(f, s), _rhs7,
               lambda i, j, val: tab.store(4 * n + a, i, j, 16 * v, val), RG[g])

    def rhs_rest(which, a, s2, v):
        lo = [1536 + 128 * f + 16 * v for f in range(2)]
        raw = [[weights(which, 0, r, a + 4 * s2 + 8 * s1) if r < F else None for s1 in range(2)] for r in lo]
        dst = m["br2"]
        for i in range(7):
            val = _rhs7(i, lambda k, n: raw[k][n])
            dst.put(a, 2 * i + s2, 16 * v, jnp.zeros((16, 128), bf16) if val is None else cast(val, bf16))
        tokens.append(dst.token(a))

    def rhs_main_tasks(which, ns, as_, gs=range(3)):
        return [(36 * len(RG[g]), rhs_main, which, n, a, v, g) for g in gs for n in ns for a in as_ for v in range(8)]

    def rhs_rest_tasks(which):
        return [(27, rhs_rest, which, a, s2, v) for a in range(4) for s2 in range(2) for v in range(8)]

    k0 = float(np.sqrt(2 / np.pi))

    def gelu_half(u):
        inner = mul(u, add(mul(mul(u, u), 8 * k0 * 0.044715), lax.full(u.shape, 2 * k0, f32)))
        return add(u, mul(u, lax.tanh(inner)))

    def fold49(ij, flip, prod, rest, done):
        i, j = divmod(ij, 7)
        for v in range(20):
            def slot(bank, par, col):
                return (lambda k, via=1: bank.get(5 * par + k, col, 8 * v, 8, via),
                        lambda k, val: bank.put(5 * par + k, col, 8 * v, val))

            def inner(r, n, h):
                h = add(h, rest(i, r, n, v)) if rest else h
                _fold7(i, h, *slot(m["hi"], flip, 2 * r + n), lambda r1, n1, c: done(2 * r1 + r, 2 * n1 + n, v, c))
            _fold7(j, rows(prod, 8 * v, 8), *slot(m["lo"], i % 2, 0), inner)

    def mm1_rest(a, j):
        def h(k):
            cuts = sorted({128 * j, 128 * j + 128} | {c for c in (160, 320, 480) if 128 * j < c < 128 * j + 128})
            return cat(*[m["hp"].get(a, 4 * (lo // 160) + k, lo % 160, hi - lo) if lo // 160 != k else
                         m["a1"].load(a, 2 + k // 2, 2 + k % 2, 4, lo % 160, hi - lo) for lo, hi in zip(cuts, cuts[1:])])
        w = lax.concatenate([w_rd[0][j % 3][1536:F, L(a + 4 * k)] for k in range(4)], 1)
        prod = _nt(paced(w), lax.concatenate([h(k) for k in range(4)], 1))
        m["mr1"].put(a % 2, j, 0, add(prod, m["mr1"].get(1 - a % 2, j) if a else None))

    def mm1_early(ij):
        k = DONE[ij]
        m["part"].put(ij // 8, ij % 8, 0, _nt(paced(m["a1"].tiles(ij, range(k), 5)), m["b1"].tiles(ij, range(k), 2)))

    def mm1_main(n, ij):
        def done(r, f, v, u):
            m["vb"].put(4 * (n % 2) + r, f, 8 * v, gelu_half(add(u, row(4 * n + f, 8))))
        k = DONE.get(ij, 0) if n == 0 else 0
        prod = _nt(paced(m["a1"].tiles(ij, range(k, 4), 1 + n)), m["b1"].tiles(ij, range(4 * n + k, 4 * n + 4), 1))
        if k:
            prod = add(prod, m["part"].get(ij // 8, ij % 8, 0, 160))
        if n == ACT and ij < 19:
            m["mr1"].mark(1, rows(prod, 152, 8))
        fold49(ij, n % 2, prod, None, done)

    def act_rest(j, n):
        height = min(128, F - 1536 - 128 * n)
        g = gelu_half(add(m["mr1"].get(1, j, 128 * n, height), m["bt"].get(0, n, 0, height)))
        g = g if height == 128 else cat(g, jnp.zeros((128 - height, 128), f32))
        m["gt"].put(0, n, 128 * j, g.T)

    def lhs_rest(v):
        g = {(r, k): m["gt"].get(0, k, 320 * r + 16 * v, 16) for r in range(2) for k in range(2)}
        for i in range(7):
            m["ar2"].put(0, i, 16 * v, cast(_lhs7(i, lambda r, k: g[r, k]), bf16))
        tokens.append(m["ar2"].token(0))

    def lhs2(n, v, g):
        split2(lambda r, f: m["vb"].get(4 * (n % 2) + r, f, 16 * v, 16, 1 + g), _lhs7,
               lambda i, j, val: m["a2"].store(n, i, j, 16 * v, val), LG[g])

    def lhs2_tasks(n):
        return [(23 * len(LG[g]), lhs2, n, v, g) for v in range(10) for g in range(3)]

    def mm2_rest(a, i):
        m["mr2"].put(7 * (a % 2) + i, a // 2 * 2, 0, _nn(paced(m["ar2"].get(0, i, via=1 + a)), m["br2"].wide(a, (2 * i, 2 * i + 1))))

    def write_out(t, j):
        out = cast(m["x0"].get(t % 4, t // 4, 128 * j, 128, 3), bf16).T
        w1b[L(t // 3), L(5 * (t % 3) + j)] = out
        if t % 4 < 3:
            m["tb"].put(0, 0, 0, rows(out, 112, 16))
            tokens.append(m["tb"].token(0))

    def mm2_main(a, ij, first):
        acc = {}
        def done(r, b, v, y):
            x = add(m["x1"].get(a, b, 160 * r + 8 * v, 8), add(y, row(64 + a + 4 * b, 8)))
            m["x0"].put(a, b, 160 * r + 8 * v, x)
            if first:
                gather(acc, 0, x)
                if v == 19:
                    m["sums"].put(a, b, 16 * r, cat(acc[0, 0], acc[0, 1]))

        def rest(i, r, n, v):
            return m["mr2"].get(7 * (a % 2) + i, a // 2 * 2 + n, 160 * r + 8 * v, 8)
        prod = _nn(paced(m["a2"].tiles(ij, range(3), 1 + a)), m["b2"].tiles(ij, range(a, 12, 4), 1, 0))
        fresh = set()
        fold49(ij, (a + 1) % 2, prod, rest, lambda r, b, v, y: (done(r, b, v, y), fresh.add((r, b))))
        for r, b in sorted(fresh if a == 3 and not first else ()):
            t = a + 4 * b
            ready.add((r, t))
            for j in range(5):
                need = {(128 * j // 160, t), ((128 * j + 127) // 160, t)}
                if (r, t) in need and need <= ready:
                    write_out(t, j)
            if all((k, t) in ready for k in range(4)):
                o_cp[t].start()

    def norm_sums(a, b):
        tot = None
        for r in range(4):
            tot = add(tot, m["sums"].get(a, b, 16 * r, 16))
        norm_once({(a + 4 * b, j): rows(tot, 8 * j, 8) for j in range(2)}, a + 4 * b)

    def after_mm2(a, first):
        if not first:
            return ([(30, write_out, a + 4 * b, j) for b in range(4) for j in range(5)] +
                    ([(1, o_cp[t].start) for t in order[:12]] + [(1, fence.wait)] if a == 2 else [])) if a < 3 else []
        return ([(20, norm_sums, a, b) for b in range(4)] +
                [(115, fwd10, "x0", a + 4 * b, c) for b in range(4) for c in range(4)])

    def post_stage(first):
        def inv4_tasks(a):
            return [(20, real_bins, a)] + [(40, inv4, a, p, c) for p in range(5) for c in (2, 3)]
        sums = [rhs_main_tasks(0, [0], [a]) if first else [] for a in range(4)]
        plan = [[(k, mm1_early, ij) for ij in part] for k, part in EARLY]
        for a in range(4):
            rest = [(4.8, mm1_rest, a - 1, j) for j in range(5)] if a else []
            _merge(inv4_tasks(a))
            inv_d0(a)
            for b in range(4):
                inv_d("x0", a, b)
                if a and 7 >> (a - 1) & 1:
                    n = 4 // plan[a][0][0]
                    _merge(plan[a][:n])
                    del plan[a][:n]
                else:
                    _merge(rest[:1])
                    del rest[:1]
            side = [(30 * len(LG[g]), lhs1, a, v, g) for v in range(10) for g in range(3)]
            if a == 0:
                _merge(side[0::3])
                tokens.clear()
                side = side[1::3] + side[2::3]
            if first and a == 1:
                for c in (w_cp[0, 1], w_cp[0, 2]):
                    c.start()
                for c in w_cp[0, 0][8:]:
                    c.wait()
            _merge(rest + plan[a], (side + (sums[2] if a == 1 else []), 0.0, 0.8))
        _merge([(1, mm1_rest, 3, j) for j in range(5)], (sums[3], -0.2, 0.8))

    def mm1_stage(first):
        for n in range(3):
            late, sums = [], []
            if first:
                if n == 0:
                    for c in [w_cp[1, k] for k in (3, 0, 1, 2)] + [fence]:
                        c.start()
                    w_cp[0, 1].wait()
                    w_cp[0, 2].wait()
                late = rhs_main_tasks(0, [n], range(4) if n else [], (1, 2))
                sums = rhs_main_tasks(0, [n + 1], range(4), (0,)) if n < 2 else [(0, w_cp[1, k].wait) for k in range(4)] + rhs_rest_tasks(1)
            _merge([(1, mm1_main, n, ij) for ij in range(49)],
                   (lhs2_tasks(n - 1) if n else [], 0.4, 0.97),
                   ([(2 - k, act_rest, j, k) for j in range(5) for k in range(2)] if n == ACT else [], 0.0, 0.38),
                   ([(1, lhs_rest, v) for v in range(20)] if n == 2 else [], 0.4, 0.95),
                   (late, 0.0, 0.39), (sums, 0.4 if n else 0.0, 0.95))

    def mm2_stage(first):
        sums = [t for a in range(4) for g in range(3) for t in rhs_main_tasks(1, range(3), [a], (g,))] if first else []
        cut = (0, 48, 124, 190, 240, 288)
        _merge([(1, mm2_rest, a, i) for a in range(4) for i in range(7)], (lhs2_tasks(2), 0.0, 0.9), (sums[:cut[1]], 0.0, 0.9))
        for a in range(4):
            _merge([(1, mm2_main, a, ij, first) for ij in range(49)],
                   (after_mm2(a - 1, first) if a else [], 0.02 if a < 3 or not first else 0.4, 0.95 if first or a < 3 else 0.3),
                   (sums[cut[a + 1]:cut[a + 2]], 0.0, 0.95 if a < 3 else 0.39))
        _merge([(1, fwd_d, a, p) for a in range(3) for p in range(5)] if first else [], (after_mm2(3, first), 0.0, 0.9))
        tokens.clear()
        if first:
            for p in range(5):
                fwd_d(3, p)
        else:
            for t in order:
                o_cp[t].wait()

    def token_mixing(first):
        tokens.clear()
        post_stage(first)
        mm1_stage(first)
        mm2_stage(first)

    def first_transform():
        cuts = (0, 80, 160, 321)
        dm_cp = copy(dm_hbm.at[:, L(0, 5)], dm_ref.at[:, L(0, 5)])
        small_cp = [copy(dm_hbm.at[:, L(5, 5)], dm_ref.at[:, L(5, 5)]), copy(b1_hbm, b1_ref), copy(b2_hbm, b2_ref.at[0:16, :])]
        f_cp = [[copy(src.at[lo:hi, :], dst.at[lo:hi, :]) for src, dst in ((wr_hbm, wrb), (wi_hbm, wib))]
                for lo, hi in zip(cuts, cuts[1:])]

        def prep(k):
            return [(1, prep_w, src, ri, k, c) for c in range(cuts[k] // 16, (cuts[k + 1] + 15) // 16)
                    for ri, src in enumerate((wrb, wib))]

        def fly(tiles):
            return [(1, fwd10, "x0", t, c) for t in tiles for c in range(4)]

        def start():
            for t in order[:4]:
                x_cp[t].start()
            for name in BANKS:
                if m[name].chained:
                    m[name].clear_tokens()
            s2, lane = (lax.broadcasted_iota(jnp.int32, (16, 128), k) for k in range(2))
            k2 = ((lane & 15) << 3) + (lane >> 4)
            base, hop = (unit(cast(k & 127, f32) * (1.0 / 128)) for k in (s2 * k2, 16 * k2))
            step = unit(cast(s2, f32) * (1.0 / S))
            for c in range(8):
                if c:
                    base, step = cmul(base, hop), cmul(step, (float(np.cos(np.pi / 64)), float(-np.sin(np.pi / 64))))
                re, im = base
                for k1 in range(16):
                    w = pltpu.bitcast(cast(lax.concatenate([re, sub(im, re), add(re, im), re], 1), bf16), u32)
                    for j in range(3):
                        part = lax.slice_in_dim(w, 128 * j, 128 * j + 128, axis=1)
                        smb[64 * k1 + 8 * c:64 * k1 + 8 * c + 8, L(j)] = pltpu.roll(part, k1, 1) if k1 else part
                    re, im = cmul((re, im), step)
            ends, ahead = (0, 2, 4, 8, 12, 16), (4, 6, 8, 12, 16, 16)
            for r in range(5):
                for c in [x_cp[t] for t in order[ahead[r]:ahead[r + 1]]] + ([], [dm_cp], [], [], f_cp[0] + f_cp[1])[r]:
                    c.start()
                for c in [x_cp[t] for t in order[ends[r]:ends[r + 1]]] + [dm_cp] * (r == 2):
                    c.wait()
                loads = [(1, load_x, t) for t in order[ends[r]:ends[r + 1]]]
                forward = [(0.8, fwd_d, r - 2, p) for p in range(5)] if r > 1 else []
                _merge(loads + forward, (fly(order[ends[r - 1]:ends[r]]) if r else [], -0.2, 0.4 if r > 1 else 0.6),
                       (fly(order[12:]) if r == 4 else [], 0.5, 0.9))
                tokens.clear()
            for c in f_cp[2]:
                c.start()
            for c in f_cp[0]:
                c.wait()
            _merge([(1, fwd_d, 3, p) for p in range(5)], prep(0))

        def prep_bias():
            half = jnp.concatenate([b1_ref[...].astype(f32).reshape(1, F), jnp.zeros((1, FP - F), f32)], axis=1) * 0.5
            for n in range(14):
                if n < 12:
                    small[n:n + 1, :] = half[:, L(n)]
                else:
                    m["bt"].put(0, n - 12, 0, bcast(half[:, L(n)], 128).T)
            small[16:32, :] = b2_ref[0:16, :].astype(f32)

        def rest():
            for c in small_cp:
                c.start()
            for c in f_cp[1]:
                c.wait()
            _merge(prep(1))
            sums = rhs_main_tasks(0, [0], [0, 1])
            spectral([[], [], [], [(0, c.start) for c in w_cp[0, 0][:8]] + [(0, c.wait) for c in f_cp[2]] + prep(2), [], [],
                      [(0, c.start) for c in [w_cp[0, 3]] + w_cp[0, 0][8:]] + [(0, c.wait) for c in small_cp + w_cp[0, 0][:8]] +
                      [(0, prep_bias)] + sums[:14], sums[14:32], sums[32:]])
            w_cp[0, 3].wait()
        start()
        rest()

    first_transform()
    token_mixing(True)
    spectral([[]] * 9)
    token_mixing(False)


@jax.jit
def pallas_interleave_layers__spectral_gfnet__mixer_token_mlp__prompt_kernel(A_x, A_w_r, A_w_i, B_x, B_w1, B_b1, B_w2, B_b2):
    hbm = pl.BlockSpec(memory_space=pl.ANY)
    V = pltpu.VMEM
    out = pl.pallas_call(
        _kernel,
        name="gfmix",
        in_specs=[pl.BlockSpec(memory_space=pltpu.SMEM), hbm, hbm, hbm, hbm, hbm, hbm, hbm, hbm],
        out_specs=hbm,
        out_shape=jax.ShapeDtypeStruct((S, D), bf16),
        scratch_shapes=[
            V((F,), bf16), V((64, 128), bf16), V((321, S), bf16), V((321, S), bf16), V((F, S), bf16), V((F, S), bf16), V((64, 1280), u32), V((16 * 64, 384), u32),
            [V((2, 16, n, 128), u32) for n in (40, 40, 80)], V((2, 16, 8, 128), f32), V((96, 128), f32),
            pltpu.SemaphoreType.DMA((72,)),
            {name: spec[0].shapes(*spec[1:]) for name, spec in BANKS.items()},
        ],
        compiler_params=pltpu.CompilerParams(vmem_limit_bytes=127 * 1024 * 1024, internal_scratch_in_bytes=11 * 4096),
    )(np.array([0] * 7 + [1], np.int32), A_x.reshape(S, D), A_w_r.T, A_w_i.T, B_w1.T, B_b1, B_w2,
      B_b2.reshape(16, 128), _DM)
    return out.reshape(1, S, D)
```

```python
import jax
import jax.experimental.pallas as pl
import jax.experimental.pallas.tpu as pltpu
import jax.numpy as jnp
import ml_dtypes
import numpy as np
from jax import lax

S, D, F = 2048, 640, 1728
MAIN = 1536
EPS = 1e-5
BINS = 336
f32, bf16, u32 = jnp.float32, jnp.bfloat16, jnp.uint32

TILE_CLASSES = ((0, 5), (2, 8), (4, 6), (7, 3), (9, 1))
SN1, SN2 = np.sin(2 * np.pi / 5), np.sin(4 * np.pi / 5)
C5 = float(np.sqrt(5) / 4)
R5 = float(SN2 / SN1)
GELU = float(np.sqrt(2 / np.pi))


def _channel_matrices():
    d, j, i = np.arange(64), np.arange(32), np.arange(128)
    out_rows = (i // 8 % 2) * 64 + (i // 16) * 8 + i % 8
    in_rows = (i // 64) * 64 + (i // 8 % 2) * 32 + (i // 16 % 4) * 8 + i % 8
    fwd, inv = [], []
    z = np.zeros((32, 64))
    for p, (ka, kb) in enumerate(TILE_CLASSES):
        ea = np.exp(-2j * np.pi * np.outer(ka + 10 * j, d) / D)
        eb = np.exp(-2j * np.pi * np.outer(kb + 10 * j, d) / D)
        weight = np.full(128, 2.0)
        if p == 0:
            m = np.block([[ea.real, z], [z, eb.real], [ea.imag, z], [z, eb.imag]])
            m[64, :64] = (-1.0) ** d
            weight[0] = weight[64] = 1.0
        else:
            m = np.block([[ea.real, SN1 * ea.imag], [eb.real, -SN1 * eb.imag],
                          [ea.imag, -SN1 * ea.real], [eb.imag, SN1 * eb.real]])
        fwd.append(m[out_rows])
        inv.append(((m * weight[:, None]).T / (S * D))[out_rows][:, in_rows])
    b = np.concatenate(fwd + inv, axis=1).astype(ml_dtypes.bfloat16).view(np.uint16).astype(np.uint32)
    return b[0::2] | (b[1::2] << 16)


_CHANNEL_MATRICES = _channel_matrices()
_OFFSETS = np.array([0] * 7 + [1], np.int32)


def L(t, n=1):
    return slice(128 * t, 128 * (t + n))


def add(a, b):
    return b if a is None else a if b is None else lax.add(a, b)


def sub(a, b):
    return lax.sub(a, b)


def mul(a, b):
    if isinstance(b, float):
        return lax.mul(a, lax.full(a.shape, b, f32))
    return lax.mul(a, b)


def tree(xs):
    return xs[0] if len(xs) == 1 else add(tree(xs[:len(xs) // 2]), tree(xs[len(xs) // 2:]))


def cast(a, dt):
    return lax.convert_element_type(a, dt)


def cat(*xs):
    return lax.concatenate(xs, 0)


def rows(x, lo, n):
    return lax.slice_in_dim(x, lo, lo + n, axis=0)


def bcast(x, n):
    return lax.broadcast_in_dim(x, (n, 128), (0, 1))


def iota(axis):
    return lax.broadcasted_iota(jnp.int32, (8, 128), axis)


def cmul(u, v):
    return sub(mul(u[0], v[0]), mul(u[1], v[1])), add(mul(u[0], v[1]), mul(u[1], v[0]))


def unit(turns):
    angle = turns * float(-2 * np.pi)
    return jnp.cos(angle), jnp.sin(angle)


def _radix5(x0, x1, x2, x3, x4):
    s1, d1, s2, d2 = add(x1, x4), sub(x1, x4), add(x2, x3), sub(x2, x3)
    t = add(s1, s2)
    m = sub(x0, mul(t, 0.25))
    q = mul(sub(s1, s2), C5)
    return add(x0, t), add(m, q), add(d1, mul(d2, R5)), sub(m, q), sub(mul(d1, R5), d2)


def _radix5_t(t0, a1, b1, a2, b2):
    m = add(a1, a2)
    q = mul(sub(a1, a2), C5)
    t = sub(t0, mul(m, 0.25))
    s1, s2 = add(t, q), sub(t, q)
    d1, d2 = add(b1, mul(b2, R5)), sub(mul(b1, R5), b2)
    return add(t0, m), add(s1, d1), add(s2, d2), sub(s2, d2), sub(s1, d1)


def _half4(u, v):
    return add(u[0], v[0]), add(u[1], v[1]), sub(u[0], v[0]), sub(u[1], v[1])


def _finish4(e, o, sign):
    pr, pi, mr, mi = e
    sr, si, tr, ti = o
    o0, o2 = (add(pr, sr), add(pi, si)), (sub(pr, sr), sub(pi, si))
    oa, ob = (add(mr, ti), sub(mi, tr)), (sub(mr, ti), add(mi, tr))
    return (o0, oa, o2, ob) if sign < 0 else (o0, ob, o2, oa)


def _radix4(v, sign):
    return _finish4(_half4(v[0], v[2]), _half4(v[1], v[3]), sign)


def _twiddle(v, e):
    r, i = v
    e %= 16
    if e == 0:
        return r, i
    if e == 4:
        return lax.neg(i), r
    if e == 12:
        return i, lax.neg(r)
    c, s = float(np.cos(np.pi * e / 8)), float(np.sin(np.pi * e / 8))
    if e % 4 == 2:
        if c * s > 0:
            return mul(sub(r, i), c), mul(add(r, i), c)
        return mul(add(r, i), c), mul(sub(i, r), c)
    return sub(mul(r, c), mul(i, s)), add(mul(r, s), mul(i, c))


def _lhs7(i, a):
    if i == 0: return add(a(0, 0), a(1, 1))
    if i == 1: return add(a(1, 0), a(1, 1))
    if i == 2: return a(0, 0)
    if i == 3: return a(1, 1)
    if i == 4: return add(a(0, 0), a(0, 1))
    if i == 5: return sub(a(1, 0), a(0, 0))
    return sub(a(0, 1), a(1, 1))


def _rhs7(i, b):
    if i == 0: return add(b(0, 0), b(1, 1))
    if i == 1: return b(0, 0)
    if i == 2: return sub(b(0, 1), b(1, 1))
    if i == 3: return sub(b(1, 0), b(0, 0))
    if i == 4: return b(1, 1)
    if i == 5: return add(b(0, 0), b(0, 1))
    return add(b(1, 0), b(1, 1))


def _fold7(j, m, get, put, done):
    if j < 3:
        put(j, m)
    elif j == 3:
        done(1, 0, add(get(1), m))
        put(3, add(get(0), m))
    elif j == 4:
        done(0, 1, add(get(2), m))
        put(4, sub(get(3), m))
    elif j == 5:
        done(1, 1, add(add(sub(get(0, 2), get(1, 2)), get(2, 2)), m))
    else:
        done(0, 0, add(get(4), m))


LHS1 = ((2, 5), (3, 6), (0, 1, 4))
LHS2 = ((2, 3, 0), (1, 5), (4, 6))
RHS = ((1, 4, 0), (2, 5), (3, 6))
_FIRST = [7 * i + j for group in LHS1 for i in group for j in range(7)]
EARLY = ([(0, 1, ij) for ij in _FIRST[:24]], [(0, 1, ij) for ij in _FIRST[24:40]],
         [(0, 2, ij) for ij in _FIRST[40:48]], [(1, 3, ij) for ij in _FIRST[:12]])
DONE = {ij: hi for part in EARLY for _, hi, ij in part}


def quarters(j):
    cuts = sorted({128 * j, 128 * j + 128} | {c for c in (160, 320, 480) if 128 * j < c < 128 * j + 128})
    return [(lo // 160, lo % 160, hi - lo) for lo, hi in zip(cuts, cuts[1:])]


def _nt(a, b):
    return lax.dot_general(a, b, (((1,), (1,)), ((), ())), preferred_element_type=f32)


def _nn(a, b):
    return lax.dot_general(a, b, (((1,), (0,)), ((), ())), preferred_element_type=f32)


def _merge(*streams):
    order = []
    for si, st in enumerate(streams):
        st, t0, t1 = st if isinstance(st, tuple) else (st, 0.0, 1.0)
        tot, acc = float(sum(t[0] for t in st)) or 1.0, 0.0
        for t in st:
            order.append((t0 + (t1 - t0) * (acc + (0.5 * t[0] if si else 0.0)) / tot, si, len(order), t))
            acc += t[0]
    for _, _, _, t in sorted(order, key=lambda o: o[:3]):
        t[1](*t[2:])


class Bank:
    def __init__(self, refs, offsets, cols, nrows, packed=0, chained=0):
        self.refs, self.offsets, self.nrows, self.packed, self.chained = refs, offsets, nrows, packed, chained
        self.cache, self.count, self.held = {}, 0, None

    @staticmethod
    def shapes(count, cols, nrows, packed=0, chained=0):
        n = ((cols + packed) >> packed) * (nrows >> packed) + 8
        return [pltpu.VMEM(((n + 31) // 32 * 32, 128 << packed), u32 if packed else f32) for _ in range(count)]

    def view(self, k, via):
        if (k, via) not in self.cache:
            r = self.refs[k]
            self.cache[k, via] = r.at[pl.ds(self.offsets[via], r.shape[0])] if via else r
        return self.cache[k, via]

    def get(self, k, col, lo=0, n=None, via=1):
        lo += (col >> self.packed) * self.nrows
        x = self.view(k, via)[lo >> self.packed:(lo + (n or self.nrows)) >> self.packed, L(col & self.packed)]
        return pltpu.bitcast(x, bf16) if self.packed else x

    def wide(self, k, cols, via=1):
        return lax.concatenate([self.get(k, c, via=via) for c in cols], 1)

    def halves(self, k, c, via=1):
        return cat(self.get(k, 2 * c, via=via), self.get(k, 2 * c + 1, via=via))

    def put(self, k, col, lo, x):
        if self.packed and col % 2 == 0:
            self.held = x
            return
        if self.packed:
            x = pltpu.bitcast(cast(lax.concatenate([self.held, x], 1), bf16), u32)
        at = ((col >> self.packed) * self.nrows + lo) >> self.packed
        self.count += 1
        self.view(k, (0, 6 + self.count % 2, 6)[self.chained])[at:at + x.shape[0], :] = x

    def clear_tokens(self):
        for r in self.refs:
            r[r.shape[0] - 8:r.shape[0], L(0)] = jnp.zeros((8, 128), r.dtype)

    def token(self, k):
        n = self.refs[k].shape[0]
        return (id(self), k), self.refs[k][n - 8:n, L(0)]


class Table(Bank):
    def __init__(self, refs, offsets, nrows, groups, chained):
        super().__init__(refs, offsets, None, nrows, 1, chained)
        self.slot = {i: (g, 7 * k) for g, group in enumerate(groups) for k, i in enumerate(group)}

    @staticmethod
    def shapes(tiles, nrows, groups, chained):
        return [s for _ in range(tiles) for g in groups for s in Bank.shapes(1, 7 * len(g), nrows, 1)]

    def load(self, k, i, j, via, lo=0, n=None):
        g, s = self.slot[i]
        return self.get(3 * k + g, s + j, lo, n, via)

    def store(self, k, i, j, lo, val):
        g, s = self.slot[i]
        self.put(3 * k + g, s + j, lo, val)

    def tiles(self, ij, ks, via, axis=1):
        return lax.concatenate([self.load(k, ij // 7, ij % 7, via) for k in ks], axis)


BANKS = dict(
    x0=(Bank, 4, 4, D),
    x1=(Bank, 4, 4, D),
    va=(Bank, 8, 4, BINS), vb=(Bank, 16, 4, 168),
    mr2=(Bank, 12, 2, 2 * BINS),
    wt=(Bank, 4, 4, F - MAIN, 1, 2), br=(Bank, 4, 12, 64, 1, 1), tb=(Bank, 4, 40, 64, 1, 1),
    a1=(Table, 4, 160, LHS1, 2), hp=(Bank, 4, 12, 160, 1, 2), bt=(Bank, 1, 1, 256),
    a2=(Table, 3, 160, LHS2, 1), ar=(Bank, 1, 18, 128, 1, 2),
    b1=(Table, 12, 128, RHS, 1), b2=(Table, 12, 128, RHS, 1),
    lo=(Bank, 10, 1, 160), hi=(Bank, 10, 4, 160), zb=(Bank, 4, 12, BINS, 1, 1),
    post=(Bank, 1, 1, 240, 1, 2), sm=(Bank, 1, 48, 128, 1), mean=(Bank, 4, 4, 40, 0, 2), sums=(Bank, 4, 4, 64))

BIAS1, BIAS2, MEAN, SCALE, SHIFT = 0, 16, 32, 48, 64


def _kernel(zero_ref, x_hbm, wr_hbm, wi_hbm, w1_hbm, b1_hbm, w2_hbm, b2_hbm, dm_hbm, o_hbm,
            b1_ref, b2_ref, wrb, wib, w1b, w2b, dm_ref, wp, wt, small, sems, kept):
    zs = [None] + [pl.multiple_of(zero_ref[k], 16) for k in range(7)]
    m = {name: spec[0](kept[name], zs, *spec[2:]) for name, spec in BANKS.items()}
    pool, a1, a2 = kept["mr2"], kept["a1"], kept["a2"]
    m.update(k1=Bank(pool[:8], zs, 4, BINS), hb=Bank(pool[8:12], zs, 4, BINS), part=Bank(pool[:6] + pool[8:9], zs, 8, 160),
             mr1=Bank(pool[6:8], zs, 5, F - MAIN), d0=Bank(pool[9:], zs, 4, 128),
             yb=Bank(a1[2::3] + a1[0::3], zs, 6, BINS, 1))

    def dm(p):
        return pltpu.bitcast(dm_ref[:, L(p)], bf16)

    wpr = [r.at[pl.ds(zs[1], 2)] for r in wp]
    w_rd = [[r.at[pl.ds(zs[1 + g], F)] for g in range(3)] for r in (w1b, w2b)]
    tokens, used, ready, backlog, plain = [], [], set(), [], {}

    def row(i, n):
        return bcast(small[i:i + 1, :], n)

    def paced(a):
        if not tokens:
            return a
        n, gates = a.shape[0] // 16, {}
        for i, (key, tok) in enumerate(tokens):
            gates.setdefault(max((i + 1) * n // len(tokens) - 1, 0), {})[key] = tok
        tokens.clear()
        parts, lo = [], 0
        for r in sorted(gates):
            if r > lo:
                parts.append(lax.slice(a, (16 * lo, 0), (16 * r, 128)))
            w = pltpu.bitcast(lax.slice(a, (16 * r, 0), (16 * r + 16, 128)), u32)
            for tok in gates[r].values():
                w = lax.bitwise_or(w, lax.bitcast_convert_type(tok, u32))
            parts.append(pltpu.bitcast(w, bf16))
            lo = r + 1
        if lo < n:
            parts.append(lax.slice(a, (16 * lo, 0), (16 * n, 128)))
        left = cat(*parts)
        return left if a.shape[1] == 128 else lax.concatenate([left, lax.slice(a, (0, 128), a.shape)], 1)

    def copy(src, dst):
        used.append(None)
        return pltpu.make_async_copy(src, dst, sems.at[len(used) - 1])

    order = [a + 4 * b for a in range(4) for b in range(4)]
    x_cp = {t: copy(x_hbm.at[L(t), :], w2b.at[L(t // 3), L(5 * (t % 3), 5)]) for t in order}
    o_cp = {t: [copy(w1b.at[L(t // 3), L(5 * (t % 3) + j, n)], o_hbm.at[L(t), L(j, n)])
                for j, n in (((0, 3), (3, 2)) if t % 4 == 3 else ((0, 5),))] for t in order}
    nudges = []

    def launch(*copies):
        k = len(nudges)
        nudges.append(copy(dm_hbm.at[0:8, L(0)], m["post"].view(0, 5).at[8 * k:8 * k + 8, L(0)]))
        for c in copies + (nudges[-1],):
            c.start()
        tokens.append(m["post"].token(0))

    w_cp = {(k, n): copy(src.at[lo:hi, :], dst.at[lo:hi, :]) for k, (src, dst) in enumerate(((w1_hbm, w1b), (w2_hbm, w2b)))
            for n, (lo, hi) in enumerate(((0, 512), (512, 1024), (1024, MAIN), (MAIN, F))) if k or n}
    w_cp[0, 0] = [copy(w1_hbm.at[0:512, L(t)], w1b.at[0:512, L(t)]) for t in order]

    def get_v(name, a, q, lo, n):
        return m[name].get(2 * a, q, lo, n), m[name].get(2 * a + 1, q, lo, n)

    def put_v(name, a, q, lo, val):
        m[name].put(2 * a, q, lo, val[0])
        m[name].put(2 * a + 1, q, lo, val[1])

    def gather(acc, t, *xs):
        acc[t, 0] = add(acc.get((t, 0)), tree(xs))
        acc[t, 1] = add(acc.get((t, 1)), tree([mul(x, x) for x in xs]))

    def moments(acc, t):
        mean = jnp.sum(acc[t, 0], axis=0, keepdims=True) * (1.0 / D)
        return mean, jnp.maximum(jnp.sum(acc[t, 1], axis=0, keepdims=True) * (1.0 / D) - mean * mean, 0.0)

    def norm_once(acc, t):
        mean, var = moments(acc, t)
        small[MEAN + t:MEAN + t + 1, :] = mean
        small[SCALE + t:SCALE + t + 1, :] = lax.rsqrt(var + EPS)

    def load_x(t):
        eye = (lax.broadcasted_iota(jnp.int32, (128, 128), 0) == lax.broadcasted_iota(jnp.int32, (128, 128), 1)).astype(bf16)
        xt = _nt(paced(eye), jnp.concatenate([w2b[L(t // 3), L(5 * (t % 3) + j)] for j in range(5)], axis=0))
        acc = {}
        for c in range(16):
            x = [lax.slice(xt, (8 * c, 128 * j), (8 * c + 8, 128 * j + 128)) for j in range(5)]
            for j in range(5):
                m["x0"].put(t % 4, t // 4, 128 * j + 8 * c, x[j])
            gather(acc, t, *x)
        norm_once(acc, t)

    def fwd10(t, c):
        halves = []
        m10, r = mul(row(MEAN + t, 8), 10.0), row(SCALE + t, 8)
        for h in range(2):
            x = [m["x0"].get(t % 4, t // 4, 64 * i + 16 * c + 8 * h, 8) for i in range(10)]
            e = _radix5(*[add(x[i], x[i + 5]) for i in range(5)])
            o = _radix5(*[sub(x[i], x[i + 5]) if i % 2 == 0 else sub(x[i + 5], x[i]) for i in range(5)])
            halves.append([mul(v, r) for v in (sub(e[0], m10), o[0], e[1], e[2], e[3], e[4], o[1], o[2], o[3], o[4])])
        for i in range(10):
            m["tb"].put(t % 4, 10 * (t // 4) + i, 16 * c, cat(halves[0][i], halves[1][i]))
        tokens.append(m["tb"].token(t % 4))

    def fwd_d(a, p):
        g = _nn(paced(dm(p)), lax.concatenate([m["tb"].halves(a, 5 * b + p) for b in range(4)], 1))
        for c in range(8):
            v = [(lax.slice(g, (16 * c, 128 * b), (16 * c + 8, 128 * b + 128)),
                  lax.slice(g, (16 * c + 8, 128 * b), (16 * c + 16, 128 * b + 128))) for b in range(4)]
            if p == 0 and c == 0:
                for q, w in enumerate(_radix4([(i, jnp.zeros((8, 128), f32)) for (_, i) in v], -1)):
                    w = _twiddle(w, -q * a)
                    put_v("va", a, q, 320, (cat(w[0], w[0]), cat(w[1], w[1])))
                v = [(r, jnp.where(iota(0) == 0, 0.0, i)) for (r, i) in v]
            for q, w in enumerate(_radix4(v, -1)):
                put_v("va", a, q, 80 * (c % 4) + 16 * p + 8 * (c // 4), _twiddle(w, -q * a))

    def permute_w(get, put):
        cur = [get((-k) % 16) for k in range(16)]
        cur = [pltpu.roll(c, (-k) % 16, 1) if k else c for k, c in enumerate(cur)]
        for bit in (1, 2, 4, 8):
            msk = (iota(1) & bit) != 0
            cur = [lax.select(msk, cur[(k - bit) % 16], cur[k]) for k in range(16)]
        for k in range(16):
            put(k, cur[k])

    def prep_w(src, ri, part, c):
        if c < 20:
            def put(k, v):
                wp[part][ri, k, 8 * (c - 5 * part):8 * (c - 5 * part) + 8, :] = v
            permute_w(lambda t: pltpu.bitcast(src[16 * c:16 * c + 16, L(t)], u32), put)
        else:
            def put(k, v):
                wt[ri, k] = v
            permute_w(lambda t: bcast(cast(src[320:321, L(t)], f32), 8), put)

    def w_rows(ri, k1, c):
        if c == 20:
            v = wt[ri, k1]
            return cat(v, v)
        out = []
        for k in TILE_CLASSES[c % 5]:
            v = wpr[min(c // 5, 2)][ri, k1, pl.ds(k // 2 + 40 * (c // 15), 8, stride=5), :]
            out.append(lax.bitwise_and(v, lax.full(v.shape, 0xFFFF0000, u32)) if k % 2 else lax.shift_left(v, lax.full(v.shape, 16, u32)))
        return pltpu.bitcast(cat(*out), f32)

    def s_in(q, c):
        z = _radix4([get_v("va", a, q, 16 * c, 16) for a in range(4)], -1)
        for p in range(4):
            for j, val in enumerate((add(z[p][0], z[p][1]), z[p][0], z[p][1])):
                m["zb"].put(q, 3 * p + j, 16 * c, val)
        tokens.append(m["zb"].token(q))

    def spectral(extra):
        units = [(h, q) for h in range(2) for q in range(4)]

        def s_dot(h, q, p, j, inverse):
            lo, n = 160 * h, 160 + 16 * h
            lhs = paced(m["yb"].get(2 * q + p % 2, 3 * (p // 2) + j, lo, n) if inverse else m["zb"].get(q, 3 * p + j, lo, n))
            return (_nt if inverse else _nn)(lhs, m["sm"].get(0, 16 * j + q + 4 * p, via=1 + 2 * h + inverse))

        def s_fwd(h, q, ps):
            prod = {(p, j): s_dot(h, q, p, j, 0) for p in ps for j in (1, 2)}
            for k in range(10 + h):
                c = 10 * h + k
                for p in ps:
                    both = m["k1"].get(2 * q, p, 16 * c, 16)
                    x = sub(both, rows(prod[p, 2], 16 * k, 16)), add(both, rows(prod[p, 1], 16 * k, 16))
                    yr, yi = cmul(x, (w_rows(0, q + 4 * p, c), w_rows(1, q + 4 * p, c)))
                    for j, val in enumerate((add(yr, yi), yi, yr)):
                        m["yb"].put(2 * q + p % 2, 3 * (p // 2) + j, 16 * c, val)

        def s_inv(h, q, odd):
            ps = (odd, odd + 2)
            prod = {(p, j): s_dot(h, q, p, j, 1) for p in ps for j in (1, 2)}
            for k in range(20 + h):
                lo, z = 160 * h + 8 * k, []
                for p in ps:
                    both = m["k1"].get(2 * q + 1, p, lo, 8)
                    z.append((add(both, rows(prod[p, 1], 8 * k, 8)), sub(both, rows(prod[p, 2], 8 * k, 8))))
                half = _half4(*z)
                if not odd:
                    for j in range(4):
                        m["hb"].put(q, j, lo, half[j])
                else:
                    for a, w in enumerate(_finish4([m["hb"].get(q, j, lo, 8) for j in range(4)], half, 1)):
                        put_v("vb", 4 * h + a, q, 8 * k, _twiddle(w, q * a))

        for c in range(10):
            s_in(0, c)
        tokens.clear()
        for u in range(9):
            now, before = units[u] if u < 8 else None, units[u - 1] if u else None
            common = ([now + (0,)] if now else []) + ([before + (1,)] if before else [])
            side, more = list(extra[u][0]), extra[u][1]
            if u < 7:
                h, q = units[u + 1]
                side += [(1, s_in, q, 10 * h + k) for k in range(10 + h)]
            early = [(1, inv4, a, p, c) for a in range(4) for p in range(5) for c in range(2)][u - 5::4] if u > 4 else []
            for k, (h, q, inverse) in enumerate(common):
                _merge(side[k * len(side) // len(common):(k + 1) * len(side) // len(common)])
                for p in range(4):
                    m["k1"].put(2 * q + inverse, p, 160 * h, s_dot(h, q, p, 0, inverse))
            for odd in range(2):
                if now:
                    s_fwd(*now, (odd, odd + 2))
                if before:
                    _merge(early[odd::2], more if odd == 0 else [])
                    s_inv(*before, odd)

    def inv4(a, p, c):
        g = _radix4([get_v("vb", 4 * (c // 2) + a, q, 80 * (c % 2) + 16 * p, 16) for q in range(4)], 1)
        if (p, c) == (0, 0):
            for b in range(4):
                m["mean"].put(a, b, 0, cat(*g[b]))
            return
        for b in range(4):
            for j in range(2):
                m["tb"].put(a, 10 * b + 2 * p + j, 16 * c, g[b][j])
        tokens.append(m["tb"].token(a))

    def real_bins(a):
        ny = _radix4([get_v("vb", 4 + a, q, 160, 8) for q in range(4)], 1)
        for b in range(4):
            t = a + 4 * b
            g = m["mean"].get(a, b, 0, 32)
            m["tb"].put(a, 10 * b, 0, rows(g, 0, 16))
            m["tb"].put(a, 10 * b + 1, 0, cat(lax.select(iota(0) == 0, ny[b][0], rows(g, 16, 8)), rows(g, 24, 8)))
            mean = small[MEAN + t:MEAN + t + 1, :] + rows(g, 0, 1) * (1.0 / (S * D))
            small[SHIFT + t:SHIFT + t + 1, :] = small[BIAS2 + t:BIAS2 + t + 1, :] + mean
            m["mean"].put(a, b, 32, bcast(mean, 8))
        tokens.append(m["mean"].token(a))

    def inv_d0(a):
        for b in range(4):
            m["d0"].put(a % 2, b, 0, _nn(paced(dm(5)), m["tb"].halves(a, 5 * b)))

    def inv_d(a, b):
        t = a + 4 * b
        tt = [_nn(dm(5 + p), m["tb"].halves(a, 5 * b + p)) for p in range(1, 5)]
        mean, sq = m["mean"].get(a, b, 32, 8), None
        for c in range(8):
            v = [rows(tt[i // 2], 16 * c + 8 * (i % 2), 8) for i in range(8)]
            e = _radix5_t(sub(m["d0"].get(a % 2, b, 16 * c, 8), mean), *v[0:4])
            o = _radix5_t(m["d0"].get(a % 2, b, 16 * c + 8, 8), *v[4:8])
            part = []
            for i in range(5):
                for j, sg in ((i, i % 2), (i + 5, 1 - i % 2)):
                    x = add(m["x0"].get(a, b, 64 * j + 8 * c, 8, 2), (sub if sg else add)(e[i], o[i]))
                    m["x1"].put(a, b, 64 * j + 8 * c, x)
                    part.append(mul(x, x))
            sq = add(sq, tree(part))
        var = jnp.sum(sq, axis=0, keepdims=True) * (1.0 / D)
        r = lax.rsqrt(var + EPS)
        small[SCALE + t:SCALE + t + 1, :] = r * lax.rsqrt(var * r * r + EPS) * 0.5

    def split2(load, pick, put, group, gate=None):
        seen = {}

        def blk(i, j):
            if (i, j) not in seen:
                seen[i, j] = load(i, j)
            return seen[i, j]
        for i in group:
            h = {(r, k): pick(i, lambda r1, k1: blk(2 * r1 + r, 2 * k1 + k)) for r in range(2) for k in range(2)}
            for j in range(7):
                put(i, j, pick(j, lambda r, k: h[r, k]))
            if i == group[-1] and len(group) % 2:
                put(i, 7, pick(6, lambda r, k: h[r, k]))
            if gate:
                tokens.append(gate())

    def lhs1(a, v, g):
        def load(r, k):
            t = a + 4 * k
            h = mul(m["x1"].get(a, k, 160 * r + 16 * v, 16, 3 + g), row(SCALE + t, 16))
            if r != k and g == k // 2:
                m["hp"].put(a, plain.setdefault((r, k), len(plain)), 16 * v, h)
            return h

        def put(i, j, val):
            m["a1"].store(a, i, j, 16 * v, val)
        split2(load, _lhs7, put, LHS1[g])
        tokens.append(m["hp"].token(a))
        tokens.append(m["a1"].token(3 * a + g))

    def weights(which, g, lo, t):
        return cast(w_rd[which][g][lo:lo + 16, L(t)], f32)

    def rhs_main(which, n, a, v, g):
        def raw(f, s):
            lo = 128 * (4 * n + f) + 16 * v
            return weights(which, g, lo, a + 4 * s)
        tab = m[("b1", "b2")[which]]
        split2(raw if which else lambda s, f: raw(f, s), _rhs7,
               lambda i, j, val: tab.store(4 * n + a, i, j, 16 * v, val), RHS[g], lambda: tab.token(3 * (4 * n + a) + g))

    def rhs_rest(a, pair, v):
        (p1, p2, p3), (q1, q2, q3) = ([weights(1, 0, MAIN + 64 * k + 16 * v, a + 8 * pair + 4 * e) for k in range(3)] for e in range(2))
        for k, val in enumerate((sub(p1, q1), p2, q2, sub(q3, p3), q1, p3)):
            m["br"].put(a, 6 * pair + k, 16 * v, val)
        tokens.append(m["br"].token(a))

    def rhs_main_tasks(which, ns, as_, gs=range(3)):
        return [(36 * len(RHS[g]), rhs_main, which, n, a, v, g) for g in gs for n in ns for a in as_ for v in range(8)]

    def rhs_rest_tasks():
        return [(22, rhs_rest, a, pair, v) for a in range(4) for pair in range(2) for v in range(4)]

    def gelu_half(u):
        inner = mul(u, add(mul(mul(u, u), 8 * GELU * 0.044715), lax.full(u.shape, 2 * GELU, f32)))
        return add(u, mul(u, lax.tanh(inner)))

    def fold49(ij, flip, prod, done):
        i, j = divmod(ij, 7)
        for v in range(20):
            def slot(bank, par, col):
                return (lambda k, via=1: bank.get(5 * par + k, col, 8 * v, 8, via),
                        lambda k, val: bank.put(5 * par + k, col, 8 * v, val))

            def inner(r, n, h):
                _fold7(i, h, *slot(m["hi"], flip, 2 * r + n), lambda r1, n1, c: done(2 * r1 + r, 2 * n1 + n, v, c))
            _fold7(j, rows(prod, 8 * v, 8), *slot(m["lo"], i % 2, 0), inner)

    def stage_w1(a, k):
        for e in (2 * k, 2 * k + 1):
            m["wt"].put(a, e, 0, cast(w1b[MAIN:F, L(a + 4 * e)], f32))
        tokens.append(m["wt"].token(a))

    def mm1_rest(a, j):
        def h(k):
            return cat(*[m["hp"].get(a, plain[r, k], lo, n) if r != k else m["a1"].load(a, 2 + k // 2, 2 + k % 2, 4, lo, n)
                         for r, lo, n in quarters(j)])
        w = m["wt"].wide(a, range(4), via=1 + j)
        prod = _nt(paced(w), lax.concatenate([h(k) for k in range(4)], 1))
        for lo in range(0, F - MAIN, 8):
            u = add(rows(prod, lo, 8), m["mr1"].get(1 - a % 2, j, lo, 8) if a else m["bt"].get(0, 0, lo, 8, 1 + j))
            m["mr1"].put(a % 2, j, lo, gelu_half(u) if a == 3 else u)

    def mm1_early(lo, hi, ij):
        prod = _nt(paced(m["a1"].tiles(ij, range(lo, hi), 5)), m["b1"].tiles(ij, range(lo, hi), 2))
        m["part"].put(ij // 8, ij % 8, 0, add(prod, m["part"].get(ij // 8, ij % 8, via=2) if lo else None))

    def mm1_main(n, ij):
        def done(r, f, v, u):
            m["vb"].put(4 * (n % 2) + r, f, 8 * v, gelu_half(add(u, row(BIAS1 + 4 * n + f, 8))))
        k = DONE.get(ij, 0) if n == 0 else 0
        prod = _nt(paced(m["a1"].tiles(ij, range(k, 4), 1 + n)), m["b1"].tiles(ij, range(4 * n + k, 4 * n + 4), 1))
        if k:
            prod = add(prod, m["part"].get(ij // 8, ij % 8, 0, 160))
        fold49(ij, n % 2, prod, done)

    def lhs_rest(j, k):
        for e in range(2):
            g = cat(*[m["mr1"].get(1, 2 * j + e, 64 * u, 64, 1 + k) if 2 * j + e < 5 else jnp.zeros((64, 128), f32)
                      for u in ((0, 1), (1, 2), (0, 2))[k]])
            m["ar"].put(0, 6 * k + 2 * j + e, 0, g.T)
        tokens.append(m["ar"].token(0))

    def lhs2(n, v, g):
        split2(lambda r, f: m["vb"].get(4 * (n % 2) + r, f, 16 * v, 16, 1 + g), _lhs7,
               lambda i, j, val: m["a2"].store(n, i, j, 16 * v, val), LHS2[g], lambda: m["a2"].token(3 * n + g))

    def lhs2_tasks(n):
        return [(23 * len(LHS2[g]), lhs2, n, v, g) for v in range(10) for g in range(3)]

    def mm2_rest(a, k, r):
        lhs = paced(cat(*[m["ar"].get(0, 6 * k + j, lo - 128 * j, n, 1 + a) for j in range(5)
                          for q, lo, n in ((q, 160 * q + at, n) for q, at, n in quarters(j)) if q == r]))
        prod = _nn(lhs, lax.concatenate([m["br"].halves(a, 3 * e + k, 1 + r) for e in range(2)], 1))
        for e in range(2):
            m["mr2"].put(3 * a + k, e, 160 * r, lax.slice_in_dim(prod, 128 * e, 128 * e + 128, axis=1))

    def write_out(t, j):
        x = m["x0"].get(t % 4, t // 4, 128 * j, 128, 3) if t % 4 < 3 else cat(
            *[m["vb"].get(4 * r + t // 4, 0, lo, n, 4) for r, lo, n in quarters(j)])
        out = x.T
        w1b[L(t // 3), L(5 * (t % 3) + j)] = cast(out, bf16)
        m["mean"].put(0, 0, 0, rows(out, 120, 8))
        tokens.append(m["mean"].token(0))

    def mm2_main(a, ij, first):
        acc = {}
        def done(r, b, v, y):
            rest = [m["mr2"].get(3 * a + k, b // 2, 160 * r + 8 * v, 8, 1 + b % 2) for k in (b % 2, 2)]
            x = add(add(m["x1"].get(a, b, 160 * r + 8 * v, 8), row(SHIFT + a + 4 * b, 8)), add(y, add(*rest)))
            if first or a < 3:
                m["x0"].put(a, b, 160 * r + 8 * v, x)
            else:
                m["vb"].put(4 * r + b, 0, 8 * v, x)
            if first:
                gather(acc, 0, x)
                if v == 19:
                    m["sums"].put(a, b, 16 * r, cat(acc[0, 0], acc[0, 1]))

        prod = _nn(paced(m["a2"].tiles(ij, range(3), 1 + a)), m["b2"].tiles(ij, range(a, 12, 4), 1, 0))
        fresh = set()
        fold49(ij, (a + 1) % 2, prod, lambda r, b, v, y: (done(r, b, v, y), fresh.add((r, b))))
        if a == 3 and not first:
            for r, b in sorted(fresh):
                t = a + 4 * b
                ready.add((r, t))
                for j in range(5):
                    need = {(128 * j // 160, t), ((128 * j + 127) // 160, t)}
                    if (r, t) in need and need <= ready:
                        backlog.append((ij, write_out, t, j))
                for part, need in enumerate(({(0, t), (1, t), (2, t)}, {(2, t), (3, t)})):
                    if (r, t) in need and need <= ready:
                        backlog.append((ij, launch, o_cp[t][part]))
            for _ in range(2 if ij < 48 else 99):
                if backlog and (backlog[0][0] + 4 <= ij or ij == 48):
                    _, fn, *args = backlog.pop(0)
                    args[0].start() if fn is launch and ij == 48 else fn(*args)

    def norm_sums(a, b):
        tot = None
        for r in range(4):
            tot = add(tot, m["sums"].get(a, b, 16 * r, 16))
        norm_once({(a + 4 * b, j): rows(tot, 8 * j, 8) for j in range(2)}, a + 4 * b)

    def after_mm2(a, first):
        if not first:
            return ([(30, write_out, a + 4 * b, j) for b in range(4) for j in range(5)] +
                    [(30, launch, *[o_cp[a + 4 * b][0] for b in range(4)])]) if a < 3 else []
        return ([(20, norm_sums, a, b) for b in range(4)] +
                [(115, fwd10, a + 4 * b, c) for b in range(4) for c in range(4)])

    def post_stage(first):
        def inv4_tasks(a):
            return [(20, real_bins, a)] + [(40, inv4, a, p, c) for p in range(5) for c in (2, 3)]
        sums = [rhs_main_tasks(0, [0], [a]) if first else [] for a in range(4)]
        plan = [[(hi - lo, mm1_early, lo, hi, ij) for lo, hi, ij in part] for part in EARLY]
        for a in range(4):
            _merge(inv4_tasks(a)[:3])
            inv_d0(a)
            _merge(inv4_tasks(a)[3:])
            tokens.clear()
            side = [[(30 * len(LHS1[g]), lhs1, a, v, g) for v in range(10)] for g in range(3)]
            for b in range(4):
                inv_d(a, b)
                if a == 0 and b == 2:
                    _merge(side.pop(0))
                    tokens.clear()
                if a or b >= 2:
                    n = 4 // plan[a][0][0]
                    _merge(plan[a][:n])
                    del plan[a][:n]
            if first:
                side.append([(40, stage_w1, a, k) for k in range(2)] + (sums[2] if a == 1 else []))
            if a == 0:
                n = 14 - (24 - len(plan[0]))
                _merge(plan[0][:n], (side.pop(0), -0.2, 0.5))
                tokens.clear()
                del plan[0][:n]
            _merge([(4.8, mm1_rest, a - 1, j) for j in range(5 if a else 0)] + plan[a],
                   ([t for part in side for t in part], 0.0, 0.8))
        if first:
            for k in (3, 0, 1, 2):
                w_cp[1, k].start()
            w_cp[0, 1].wait()
            w_cp[0, 2].wait()
        _merge([(1, mm1_rest, 3, j) for j in range(5)], (sums[3][:8], -0.2, 0.8))

    cut = (32, 72, 150, 202, 240, 288)

    def w2_sums():
        return [t for a in range(4) for g in range(3) for t in rhs_main_tasks(1, range(3), [a], (g,))]

    def mm1_stage(first):
        for n in range(3):
            late, sums = [], []
            if first:
                late = rhs_main_tasks(0, [n], range(4) if n else [3], (1, 2))
                sums = rhs_main_tasks(0, [n + 1], range(4), (0,)) if n < 2 else [(0, w_cp[1, k].wait) for k in range(4)] + rhs_rest_tasks() + w2_sums()[:cut[0]]
            _merge([(1, mm1_main, n, ij) for ij in range(49)],
                   (lhs2_tasks(n - 1) if n else [], 0.45, 0.97),
                   ([(1, lhs_rest, j, k) for j in range(3) for k in range(3)] if n == 2 else [], 0.4, 0.95),
                   (late, 0.0, 0.39), (sums, 0.4 if n else 0.0, 0.95))

    def mm2_stage(first):
        sums = w2_sums() if first else []
        _merge([(1, mm2_rest, a, k, r) for a in range(4) for k in range(3) for r in range(4)], (lhs2_tasks(2), 0.0, 0.9), (sums[cut[0]:cut[1]], 0.0, 0.9))
        for a in range(4):
            _merge([(1, mm2_main, a, ij, first) for ij in range(49)],
                   (after_mm2(a - 1, first) if a else [], 0.1 if a < 3 or not first else 0.4, 0.95 if first else 0.45),
                   (sums[cut[a + 1]:cut[a + 2]], 0.0, 0.95 if a < 3 else 0.39))
        _merge([(1, fwd_d, a, p) for a in range(3) for p in range(5)] if first else [], (after_mm2(3, first), 0.0, 0.9))
        tokens.clear()
        if first:
            for p in range(5):
                fwd_d(3, p)
        else:
            for c in nudges + [c for t in order for c in o_cp[t]]:
                c.wait()

    def token_mixing(first):
        tokens.clear()
        post_stage(first)
        mm1_stage(first)
        mm2_stage(first)

    def first_transform():
        cuts = (0, 80, 160, 321)
        dm_cp = copy(dm_hbm.at[:, L(0, 5)], dm_ref.at[:, L(0, 5)])
        small_cp = [copy(dm_hbm.at[:, L(5, 5)], dm_ref.at[:, L(5, 5)]), copy(b1_hbm, b1_ref), copy(b2_hbm, b2_ref.at[0:16, :])]
        f_cp = [[copy(src.at[lo:hi, :], dst.at[lo:hi, :]) for src, dst in ((wr_hbm, wrb), (wi_hbm, wib))]
                for lo, hi in zip(cuts, cuts[1:])]

        def prep(k):
            return [(1, prep_w, src, ri, k, c) for c in range(cuts[k] // 16, (cuts[k + 1] + 15) // 16)
                    for ri, src in enumerate((wrb, wib))]

        def fly(tiles):
            return [(1, fwd10, t, c) for t in tiles for c in range(4)]

        def start():
            for name in BANKS:
                if m[name].chained:
                    m[name].clear_tokens()
            launch(*[x_cp[t] for t in order[:6]])
            gate = lax.bitcast_convert_type(tokens.pop()[1], jnp.int32)
            s2, lane = (lax.broadcasted_iota(jnp.int32, (16, 128), k) for k in range(2))
            s2, lane = s2 + cat(gate, gate), lane + cat(gate, gate)
            k2 = ((lane & 15) << 3) + (lane >> 4)
            base, hop = (unit(cast(k & 127, f32) * (1.0 / 128)) for k in (s2 * k2, 16 * k2))
            step = unit(cast(s2, f32) * (1.0 / S))
            for c in range(8):
                if c:
                    base, step = cmul(base, hop), cmul(step, (float(np.cos(np.pi / 64)), float(-np.sin(np.pi / 64))))
                re, im = base
                for k1 in range(0, 16, 2):
                    nxt = cmul((re, im), step)
                    two = [[pltpu.roll(x, k, 1) if k else x for x in z] for k, z in enumerate(((re, im), nxt), k1)]
                    for j in range(3):
                        for k, (x, y) in enumerate(two, k1):
                            m["sm"].put(0, 16 * j + k, 16 * c, (x, sub(y, x), add(x, y))[j])
                    re, im = cmul(nxt, step)
            queue = [[x_cp[t] for t in order[k:k + 2]] + [dm_cp] * (k == 6) for k in range(6, 16, 2)] + f_cp[:2] + [[]]
            for before, lo, hi in ((0, 0, 2), (0, 2, 4), (2, 4, 8), (4, 8, 12), (8, 12, 16)):
                for c in queue.pop(0):
                    c.start()
                for c in [x_cp[t] for t in order[lo:hi]] + [dm_cp] * (lo == 4):
                    c.wait()
                _merge([(1, load_x, t) for t in order[lo:hi]] + [(0.8, fwd_d, lo // 4 - 1, p) for p in range(5 * (lo > 3))],
                       (fly(order[before:lo]), -0.2, 0.6 if lo == 2 else 0.3),
                       (fly(order[12:] if hi == 16 else []), 0.5, 0.88),
                       ([(1, launch, *queue.pop(0))] if lo > 3 else [], 0.2, 0.3))
                tokens.clear()
            for c in f_cp[2]:
                c.start()
            for c in f_cp[0]:
                c.wait()
            _merge([(1, fwd_d, 3, p) for p in range(5)], prep(0))

        def prep_bias():
            half = jnp.concatenate([b1_ref[...].astype(f32).reshape(1, F), jnp.zeros((1, 64), f32)], axis=1) * 0.5
            for n in range(14):
                if n < 12:
                    small[BIAS1 + n:BIAS1 + n + 1, :] = half[:, L(n)]
                else:
                    m["bt"].put(0, 0, 128 * (n - 12), bcast(half[:, L(n)], 128).T)
            small[BIAS2:BIAS2 + 16, :] = b2_ref[0:16, :].astype(f32)

        def rest():
            for c in small_cp + w_cp[0, 0][:4]:
                c.start()
            for c in f_cp[1]:
                c.wait()
            _merge(prep(1))
            sums = rhs_main_tasks(0, [0], [0, 1])
            cut = (0, 4, 10, 28, 34, 44, 48)
            sums = [sums[lo:hi] for lo, hi in zip(cut, cut[1:])]
            none = [], []
            spectral([none, none, none,
                      ([(0, c.start) for c in w_cp[0, 0][4:8] + [w_cp[0, 3]]] + [(0, c.wait) for c in f_cp[2]] + prep(2), []),
                      none, none,
                      ([(0, c.start) for c in w_cp[0, 0][8:]] + [(0, c.wait) for c in small_cp + w_cp[0, 0][:8]] +
                       [(0, prep_bias)] + sums[0], sums[1]), sums[2:4], sums[4:6]])
            w_cp[0, 1].start()
            w_cp[0, 2].start()
            for c in [w_cp[0, 3]] + w_cp[0, 0][8:]:
                c.wait()
        start()
        rest()

    first_transform()
    token_mixing(True)
    spectral([([], [])] * 9)
    token_mixing(False)


@jax.jit
def pallas_interleave_layers__spectral_gfnet__mixer_token_mlp__prompt_kernel(A_x, A_w_r, A_w_i, B_x, B_w1, B_b1, B_w2, B_b2):
    hbm = pl.BlockSpec(memory_space=pl.ANY)
    V = pltpu.VMEM
    out = pl.pallas_call(
        _kernel,
        in_specs=[pl.BlockSpec(memory_space=pltpu.SMEM), hbm, hbm, hbm, hbm, hbm, hbm, hbm, hbm],
        out_specs=hbm,
        out_shape=jax.ShapeDtypeStruct((S, D), bf16),
        scratch_shapes=[
            V((F,), bf16), V((64, 128), bf16), V((321, S), bf16), V((321, S), bf16), V((F, S), bf16), V((F, S), bf16), V((64, 1280), u32),
            [V((2, 16, n, 128), u32) for n in (40, 40, 80)], V((2, 16, 8, 128), f32), V((96, 128), f32),
            pltpu.SemaphoreType.DMA((88,)),
            {name: spec[0].shapes(*spec[1:]) for name, spec in BANKS.items()},
        ],
        compiler_params=pltpu.CompilerParams(vmem_limit_bytes=127 * 1024 * 1024, internal_scratch_in_bytes=11 * 4096),
    )(_OFFSETS, A_x.reshape(S, D), A_w_r.T, A_w_i.T, B_w1.T, B_b1, B_w2,
      B_b2.reshape(16, 128), _CHANNEL_MATRICES)
    return out.reshape(1, S, D)
```

```python
import jax
import jax.experimental.pallas as pl
import jax.experimental.pallas.tpu as pltpu
import jax.numpy as jnp
import ml_dtypes
import numpy as np
from jax import lax

S, D, F = 2048, 640, 1728
MAIN = 1536
EPS = 1e-5
BINS = 336
f32, bf16, u32 = jnp.float32, jnp.bfloat16, jnp.uint32

TILE_CLASSES = ((0, 5), (2, 8), (4, 6), (7, 3), (9, 1))
SN1, SN2 = np.sin(2 * np.pi / 5), np.sin(4 * np.pi / 5)
C5 = float(np.sqrt(5) / 4)
R5 = float(SN2 / SN1)
GELU = float(np.sqrt(2 / np.pi))


def _channel_matrices():
    d, j, i = np.arange(64), np.arange(32), np.arange(128)
    out_rows = (i // 8 % 2) * 64 + (i // 16) * 8 + i % 8
    in_rows = (i // 64) * 64 + (i // 8 % 2) * 32 + (i // 16 % 4) * 8 + i % 8
    fwd, inv = [], []
    z = np.zeros((32, 64))
    for p, (ka, kb) in enumerate(TILE_CLASSES):
        ea = np.exp(-2j * np.pi * np.outer(ka + 10 * j, d) / D)
        eb = np.exp(-2j * np.pi * np.outer(kb + 10 * j, d) / D)
        weight = np.full(128, 2.0)
        if p == 0:
            m = np.block([[ea.real, z], [z, eb.real], [ea.imag, z], [z, eb.imag]])
            m[64, :64] = (-1.0) ** d
            weight[0] = weight[64] = 1.0
        else:
            m = np.block([[ea.real, SN1 * ea.imag], [eb.real, -SN1 * eb.imag],
                          [ea.imag, -SN1 * ea.real], [eb.imag, SN1 * eb.real]])
        fwd.append(m[out_rows])
        inv.append(((m * weight[:, None]).T / (S * D))[out_rows][:, in_rows])
    b = np.concatenate(fwd + inv, axis=1).astype(ml_dtypes.bfloat16).view(np.uint16).astype(np.uint32)
    return b[0::2] | (b[1::2] << 16)


_CHANNEL_MATRICES = _channel_matrices()


def L(t, n=1):
    return slice(128 * t, 128 * (t + n))


def add(a, b):
    return b if a is None else a if b is None else lax.add(a, b)


def sub(a, b):
    return lax.sub(a, b)


def mul(a, b):
    if isinstance(b, float):
        return lax.mul(a, lax.full(a.shape, b, f32))
    return lax.mul(a, b)


def tree(xs):
    return xs[0] if len(xs) == 1 else add(tree(xs[:len(xs) // 2]), tree(xs[len(xs) // 2:]))


def cast(a, dt):
    return lax.convert_element_type(a, dt)


def cat(*xs):
    return lax.concatenate(xs, 0)


def rows(x, lo, n):
    return lax.slice_in_dim(x, lo, lo + n, axis=0)


def bcast(x, n):
    return lax.broadcast_in_dim(x, (n, 128), (0, 1))


def iota(axis):
    return lax.broadcasted_iota(jnp.int32, (8, 128), axis)


def cmul(u, v):
    return sub(mul(u[0], v[0]), mul(u[1], v[1])), add(mul(u[0], v[1]), mul(u[1], v[0]))


def unit(turns):
    angle = turns * float(-2 * np.pi)
    return jnp.cos(angle), jnp.sin(angle)


def _radix5(x0, x1, x2, x3, x4):
    s1, d1, s2, d2 = add(x1, x4), sub(x1, x4), add(x2, x3), sub(x2, x3)
    t = add(s1, s2)
    m = sub(x0, mul(t, 0.25))
    q = mul(sub(s1, s2), C5)
    return add(x0, t), add(m, q), add(d1, mul(d2, R5)), sub(m, q), sub(mul(d1, R5), d2)


def _radix5_t(t0, a1, b1, a2, b2):
    m = add(a1, a2)
    q = mul(sub(a1, a2), C5)
    t = sub(t0, mul(m, 0.25))
    s1, s2 = add(t, q), sub(t, q)
    d1, d2 = add(b1, mul(b2, R5)), sub(mul(b1, R5), b2)
    return add(t0, m), add(s1, d1), add(s2, d2), sub(s2, d2), sub(s1, d1)


def _half4(u, v):
    return add(u[0], v[0]), add(u[1], v[1]), sub(u[0], v[0]), sub(u[1], v[1])


def _finish4(e, o, sign):
    pr, pi, mr, mi = e
    sr, si, tr, ti = o
    o0, o2 = (add(pr, sr), add(pi, si)), (sub(pr, sr), sub(pi, si))
    oa, ob = (add(mr, ti), sub(mi, tr)), (sub(mr, ti), add(mi, tr))
    return (o0, oa, o2, ob) if sign < 0 else (o0, ob, o2, oa)


def _radix4(v, sign):
    return _finish4(_half4(v[0], v[2]), _half4(v[1], v[3]), sign)


def _twiddle(v, e):
    r, i = v
    e %= 16
    if e == 0:
        return r, i
    if e == 4:
        return lax.neg(i), r
    if e == 12:
        return i, lax.neg(r)
    c, s = float(np.cos(np.pi * e / 8)), float(np.sin(np.pi * e / 8))
    if e % 4 == 2:
        if c * s > 0:
            return mul(sub(r, i), c), mul(add(r, i), c)
        return mul(add(r, i), c), mul(sub(i, r), c)
    return sub(mul(r, c), mul(i, s)), add(mul(r, s), mul(i, c))


def _lhs7(i, a):
    if i == 0: return add(a(0, 0), a(1, 1))
    if i == 1: return add(a(1, 0), a(1, 1))
    if i == 2: return a(0, 0)
    if i == 3: return a(1, 1)
    if i == 4: return add(a(0, 0), a(0, 1))
    if i == 5: return sub(a(1, 0), a(0, 0))
    return sub(a(0, 1), a(1, 1))


def _rhs7(i, b):
    if i == 0: return add(b(0, 0), b(1, 1))
    if i == 1: return b(0, 0)
    if i == 2: return sub(b(0, 1), b(1, 1))
    if i == 3: return sub(b(1, 0), b(0, 0))
    if i == 4: return b(1, 1)
    if i == 5: return add(b(0, 0), b(0, 1))
    return add(b(1, 0), b(1, 1))


def _fold7(j, m, get, put, done):
    if j < 3:
        put(j, m)
    elif j == 3:
        done(1, 0, add(get(1), m))
        put(3, add(get(0), m))
    elif j == 4:
        done(0, 1, add(get(2), m))
        put(4, sub(get(3), m))
    elif j == 5:
        done(1, 1, add(add(sub(get(0, 2), get(1, 2)), get(2, 2)), m))
    else:
        done(0, 0, add(get(4), m))


LHS1 = ((2, 5), (3, 6), (0, 1, 4))
LHS2 = ((2, 3, 0), (1, 5), (4, 6))
RHS = ((1, 4, 0), (2, 5), (3, 6))
_FIRST = [7 * i + j for group in LHS1 for i in group for j in range(7)]
EARLY = ([(0, 1, ij) for ij in _FIRST[:24]], [(0, 1, ij) for ij in _FIRST[24:40]],
         [(0, 2, ij) for ij in _FIRST[40:48]], [(1, 3, ij) for ij in _FIRST[:12]])
DONE = {ij: hi for part in EARLY for _, hi, ij in part}


def quarters(j):
    cuts = sorted({128 * j, 128 * j + 128} | {c for c in (160, 320, 480) if 128 * j < c < 128 * j + 128})
    return [(lo // 160, lo % 160, hi - lo) for lo, hi in zip(cuts, cuts[1:])]


def _nt(a, b):
    return lax.dot_general(a, b, (((1,), (1,)), ((), ())), preferred_element_type=f32)


def _nn(a, b):
    return lax.dot_general(a, b, (((1,), (0,)), ((), ())), preferred_element_type=f32)


def _merge(*streams):
    order = []
    for si, st in enumerate(streams):
        st, t0, t1 = st if isinstance(st, tuple) else (st, 0.0, 1.0)
        tot, acc = float(sum(t[0] for t in st)) or 1.0, 0.0
        for t in st:
            order.append((t0 + (t1 - t0) * (acc + (0.5 * t[0] if si else 0.0)) / tot, si, len(order), t))
            acc += t[0]
    for _, _, _, t in sorted(order, key=lambda o: o[:3]):
        t[1](*t[2:])


class Bank:
    def __init__(self, refs, offsets, cols, nrows, packed=0, chained=0):
        self.refs, self.offsets, self.nrows, self.packed, self.chained = refs, offsets, nrows, packed, chained
        self.cache, self.count, self.held = {}, 0, None

    @staticmethod
    def shapes(count, cols, nrows, packed=0, chained=0):
        n = ((cols + packed) >> packed) * (nrows >> packed) + 8
        return [pltpu.VMEM(((n + 31) // 32 * 32, 128 << packed), u32 if packed else f32) for _ in range(count)]

    def view(self, k, via):
        if (k, via) not in self.cache:
            r = self.refs[k]
            self.cache[k, via] = r.at[pl.ds(self.offsets[via], r.shape[0])] if via else r
        return self.cache[k, via]

    def get(self, k, col, lo=0, n=None, via=1):
        lo += (col >> self.packed) * self.nrows
        x = self.view(k, via)[lo >> self.packed:(lo + (n or self.nrows)) >> self.packed, L(col & self.packed)]
        return pltpu.bitcast(x, bf16) if self.packed else x

    def wide(self, k, cols, via=1):
        return lax.concatenate([self.get(k, c, via=via) for c in cols], 1)

    def halves(self, k, c, via=1):
        return cat(self.get(k, 2 * c, via=via), self.get(k, 2 * c + 1, via=via))

    def put(self, k, col, lo, x):
        if self.packed and col % 2 == 0:
            self.held = x
            return
        if self.packed:
            x = pltpu.bitcast(cast(lax.concatenate([self.held, x], 1), bf16), u32)
        at = ((col >> self.packed) * self.nrows + lo) >> self.packed
        self.count += 1
        self.view(k, (0, 6 + self.count % 2, 6)[self.chained])[at:at + x.shape[0], :] = x

    def clear_tokens(self):
        for r in self.refs:
            r[r.shape[0] - 8:r.shape[0], L(0)] = jnp.zeros((8, 128), r.dtype)

    def token(self, k):
        n = self.refs[k].shape[0]
        return (id(self), k), self.refs[k][n - 8:n, L(0)]


class Table(Bank):
    def __init__(self, refs, offsets, nrows, groups, chained):
        super().__init__(refs, offsets, None, nrows, 1, chained)
        self.slot = {i: (g, 7 * k) for g, group in enumerate(groups) for k, i in enumerate(group)}

    @staticmethod
    def shapes(tiles, nrows, groups, chained):
        return [s for _ in range(tiles) for g in groups for s in Bank.shapes(1, 7 * len(g), nrows, 1)]

    def load(self, k, i, j, via, lo=0, n=None):
        g, s = self.slot[i]
        return self.get(3 * k + g, s + j, lo, n, via)

    def store(self, k, i, j, lo, val):
        g, s = self.slot[i]
        self.put(3 * k + g, s + j, lo, val)

    def tiles(self, ij, ks, via, axis=1):
        return lax.concatenate([self.load(k, ij // 7, ij % 7, via) for k in ks], axis)


BANKS = dict(
    x0=(Bank, 4, 4, D),
    x1=(Bank, 4, 4, D),
    va=(Bank, 8, 4, BINS), vb=(Bank, 16, 4, 168),
    mr2=(Bank, 12, 2, 2 * BINS),
    wt=(Bank, 4, 4, F - MAIN, 1, 2), br=(Bank, 4, 12, 64, 1, 1), tb=(Bank, 4, 40, 64, 1, 1),
    a1=(Table, 4, 160, LHS1, 2), hp=(Bank, 4, 12, 160, 1, 2), bt=(Bank, 1, 1, 256),
    a2=(Table, 3, 160, LHS2, 1), ar=(Bank, 1, 18, 128, 1, 2),
    b1=(Table, 12, 128, RHS, 1), b2=(Table, 12, 128, RHS, 1),
    lo=(Bank, 10, 1, 160), hi=(Bank, 10, 4, 160), zb=(Bank, 4, 12, BINS, 1, 1),
    post=(Bank, 1, 1, 240, 1, 2), sm=(Bank, 1, 48, 128, 1), mean=(Bank, 4, 4, 40, 0, 2), sums=(Bank, 4, 4, 64))

BIAS1, BIAS2, MEAN, SCALE, SHIFT = 0, 16, 32, 48, 64


def _kernel(x_hbm, wr_hbm, wi_hbm, w1_hbm, b1_hbm, w2_hbm, b2_hbm, dm_hbm, o_hbm,
            b1_ref, b2_ref, wrb, wib, w1b, w2b, dm_ref, wp, wt, small, sems, kept):
    zero = iota(1)[0, 0]
    zs = [None] + [pl.multiple_of(zero << (4 + k), 16) for k in range(7)]
    m = {name: spec[0](kept[name], zs, *spec[2:]) for name, spec in BANKS.items()}
    pool, a1, a2 = kept["mr2"], kept["a1"], kept["a2"]
    m.update(k1=Bank(pool[:8], zs, 4, BINS), hb=Bank(pool[8:12], zs, 4, BINS), part=Bank(pool[:6] + pool[8:9], zs, 8, 160),
             mr1=Bank(pool[6:8], zs, 5, F - MAIN), d0=Bank(pool[9:], zs, 4, 128),
             yb=Bank(a1[2::3] + a1[0::3], zs, 6, BINS, 1))

    def dm(p):
        return pltpu.bitcast(dm_ref[:, L(p)], bf16)

    wpr = [r.at[pl.ds(zs[1], 2)] for r in wp]
    w_rd = [[r.at[pl.ds(zs[1 + g], F)] for g in range(3)] for r in (w1b, w2b)]
    tokens, ready, backlog, plain = [], set(), [], {}

    def row(i, n):
        return bcast(small[i:i + 1, :], n)

    def paced(a):
        if not tokens:
            return a
        n, gates = a.shape[0] // 16, {}
        for i, (key, tok) in enumerate(tokens):
            gates.setdefault(max((i + 1) * n // len(tokens) - 1, 0), {})[key] = tok
        tokens.clear()
        parts, lo = [], 0
        for r in sorted(gates):
            if r > lo:
                parts.append(lax.slice(a, (16 * lo, 0), (16 * r, 128)))
            w = pltpu.bitcast(lax.slice(a, (16 * r, 0), (16 * r + 16, 128)), u32)
            for tok in gates[r].values():
                w = lax.bitwise_or(w, lax.bitcast_convert_type(tok, u32))
            parts.append(pltpu.bitcast(w, bf16))
            lo = r + 1
        if lo < n:
            parts.append(lax.slice(a, (16 * lo, 0), (16 * n, 128)))
        left = cat(*parts)
        return left if a.shape[1] == 128 else lax.concatenate([left, lax.slice(a, (0, 128), a.shape)], 1)

    def copy(src, dst, group):
        return pltpu.make_async_copy(src, dst, sems.at[group])

    order = [a + 4 * b for a in range(4) for b in range(4)]
    x_cp = {t: copy(x_hbm.at[L(t), :], w2b.at[L(t // 3), L(5 * (t % 3), 5)], (0, 1, 2, 2, 3, 3, 4, 4)[k // 2])
            for k, t in enumerate(order)}
    o_cp = {t: [copy(w1b.at[L(t // 3), L(5 * (t % 3) + j, n)], o_hbm.at[L(t), L(j, n)], 5)
                for j, n in (((0, 3), (3, 2)) if t % 4 == 3 else ((0, 5),))] for t in order}
    nudges = []

    def launch(*copies):
        k = len(nudges)
        nudges.append(copy(dm_hbm.at[0:8, L(0)], m["post"].view(0, 5).at[8 * k:8 * k + 8, L(0)], 5))
        for c in copies + (nudges[-1],):
            c.start()
        tokens.append(m["post"].token(0))

    w_cp = {(k, n): copy(src.at[lo:hi, :], dst.at[lo:hi, :], 3 if k or n == 3 else 4) for k, (src, dst) in enumerate(((w1_hbm, w1b), (w2_hbm, w2b)))
            for n, (lo, hi) in enumerate(((0, 512), (512, 1024), (1024, MAIN), (MAIN, F))) if k or n}
    w_cp[0, 0] = [copy(w1_hbm.at[0:512, L(t)], w1b.at[0:512, L(t)], 0 if k < 8 else 3) for k, t in enumerate(order)]

    def get_v(name, a, q, lo, n):
        return m[name].get(2 * a, q, lo, n), m[name].get(2 * a + 1, q, lo, n)

    def put_v(name, a, q, lo, val):
        m[name].put(2 * a, q, lo, val[0])
        m[name].put(2 * a + 1, q, lo, val[1])

    def gather(acc, t, *xs):
        acc[t, 0] = add(acc.get((t, 0)), tree(xs))
        acc[t, 1] = add(acc.get((t, 1)), tree([mul(x, x) for x in xs]))

    def moments(acc, t):
        mean = jnp.sum(acc[t, 0], axis=0, keepdims=True) * (1.0 / D)
        return mean, jnp.maximum(jnp.sum(acc[t, 1], axis=0, keepdims=True) * (1.0 / D) - mean * mean, 0.0)

    def norm_once(acc, t):
        mean, var = moments(acc, t)
        small[MEAN + t:MEAN + t + 1, :] = mean
        small[SCALE + t:SCALE + t + 1, :] = lax.rsqrt(var + EPS)

    def load_x(t):
        eye = (lax.broadcasted_iota(jnp.int32, (128, 128), 0) == lax.broadcasted_iota(jnp.int32, (128, 128), 1)).astype(bf16)
        xt = _nt(paced(eye), jnp.concatenate([w2b[L(t // 3), L(5 * (t % 3) + j)] for j in range(5)], axis=0))
        acc = {}
        for c in range(16):
            x = [lax.slice(xt, (8 * c, 128 * j), (8 * c + 8, 128 * j + 128)) for j in range(5)]
            for j in range(5):
                m["x0"].put(t % 4, t // 4, 128 * j + 8 * c, x[j])
            gather(acc, t, *x)
        norm_once(acc, t)

    def fwd10(t, c):
        halves = []
        m10, r = mul(row(MEAN + t, 8), 10.0), row(SCALE + t, 8)
        for h in range(2):
            x = [m["x0"].get(t % 4, t // 4, 64 * i + 16 * c + 8 * h, 8) for i in range(10)]
            e = _radix5(*[add(x[i], x[i + 5]) for i in range(5)])
            o = _radix5(*[sub(x[i], x[i + 5]) if i % 2 == 0 else sub(x[i + 5], x[i]) for i in range(5)])
            halves.append([mul(v, r) for v in (sub(e[0], m10), o[0], e[1], e[2], e[3], e[4], o[1], o[2], o[3], o[4])])
        for i in range(10):
            m["tb"].put(t % 4, 10 * (t // 4) + i, 16 * c, cat(halves[0][i], halves[1][i]))
        tokens.append(m["tb"].token(t % 4))

    def fwd_d(a, p):
        g = _nn(paced(dm(p)), lax.concatenate([m["tb"].halves(a, 5 * b + p) for b in range(4)], 1))
        for c in range(8):
            v = [(lax.slice(g, (16 * c, 128 * b), (16 * c + 8, 128 * b + 128)),
                  lax.slice(g, (16 * c + 8, 128 * b), (16 * c + 16, 128 * b + 128))) for b in range(4)]
            if p == 0 and c == 0:
                for q, w in enumerate(_radix4([(i, jnp.zeros((8, 128), f32)) for (_, i) in v], -1)):
                    w = _twiddle(w, -q * a)
                    put_v("va", a, q, 320, (cat(w[0], w[0]), cat(w[1], w[1])))
                v = [(r, jnp.where(iota(0) == 0, 0.0, i)) for (r, i) in v]
            for q, w in enumerate(_radix4(v, -1)):
                put_v("va", a, q, 80 * (c % 4) + 16 * p + 8 * (c // 4), _twiddle(w, -q * a))

    def permute_w(get, put):
        cur = [get((-k) % 16) for k in range(16)]
        cur = [pltpu.roll(c, (-k) % 16, 1) if k else c for k, c in enumerate(cur)]
        for bit in (1, 2, 4, 8):
            msk = (iota(1) & bit) != 0
            cur = [lax.select(msk, cur[(k - bit) % 16], cur[k]) for k in range(16)]
        for k in range(16):
            put(k, cur[k])

    def prep_w(src, ri, part, c):
        if c < 20:
            def put(k, v):
                wp[part][ri, k, 8 * (c - 5 * part):8 * (c - 5 * part) + 8, :] = v
            permute_w(lambda t: pltpu.bitcast(src[16 * c:16 * c + 16, L(t)], u32), put)
        else:
            def put(k, v):
                wt[ri, k] = v
            permute_w(lambda t: bcast(cast(src[320:321, L(t)], f32), 8), put)

    def w_rows(ri, k1, c):
        if c == 20:
            v = wt[ri, k1]
            return cat(v, v)
        out = []
        for k in TILE_CLASSES[c % 5]:
            v = wpr[min(c // 5, 2)][ri, k1, pl.ds(k // 2 + 40 * (c // 15), 8, stride=5), :]
            out.append(lax.bitwise_and(v, lax.full(v.shape, 0xFFFF0000, u32)) if k % 2 else lax.shift_left(v, lax.full(v.shape, 16, u32)))
        return pltpu.bitcast(cat(*out), f32)

    def s_in(q, c):
        z = _radix4([get_v("va", a, q, 16 * c, 16) for a in range(4)], -1)
        for p in range(4):
            for j, val in enumerate((add(z[p][0], z[p][1]), z[p][0], z[p][1])):
                m["zb"].put(q, 3 * p + j, 16 * c, val)
        tokens.append(m["zb"].token(q))

    def spectral(extra):
        units = [(h, q) for h in range(2) for q in range(4)]

        def s_dot(h, q, p, j, inverse):
            lo, n = 160 * h, 160 + 16 * h
            lhs = paced(m["yb"].get(2 * q + p % 2, 3 * (p // 2) + j, lo, n) if inverse else m["zb"].get(q, 3 * p + j, lo, n))
            return (_nt if inverse else _nn)(lhs, m["sm"].get(0, 16 * j + q + 4 * p, via=1 + 2 * h + inverse))

        def s_fwd(h, q, ps):
            prod = {(p, j): s_dot(h, q, p, j, 0) for p in ps for j in (1, 2)}
            for k in range(10 + h):
                c = 10 * h + k
                for p in ps:
                    both = m["k1"].get(2 * q, p, 16 * c, 16)
                    x = sub(both, rows(prod[p, 2], 16 * k, 16)), add(both, rows(prod[p, 1], 16 * k, 16))
                    yr, yi = cmul(x, (w_rows(0, q + 4 * p, c), w_rows(1, q + 4 * p, c)))
                    for j, val in enumerate((add(yr, yi), yi, yr)):
                        m["yb"].put(2 * q + p % 2, 3 * (p // 2) + j, 16 * c, val)

        def s_inv(h, q, odd):
            ps = (odd, odd + 2)
            prod = {(p, j): s_dot(h, q, p, j, 1) for p in ps for j in (1, 2)}
            for k in range(20 + h):
                lo, z = 160 * h + 8 * k, []
                for p in ps:
                    both = m["k1"].get(2 * q + 1, p, lo, 8)
                    z.append((add(both, rows(prod[p, 1], 8 * k, 8)), sub(both, rows(prod[p, 2], 8 * k, 8))))
                half = _half4(*z)
                if not odd:
                    for j in range(4):
                        m["hb"].put(q, j, lo, half[j])
                else:
                    for a, w in enumerate(_finish4([m["hb"].get(q, j, lo, 8) for j in range(4)], half, 1)):
                        put_v("vb", 4 * h + a, q, 8 * k, _twiddle(w, q * a))

        for c in range(10):
            s_in(0, c)
        tokens.clear()
        for u in range(9):
            now, before = units[u] if u < 8 else None, units[u - 1] if u else None
            common = ([now + (0,)] if now else []) + ([before + (1,)] if before else [])
            side, more = list(extra[u][0]), extra[u][1]
            if u < 7:
                h, q = units[u + 1]
                side += [(1, s_in, q, 10 * h + k) for k in range(10 + h)]
            early = [(1, inv4, a, p, c) for a in range(4) for p in range(5) for c in range(2)][u - 5::4] if u > 4 else []
            for k, (h, q, inverse) in enumerate(common):
                _merge(side[k * len(side) // len(common):(k + 1) * len(side) // len(common)])
                for p in range(4):
                    m["k1"].put(2 * q + inverse, p, 160 * h, s_dot(h, q, p, 0, inverse))
            for odd in range(2):
                if now:
                    s_fwd(*now, (odd, odd + 2))
                if before:
                    _merge(early[odd::2], more if odd == 0 else [])
                    s_inv(*before, odd)

    def inv4(a, p, c):
        g = _radix4([get_v("vb", 4 * (c // 2) + a, q, 80 * (c % 2) + 16 * p, 16) for q in range(4)], 1)
        if (p, c) == (0, 0):
            for b in range(4):
                m["mean"].put(a, b, 0, cat(*g[b]))
            return
        for b in range(4):
            for j in range(2):
                m["tb"].put(a, 10 * b + 2 * p + j, 16 * c, g[b][j])
        tokens.append(m["tb"].token(a))

    def real_bins(a):
        ny = _radix4([get_v("vb", 4 + a, q, 160, 8) for q in range(4)], 1)
        for b in range(4):
            t = a + 4 * b
            g = m["mean"].get(a, b, 0, 32)
            m["tb"].put(a, 10 * b, 0, rows(g, 0, 16))
            m["tb"].put(a, 10 * b + 1, 0, cat(lax.select(iota(0) == 0, ny[b][0], rows(g, 16, 8)), rows(g, 24, 8)))
            mean = small[MEAN + t:MEAN + t + 1, :] + rows(g, 0, 1) * (1.0 / (S * D))
            small[SHIFT + t:SHIFT + t + 1, :] = small[BIAS2 + t:BIAS2 + t + 1, :] + mean
            m["mean"].put(a, b, 32, bcast(mean, 8))
        tokens.append(m["mean"].token(a))

    def inv_d0(a):
        for b in range(4):
            m["d0"].put(a % 2, b, 0, _nn(paced(dm(5)), m["tb"].halves(a, 5 * b)))

    def inv_d(a, b):
        t = a + 4 * b
        tt = [_nn(dm(5 + p), m["tb"].halves(a, 5 * b + p)) for p in range(1, 5)]
        mean, sq = m["mean"].get(a, b, 32, 8), None
        for c in range(8):
            v = [rows(tt[i // 2], 16 * c + 8 * (i % 2), 8) for i in range(8)]
            e = _radix5_t(sub(m["d0"].get(a % 2, b, 16 * c, 8), mean), *v[0:4])
            o = _radix5_t(m["d0"].get(a % 2, b, 16 * c + 8, 8), *v[4:8])
            part = []
            for i in range(5):
                for j, sg in ((i, i % 2), (i + 5, 1 - i % 2)):
                    x = add(m["x0"].get(a, b, 64 * j + 8 * c, 8, 2), (sub if sg else add)(e[i], o[i]))
                    m["x1"].put(a, b, 64 * j + 8 * c, x)
                    part.append(mul(x, x))
            sq = add(sq, tree(part))
        var = jnp.sum(sq, axis=0, keepdims=True) * (1.0 / D)
        r = lax.rsqrt(var + EPS)
        small[SCALE + t:SCALE + t + 1, :] = r * lax.rsqrt(var * r * r + EPS) * 0.5

    def split2(load, pick, put, group, gate=None):
        seen = {}

        def blk(i, j):
            if (i, j) not in seen:
                seen[i, j] = load(i, j)
            return seen[i, j]
        for i in group:
            h = {(r, k): pick(i, lambda r1, k1: blk(2 * r1 + r, 2 * k1 + k)) for r in range(2) for k in range(2)}
            for j in range(7):
                put(i, j, pick(j, lambda r, k: h[r, k]))
            if i == group[-1] and len(group) % 2:
                put(i, 7, pick(6, lambda r, k: h[r, k]))
            if gate:
                tokens.append(gate())

    def lhs1(a, v, g):
        def load(r, k):
            t = a + 4 * k
            h = mul(m["x1"].get(a, k, 160 * r + 16 * v, 16, 3 + g), row(SCALE + t, 16))
            if r != k and g == k // 2:
                m["hp"].put(a, plain.setdefault((r, k), len(plain)), 16 * v, h)
            return h

        def put(i, j, val):
            m["a1"].store(a, i, j, 16 * v, val)
        split2(load, _lhs7, put, LHS1[g])
        tokens.append(m["hp"].token(a))
        tokens.append(m["a1"].token(3 * a + g))

    def weights(which, g, lo, t):
        return cast(w_rd[which][g][lo:lo + 16, L(t)], f32)

    def rhs_main(which, n, a, v, g):
        def raw(f, s):
            lo = 128 * (4 * n + f) + 16 * v
            return weights(which, g, lo, a + 4 * s)
        tab = m[("b1", "b2")[which]]
        split2(raw if which else lambda s, f: raw(f, s), _rhs7,
               lambda i, j, val: tab.store(4 * n + a, i, j, 16 * v, val), RHS[g], lambda: tab.token(3 * (4 * n + a) + g))

    def rhs_rest(a, pair, v):
        (p1, p2, p3), (q1, q2, q3) = ([weights(1, 0, MAIN + 64 * k + 16 * v, a + 8 * pair + 4 * e) for k in range(3)] for e in range(2))
        for k, val in enumerate((sub(p1, q1), p2, q2, sub(q3, p3), q1, p3)):
            m["br"].put(a, 6 * pair + k, 16 * v, val)
        tokens.append(m["br"].token(a))

    def rhs_main_tasks(which, ns, as_, gs=range(3)):
        return [(36 * len(RHS[g]), rhs_main, which, n, a, v, g) for g in gs for n in ns for a in as_ for v in range(8)]

    def rhs_rest_tasks():
        return [(22, rhs_rest, a, pair, v) for a in range(4) for pair in range(2) for v in range(4)]

    def gelu_half(u):
        inner = mul(u, add(mul(mul(u, u), 8 * GELU * 0.044715), lax.full(u.shape, 2 * GELU, f32)))
        return add(u, mul(u, lax.tanh(inner)))

    def fold49(ij, flip, prod, done):
        i, j = divmod(ij, 7)
        for v in range(20):
            def slot(bank, par, col):
                return (lambda k, via=1: bank.get(5 * par + k, col, 8 * v, 8, via),
                        lambda k, val: bank.put(5 * par + k, col, 8 * v, val))

            def inner(r, n, h):
                _fold7(i, h, *slot(m["hi"], flip, 2 * r + n), lambda r1, n1, c: done(2 * r1 + r, 2 * n1 + n, v, c))
            _fold7(j, rows(prod, 8 * v, 8), *slot(m["lo"], i % 2, 0), inner)

    def stage_w1(a, k):
        for e in (2 * k, 2 * k + 1):
            m["wt"].put(a, e, 0, cast(w1b[MAIN:F, L(a + 4 * e)], f32))
        tokens.append(m["wt"].token(a))

    def mm1_rest(a, j):
        def h(k):
            return cat(*[m["hp"].get(a, plain[r, k], lo, n) if r != k else m["a1"].load(a, 2 + k // 2, 2 + k % 2, 4, lo, n)
                         for r, lo, n in quarters(j)])
        w = m["wt"].wide(a, range(4), via=1 + j)
        prod = _nt(paced(w), lax.concatenate([h(k) for k in range(4)], 1))
        for lo in range(0, F - MAIN, 8):
            u = add(rows(prod, lo, 8), m["mr1"].get(1 - a % 2, j, lo, 8) if a else m["bt"].get(0, 0, lo, 8, 1 + j))
            m["mr1"].put(a % 2, j, lo, gelu_half(u) if a == 3 else u)

    def mm1_early(lo, hi, ij):
        prod = _nt(paced(m["a1"].tiles(ij, range(lo, hi), 5)), m["b1"].tiles(ij, range(lo, hi), 2))
        m["part"].put(ij // 8, ij % 8, 0, add(prod, m["part"].get(ij // 8, ij % 8, via=2) if lo else None))

    def mm1_main(n, ij):
        def done(r, f, v, u):
            m["vb"].put(4 * (n % 2) + r, f, 8 * v, gelu_half(add(u, row(BIAS1 + 4 * n + f, 8))))
        k = DONE.get(ij, 0) if n == 0 else 0
        prod = _nt(paced(m["a1"].tiles(ij, range(k, 4), 1 + n)), m["b1"].tiles(ij, range(4 * n + k, 4 * n + 4), 1))
        if k:
            prod = add(prod, m["part"].get(ij // 8, ij % 8, 0, 160))
        fold49(ij, n % 2, prod, done)

    def lhs_rest(j, k):
        for e in range(2):
            g = cat(*[m["mr1"].get(1, 2 * j + e, 64 * u, 64, 1 + k) if 2 * j + e < 5 else jnp.zeros((64, 128), f32)
                      for u in ((0, 1), (1, 2), (0, 2))[k]])
            m["ar"].put(0, 6 * k + 2 * j + e, 0, g.T)
        tokens.append(m["ar"].token(0))

    def lhs2(n, v, g):
        split2(lambda r, f: m["vb"].get(4 * (n % 2) + r, f, 16 * v, 16, 1 + g), _lhs7,
               lambda i, j, val: m["a2"].store(n, i, j, 16 * v, val), LHS2[g], lambda: m["a2"].token(3 * n + g))

    def lhs2_tasks(n):
        return [(23 * len(LHS2[g]), lhs2, n, v, g) for v in range(10) for g in range(3)]

    def mm2_rest(a, k, r):
        lhs = paced(cat(*[m["ar"].get(0, 6 * k + j, lo - 128 * j, n, 1 + a) for j in range(5)
                          for q, lo, n in ((q, 160 * q + at, n) for q, at, n in quarters(j)) if q == r]))
        prod = _nn(lhs, lax.concatenate([m["br"].halves(a, 3 * e + k, 1 + r) for e in range(2)], 1))
        for e in range(2):
            m["mr2"].put(3 * a + k, e, 160 * r, lax.slice_in_dim(prod, 128 * e, 128 * e + 128, axis=1))

    def write_out(t, j):
        x = m["x0"].get(t % 4, t // 4, 128 * j, 128, 3) if t % 4 < 3 else cat(
            *[m["vb"].get(4 * r + t // 4, 0, lo, n, 4) for r, lo, n in quarters(j)])
        out = x.T
        w1b[L(t // 3), L(5 * (t % 3) + j)] = cast(out, bf16)
        m["mean"].put(0, 0, 0, rows(out, 120, 8))
        tokens.append(m["mean"].token(0))

    def mm2_main(a, ij, first):
        acc = {}
        def done(r, b, v, y):
            rest = [m["mr2"].get(3 * a + k, b // 2, 160 * r + 8 * v, 8, 1 + b % 2) for k in (b % 2, 2)]
            x = add(add(m["x1"].get(a, b, 160 * r + 8 * v, 8), row(SHIFT + a + 4 * b, 8)), add(y, add(*rest)))
            if first or a < 3:
                m["x0"].put(a, b, 160 * r + 8 * v, x)
            else:
                m["vb"].put(4 * r + b, 0, 8 * v, x)
            if first:
                gather(acc, 0, x)
                if v == 19:
                    m["sums"].put(a, b, 16 * r, cat(acc[0, 0], acc[0, 1]))

        prod = _nn(paced(m["a2"].tiles(ij, range(3), 1 + a)), m["b2"].tiles(ij, range(a, 12, 4), 1, 0))
        fresh = set()
        fold49(ij, (a + 1) % 2, prod, lambda r, b, v, y: (done(r, b, v, y), fresh.add((r, b))))
        if a == 3 and not first:
            for r, b in sorted(fresh):
                t = a + 4 * b
                ready.add((r, t))
                for j in range(5):
                    need = {(128 * j // 160, t), ((128 * j + 127) // 160, t)}
                    if (r, t) in need and need <= ready:
                        backlog.append((ij, write_out, t, j))
                for part, need in enumerate(({(0, t), (1, t), (2, t)}, {(2, t), (3, t)})):
                    if (r, t) in need and need <= ready:
                        backlog.append((ij, launch, o_cp[t][part]))
            for _ in range(2 if ij < 48 else 99):
                if backlog and (backlog[0][0] + 4 <= ij or ij == 48):
                    _, fn, *args = backlog.pop(0)
                    args[0].start() if fn is launch and ij == 48 else fn(*args)

    def norm_sums(a, b):
        tot = None
        for r in range(4):
            tot = add(tot, m["sums"].get(a, b, 16 * r, 16))
        norm_once({(a + 4 * b, j): rows(tot, 8 * j, 8) for j in range(2)}, a + 4 * b)

    def after_mm2(a, first):
        if not first:
            return ([(30, write_out, a + 4 * b, j) for b in range(4) for j in range(5)] +
                    [(30, launch, *[o_cp[a + 4 * b][0] for b in range(4)])]) if a < 3 else []
        return ([(20, norm_sums, a, b) for b in range(4)] +
                [(115, fwd10, a + 4 * b, c) for b in range(4) for c in range(4)])

    def post_stage(first):
        def inv4_tasks(a):
            return [(20, real_bins, a)] + [(40, inv4, a, p, c) for p in range(5) for c in (2, 3)]
        sums = [rhs_main_tasks(0, [0], [a]) if first else [] for a in range(4)]
        plan = [[(hi - lo, mm1_early, lo, hi, ij) for lo, hi, ij in part] for part in EARLY]
        for a in range(4):
            _merge(inv4_tasks(a)[:3])
            inv_d0(a)
            _merge(inv4_tasks(a)[3:])
            tokens.clear()
            side = [[(30 * len(LHS1[g]), lhs1, a, v, g) for v in range(10)] for g in range(3)]
            for b in range(4):
                inv_d(a, b)
                if a == 0 and b == 2:
                    _merge(side.pop(0))
                    tokens.clear()
                if a or b >= 2:
                    n = 4 // plan[a][0][0]
                    _merge(plan[a][:n])
                    del plan[a][:n]
            if first:
                side.append([(40, stage_w1, a, k) for k in range(2)] + (sums[2] if a == 1 else []))
            if a == 0:
                n = 14 - (24 - len(plan[0]))
                _merge(plan[0][:n], (side.pop(0), -0.2, 0.5))
                tokens.clear()
                del plan[0][:n]
            _merge([(4.8, mm1_rest, a - 1, j) for j in range(5 if a else 0)] + plan[a],
                   ([t for part in side for t in part], 0.0, 0.8))
        if first:
            for k in (3, 0, 1, 2):
                w_cp[1, k].start()
            w_cp[0, 1].wait()
            w_cp[0, 2].wait()
        _merge([(1, mm1_rest, 3, j) for j in range(5)], (sums[3][:8], -0.2, 0.8))

    cut = (32, 72, 150, 202, 240, 288)

    def w2_sums():
        return [t for a in range(4) for g in range(3) for t in rhs_main_tasks(1, range(3), [a], (g,))]

    def mm1_stage(first):
        for n in range(3):
            late, sums = [], []
            if first:
                late = rhs_main_tasks(0, [n], range(4) if n else [3], (1, 2))
                sums = rhs_main_tasks(0, [n + 1], range(4), (0,)) if n < 2 else [(0, w_cp[1, k].wait) for k in range(4)] + rhs_rest_tasks() + w2_sums()[:cut[0]]
            _merge([(1, mm1_main, n, ij) for ij in range(49)],
                   (lhs2_tasks(n - 1) if n else [], 0.45, 0.97),
                   ([(1, lhs_rest, j, k) for j in range(3) for k in range(3)] if n == 2 else [], 0.4, 0.95),
                   (late, 0.0, 0.39), (sums, 0.4 if n else 0.0, 0.95))

    def mm2_stage(first):
        sums = w2_sums() if first else []
        _merge([(1, mm2_rest, a, k, r) for a in range(4) for k in range(3) for r in range(4)], (lhs2_tasks(2), 0.0, 0.9), (sums[cut[0]:cut[1]], 0.0, 0.9))
        for a in range(4):
            _merge([(1, mm2_main, a, ij, first) for ij in range(49)],
                   (after_mm2(a - 1, first) if a else [], 0.1 if a < 3 or not first else 0.4, 0.95 if first else 0.45),
                   (sums[cut[a + 1]:cut[a + 2]], 0.0, 0.95 if a < 3 else 0.39))
        _merge([(1, fwd_d, a, p) for a in range(3) for p in range(5)] if first else [], (after_mm2(3, first), 0.0, 0.9))
        tokens.clear()
        if first:
            for p in range(5):
                fwd_d(3, p)
        else:
            for c in nudges + [c for t in order for c in o_cp[t]]:
                c.wait()

    def token_mixing(first):
        tokens.clear()
        post_stage(first)
        mm1_stage(first)
        mm2_stage(first)

    def first_transform():
        cuts = (0, 80, 160, 321)
        dm_cp = copy(dm_hbm.at[:, L(0, 5)], dm_ref.at[:, L(0, 5)], 2)
        small_cp = [copy(dm_hbm.at[:, L(5, 5)], dm_ref.at[:, L(5, 5)], 0), copy(b1_hbm, b1_ref, 0),
                    copy(b2_hbm, b2_ref.at[0:16, :], 0)]
        f_cp = [[copy(src.at[lo:hi, :], dst.at[lo:hi, :], k) for src, dst in ((wr_hbm, wrb), (wi_hbm, wib))]
                for k, (lo, hi) in enumerate(zip(cuts, cuts[1:]))]

        def prep(k):
            return [(1, prep_w, src, ri, k, c) for c in range(cuts[k] // 16, (cuts[k + 1] + 15) // 16)
                    for ri, src in enumerate((wrb, wib))]

        def fly(tiles):
            return [(1, fwd10, t, c) for t in tiles for c in range(4)]

        def start():
            for name in BANKS:
                if m[name].chained:
                    m[name].clear_tokens()
            launch(*[x_cp[t] for t in order[:6]])
            gate = lax.bitcast_convert_type(tokens.pop()[1], jnp.int32)
            s2, lane = (lax.broadcasted_iota(jnp.int32, (16, 128), k) for k in range(2))
            s2, lane = s2 + cat(gate, gate), lane + cat(gate, gate)
            k2 = ((lane & 15) << 3) + (lane >> 4)
            base, hop = (unit(cast(k & 127, f32) * (1.0 / 128)) for k in (s2 * k2, 16 * k2))
            step = unit(cast(s2, f32) * (1.0 / S))
            for c in range(8):
                if c:
                    base, step = cmul(base, hop), cmul(step, (float(np.cos(np.pi / 64)), float(-np.sin(np.pi / 64))))
                re, im = base
                for k1 in range(0, 16, 2):
                    nxt = cmul((re, im), step)
                    two = [[pltpu.roll(x, k, 1) if k else x for x in z] for k, z in enumerate(((re, im), nxt), k1)]
                    for j in range(3):
                        for k, (x, y) in enumerate(two, k1):
                            m["sm"].put(0, 16 * j + k, 16 * c, (x, sub(y, x), add(x, y))[j])
                    re, im = cmul(nxt, step)
            queue = [[x_cp[t] for t in order[k:k + 2]] + [dm_cp] * (k == 6) for k in range(6, 16, 2)] + f_cp[:2] + [[]]
            for before, lo, hi in ((0, 0, 2), (0, 2, 4), (2, 4, 8), (4, 8, 12), (8, 12, 16)):
                for c in queue.pop(0):
                    c.start()
                for c in [x_cp[t] for t in order[lo:hi]] + [dm_cp] * (lo == 4):
                    c.wait()
                _merge([(1, load_x, t) for t in order[lo:hi]] + [(0.8, fwd_d, lo // 4 - 1, p) for p in range(5 * (lo > 3))],
                       (fly(order[before:lo]), -0.2, 0.6 if lo == 2 else 0.3),
                       (fly(order[12:] if hi == 16 else []), 0.5, 0.88),
                       ([(1, launch, *queue.pop(0))] if lo > 3 else [], 0.2, 0.3))
                tokens.clear()
            for c in f_cp[2]:
                c.start()
            for c in f_cp[0]:
                c.wait()
            _merge([(1, fwd_d, 3, p) for p in range(5)], prep(0))

        def prep_bias():
            half = jnp.concatenate([b1_ref[...].astype(f32).reshape(1, F), jnp.zeros((1, 64), f32)], axis=1) * 0.5
            for n in range(14):
                if n < 12:
                    small[BIAS1 + n:BIAS1 + n + 1, :] = half[:, L(n)]
                else:
                    m["bt"].put(0, 0, 128 * (n - 12), bcast(half[:, L(n)], 128).T)
            small[BIAS2:BIAS2 + 16, :] = b2_ref[0:16, :].astype(f32)

        def rest():
            for c in small_cp + w_cp[0, 0][:4]:
                c.start()
            for c in f_cp[1]:
                c.wait()
            _merge(prep(1))
            sums = rhs_main_tasks(0, [0], [0, 1])
            cut = (0, 4, 10, 28, 34, 44, 48)
            sums = [sums[lo:hi] for lo, hi in zip(cut, cut[1:])]
            none = [], []
            spectral([none, none, none,
                      ([(0, c.start) for c in w_cp[0, 0][4:8] + [w_cp[0, 3]]] + [(0, c.wait) for c in f_cp[2]] + prep(2), []),
                      none, none,
                      ([(0, c.start) for c in w_cp[0, 0][8:]] + [(0, c.wait) for c in small_cp + w_cp[0, 0][:8]] +
                       [(0, prep_bias)] + sums[0], sums[1]), sums[2:4], sums[4:6]])
            w_cp[0, 1].start()
            w_cp[0, 2].start()
            for c in [w_cp[0, 3]] + w_cp[0, 0][8:]:
                c.wait()
        start()
        rest()

    first_transform()
    token_mixing(True)
    spectral([([], [])] * 9)
    token_mixing(False)


@jax.jit
def pallas_interleave_layers__spectral_gfnet__mixer_token_mlp__prompt_kernel(A_x, A_w_r, A_w_i, B_x, B_w1, B_b1, B_w2, B_b2):
    hbm = pl.BlockSpec(memory_space=pl.ANY)
    V = pltpu.VMEM
    out = pl.pallas_call(
        _kernel,
        in_specs=[hbm, hbm, hbm, hbm, hbm, hbm, hbm, hbm],
        out_specs=hbm,
        out_shape=jax.ShapeDtypeStruct((S, D), bf16),
        scratch_shapes=[
            V((F,), bf16), V((64, 128), bf16), V((321, S), bf16), V((321, S), bf16), V((F, S), bf16), V((F, S), bf16), V((64, 1280), u32),
            [V((2, 16, n, 128), u32) for n in (40, 40, 80)], V((2, 16, 8, 128), f32), V((96, 128), f32),
            pltpu.SemaphoreType.DMA((6,)),
            {name: spec[0].shapes(*spec[1:]) for name, spec in BANKS.items()},
        ],
        compiler_params=pltpu.CompilerParams(vmem_limit_bytes=127 * 1024 * 1024, internal_scratch_in_bytes=11 * 4096),
    )(A_x.reshape(S, D), A_w_r.T, A_w_i.T, B_w1.T, B_b1, B_w2,
      B_b2.reshape(16, 128), _CHANNEL_MATRICES)
    return out.reshape(1, S, D)
```

```python
import jax
import jax.experimental.pallas as pl
import jax.experimental.pallas.tpu as pltpu
import jax.numpy as jnp
import ml_dtypes
import numpy as np
from jax import lax

S, D, F = 2048, 640, 1728
MAIN = 1536
EPS = 1e-5
BINS = 336
f32, bf16, u32 = jnp.float32, jnp.bfloat16, jnp.uint32

TILE_CLASSES = ((0, 5), (2, 8), (4, 6), (7, 3), (9, 1))
SN1, SN2 = np.sin(2 * np.pi / 5), np.sin(4 * np.pi / 5)
C5 = float(np.sqrt(5) / 4)
R5 = float(SN2 / SN1)
GELU = float(np.sqrt(2 / np.pi))


def _channel_matrices():
    d, j, i = np.arange(64), np.arange(32), np.arange(128)
    out_rows = (i // 8 % 2) * 64 + (i // 16) * 8 + i % 8
    in_rows = (i // 64) * 64 + (i // 8 % 2) * 32 + (i // 16 % 4) * 8 + i % 8
    fwd, inv = [], []
    z = np.zeros((32, 64))
    for p, (ka, kb) in enumerate(TILE_CLASSES):
        ea = np.exp(-2j * np.pi * np.outer(ka + 10 * j, d) / D)
        eb = np.exp(-2j * np.pi * np.outer(kb + 10 * j, d) / D)
        weight = np.full(128, 2.0)
        if p == 0:
            m = np.block([[ea.real, z], [z, eb.real], [ea.imag, z], [z, eb.imag]])
            m[64, :64] = (-1.0) ** d
            weight[0] = weight[64] = 1.0
        else:
            m = np.block([[ea.real, SN1 * ea.imag], [eb.real, -SN1 * eb.imag],
                          [ea.imag, -SN1 * ea.real], [eb.imag, SN1 * eb.real]])
        fwd.append(m[out_rows])
        inv.append(((m * weight[:, None]).T / (S * D))[out_rows][:, in_rows])
    b = np.concatenate(fwd + inv, axis=1).astype(ml_dtypes.bfloat16).view(np.uint16).astype(np.uint32)
    return b[0::2] | (b[1::2] << 16)


_CHANNEL_MATRICES = _channel_matrices()


def L(t, n=1):
    return slice(128 * t, 128 * (t + n))


def add(a, b):
    return b if a is None else a if b is None else lax.add(a, b)


def sub(a, b):
    return lax.sub(a, b)


def mul(a, b):
    if isinstance(b, float):
        return lax.mul(a, lax.full(a.shape, b, f32))
    return lax.mul(a, b)


def tree(xs):
    return xs[0] if len(xs) == 1 else add(tree(xs[:len(xs) // 2]), tree(xs[len(xs) // 2:]))


def cast(a, dt):
    return lax.convert_element_type(a, dt)


def cat(*xs):
    return lax.concatenate(xs, 0)


def rows(x, lo, n):
    return lax.slice_in_dim(x, lo, lo + n, axis=0)


def bcast(x, n):
    return lax.broadcast_in_dim(x, (n, 128), (0, 1))


def iota(axis):
    return lax.broadcasted_iota(jnp.int32, (8, 128), axis)


def cmul(u, v):
    return sub(mul(u[0], v[0]), mul(u[1], v[1])), add(mul(u[0], v[1]), mul(u[1], v[0]))


def unit(turns):
    angle = turns * float(-2 * np.pi)
    return jnp.cos(angle), jnp.sin(angle)


def _radix5(x0, x1, x2, x3, x4):
    s1, d1, s2, d2 = add(x1, x4), sub(x1, x4), add(x2, x3), sub(x2, x3)
    t = add(s1, s2)
    m = sub(x0, mul(t, 0.25))
    q = mul(sub(s1, s2), C5)
    return add(x0, t), add(m, q), add(d1, mul(d2, R5)), sub(m, q), sub(mul(d1, R5), d2)


def _radix5_t(t0, a1, b1, a2, b2):
    m = add(a1, a2)
    q = mul(sub(a1, a2), C5)
    t = sub(t0, mul(m, 0.25))
    s1, s2 = add(t, q), sub(t, q)
    d1, d2 = add(b1, mul(b2, R5)), sub(mul(b1, R5), b2)
    return add(t0, m), add(s1, d1), add(s2, d2), sub(s2, d2), sub(s1, d1)


def _half4(u, v):
    return add(u[0], v[0]), add(u[1], v[1]), sub(u[0], v[0]), sub(u[1], v[1])


def _finish4(e, o, sign):
    pr, pi, mr, mi = e
    sr, si, tr, ti = o
    o0, o2 = (add(pr, sr), add(pi, si)), (sub(pr, sr), sub(pi, si))
    oa, ob = (add(mr, ti), sub(mi, tr)), (sub(mr, ti), add(mi, tr))
    return (o0, oa, o2, ob) if sign < 0 else (o0, ob, o2, oa)


def _radix4(v, sign):
    return _finish4(_half4(v[0], v[2]), _half4(v[1], v[3]), sign)


def _twiddle(v, e):
    r, i = v
    e %= 16
    if e == 0:
        return r, i
    if e == 4:
        return lax.neg(i), r
    if e == 12:
        return i, lax.neg(r)
    c, s = float(np.cos(np.pi * e / 8)), float(np.sin(np.pi * e / 8))
    if e % 4 == 2:
        if c * s > 0:
            return mul(sub(r, i), c), mul(add(r, i), c)
        return mul(add(r, i), c), mul(sub(i, r), c)
    return sub(mul(r, c), mul(i, s)), add(mul(r, s), mul(i, c))


def _lhs7(i, a):
    if i == 0: return add(a(0, 0), a(1, 1))
    if i == 1: return add(a(1, 0), a(1, 1))
    if i == 2: return a(0, 0)
    if i == 3: return a(1, 1)
    if i == 4: return add(a(0, 0), a(0, 1))
    if i == 5: return sub(a(1, 0), a(0, 0))
    return sub(a(0, 1), a(1, 1))


def _rhs7(i, b):
    if i == 0: return add(b(0, 0), b(1, 1))
    if i == 1: return b(0, 0)
    if i == 2: return sub(b(0, 1), b(1, 1))
    if i == 3: return sub(b(1, 0), b(0, 0))
    if i == 4: return b(1, 1)
    if i == 5: return add(b(0, 0), b(0, 1))
    return add(b(1, 0), b(1, 1))


def _fold7(j, m, get, put, done):
    if j < 3:
        put(j, m)
    elif j == 3:
        done(1, 0, add(get(1), m))
        put(3, add(get(0), m))
    elif j == 4:
        done(0, 1, add(get(2), m))
        put(4, sub(get(3), m))
    elif j == 5:
        done(1, 1, add(add(sub(get(0, 2), get(1, 2)), get(2, 2)), m))
    else:
        done(0, 0, add(get(4), m))


LHS1 = ((2, 5), (3, 6), (0, 1, 4))
LHS2 = ((2, 3, 0), (1, 5), (4, 6))
RHS = ((1, 4, 0), (2, 5), (3, 6))
_FIRST = [7 * i + j for group in LHS1 for i in group for j in range(7)]
EARLY = ([(0, 1, ij) for ij in _FIRST[:24]], [(0, 1, ij) for ij in _FIRST[24:40]],
         [(0, 2, ij) for ij in _FIRST[40:48]], [(1, 3, ij) for ij in _FIRST[:12]])
DONE = {ij: hi for part in EARLY for _, hi, ij in part}


def quarters(j):
    cuts = sorted({128 * j, 128 * j + 128} | {c for c in (160, 320, 480) if 128 * j < c < 128 * j + 128})
    return [(lo // 160, lo % 160, hi - lo) for lo, hi in zip(cuts, cuts[1:])]


def _nt(a, b):
    return lax.dot_general(a, b, (((1,), (1,)), ((), ())), preferred_element_type=f32)


def _nn(a, b):
    return lax.dot_general(a, b, (((1,), (0,)), ((), ())), preferred_element_type=f32)


def _merge(*streams):
    order = []
    for si, st in enumerate(streams):
        st, t0, t1 = st if isinstance(st, tuple) else (st, 0.0, 1.0)
        tot, acc = float(sum(t[0] for t in st)) or 1.0, 0.0
        for t in st:
            order.append((t0 + (t1 - t0) * (acc + (0.5 * t[0] if si else 0.0)) / tot, si, len(order), t))
            acc += t[0]
    for _, _, _, t in sorted(order, key=lambda o: o[:3]):
        t[1](*t[2:])


class Bank:
    def __init__(self, refs, offsets, cols, nrows, packed=0, chained=0):
        self.refs, self.offsets, self.nrows, self.packed, self.chained = refs, offsets, nrows, packed, chained
        self.cache, self.count, self.held = {}, 0, None

    @staticmethod
    def shapes(count, cols, nrows, packed=0, chained=0):
        n = ((cols + packed) >> packed) * (nrows >> packed) + 8
        return [pltpu.VMEM(((n + 31) // 32 * 32, 128 << packed), u32 if packed else f32) for _ in range(count)]

    def view(self, k, via):
        if (k, via) not in self.cache:
            r = self.refs[k]
            self.cache[k, via] = r.at[pl.ds(self.offsets[via], r.shape[0])] if via else r
        return self.cache[k, via]

    def get(self, k, col, lo=0, n=None, via=1):
        lo += (col >> self.packed) * self.nrows
        x = self.view(k, via)[lo >> self.packed:(lo + (n or self.nrows)) >> self.packed, L(col & self.packed)]
        return pltpu.bitcast(x, bf16) if self.packed else x

    def wide(self, k, cols, via=1):
        return lax.concatenate([self.get(k, c, via=via) for c in cols], 1)

    def halves(self, k, c, via=1):
        return cat(self.get(k, 2 * c, via=via), self.get(k, 2 * c + 1, via=via))

    def put(self, k, col, lo, x):
        if self.packed and col % 2 == 0:
            self.held = x
            return
        if self.packed:
            x = pltpu.bitcast(cast(lax.concatenate([self.held, x], 1), bf16), u32)
        at = ((col >> self.packed) * self.nrows + lo) >> self.packed
        self.count += 1
        self.view(k, (0, 6 + self.count % 2, 6)[self.chained])[at:at + x.shape[0], :] = x

    def clear_tokens(self):
        for r in self.refs:
            r[r.shape[0] - 8:r.shape[0], L(0)] = jnp.zeros((8, 128), r.dtype)

    def token(self, k):
        n = self.refs[k].shape[0]
        return (id(self), k), self.refs[k][n - 8:n, L(0)]


class Table(Bank):
    def __init__(self, refs, offsets, nrows, groups, chained):
        super().__init__(refs, offsets, None, nrows, 1, chained)
        self.slot = {i: (g, 7 * k) for g, group in enumerate(groups) for k, i in enumerate(group)}

    @staticmethod
    def shapes(tiles, nrows, groups, chained):
        return [s for _ in range(tiles) for g in groups for s in Bank.shapes(1, 7 * len(g), nrows, 1)]

    def load(self, k, i, j, via, lo=0, n=None):
        g, s = self.slot[i]
        return self.get(3 * k + g, s + j, lo, n, via)

    def store(self, k, i, j, lo, val):
        g, s = self.slot[i]
        self.put(3 * k + g, s + j, lo, val)

    def tiles(self, ij, ks, via, axis=1):
        return lax.concatenate([self.load(k, ij // 7, ij % 7, via) for k in ks], axis)


BANKS = dict(
    x0=(Bank, 4, 4, D),
    x1=(Bank, 4, 4, 2 * BINS),
    vb=(Bank, 16, 4, 168),
    mr2=(Bank, 12, 2, 2 * BINS),
    wt=(Bank, 4, 4, F - MAIN, 1, 2), br=(Bank, 4, 12, 64, 1, 1), tb=(Bank, 4, 40, 64, 1, 1),
    a1=(Table, 4, 160, LHS1, 2), hp=(Bank, 4, 12, 160, 1, 2), bt=(Bank, 1, 1, 256),
    a2=(Table, 3, 160, LHS2, 1), ar=(Bank, 1, 18, 128, 1, 2),
    b1=(Table, 12, 128, RHS, 1), b2=(Table, 12, 128, RHS, 1),
    lo=(Bank, 10, 1, 160), hi=(Bank, 10, 4, 160), zb=(Bank, 4, 12, BINS, 1, 1),
    post=(Bank, 1, 1, 240, 1, 2), sm=(Bank, 1, 48, 128, 1), mean=(Bank, 4, 4, 40, 0, 2), sums=(Bank, 4, 4, 64))

BIAS1, BIAS2, MEAN, SCALE, SHIFT = 0, 16, 32, 48, 64


def _kernel(x_hbm, wr_hbm, wi_hbm, w1_hbm, b1_hbm, w2_hbm, b2_hbm, dm_hbm, o_hbm,
            b1_ref, b2_ref, wrb, wib, w1b, w2b, dm_ref, wp, wt, small, sems, kept):
    zero = iota(1)[0, 0]
    zs = [None] + [pl.multiple_of(zero << (4 + k), 16) for k in range(7)]
    m = {name: spec[0](kept[name], zs, *spec[2:]) for name, spec in BANKS.items()}
    pool, a1, a2 = kept["mr2"], kept["a1"], kept["a2"]
    m.update(va=Bank(kept["x1"], zs, 8, BINS), k1=Bank(pool[:8], zs, 4, BINS), hb=Bank(pool[8:12], zs, 4, BINS),
             part=Bank(pool[:6] + pool[8:9], zs, 8, 160),
             mr1=Bank(pool[6:8], zs, 5, F - MAIN), d0=Bank(pool[9:], zs, 4, 128),
             yb=Bank(a1[2::3] + a1[0::3], zs, 6, BINS, 1))

    def dm(p):
        return pltpu.bitcast(dm_ref[:, L(p)], bf16)

    wpr = [r.at[pl.ds(zs[1], 2)] for r in wp]
    w_rd = [[r.at[pl.ds(zs[1 + g], F)] for g in range(3)] for r in (w1b, w2b)]
    tokens, ready, backlog, plain = [], set(), [], {}

    def row(i, n):
        return bcast(small[i:i + 1, :], n)

    def paced(a):
        if not tokens:
            return a
        n, gates = a.shape[0] // 16, {}
        for i, (key, tok) in enumerate(tokens):
            gates.setdefault(max((i + 1) * n // len(tokens) - 1, 0), {})[key] = tok
        tokens.clear()
        parts, lo = [], 0
        for r in sorted(gates):
            if r > lo:
                parts.append(lax.slice(a, (16 * lo, 0), (16 * r, 128)))
            w = pltpu.bitcast(lax.slice(a, (16 * r, 0), (16 * r + 16, 128)), u32)
            for tok in gates[r].values():
                w = lax.bitwise_or(w, lax.bitcast_convert_type(tok, u32))
            parts.append(pltpu.bitcast(w, bf16))
            lo = r + 1
        if lo < n:
            parts.append(lax.slice(a, (16 * lo, 0), (16 * n, 128)))
        left = cat(*parts)
        return left if a.shape[1] == 128 else lax.concatenate([left, lax.slice(a, (0, 128), a.shape)], 1)

    def copy(src, dst, group):
        return pltpu.make_async_copy(src, dst, sems.at[group])

    order = [a + 4 * b for a in range(4) for b in range(4)]
    x_cp = {t: copy(x_hbm.at[L(t), :], w2b.at[L(t // 3), L(5 * (t % 3), 5)], (0, 1, 2, 2, 3, 3, 4, 4)[k // 2])
            for k, t in enumerate(order)}
    o_cp = {t: [copy(w1b.at[L(t // 3), L(5 * (t % 3) + j, n)], o_hbm.at[L(t), L(j, n)], 5)
                for j, n in (((0, 3), (3, 2)) if t % 4 == 3 else ((0, 5),))] for t in order}
    nudges = []

    def launch(*copies):
        k = len(nudges)
        nudges.append(copy(dm_hbm.at[0:8, L(0)], m["post"].view(0, 5).at[8 * k:8 * k + 8, L(0)], 5))
        for c in copies + (nudges[-1],):
            c.start()
        tokens.append(m["post"].token(0))

    w_cp = {(k, n): copy(src.at[lo:hi, :], dst.at[lo:hi, :], 3 if k or n == 3 else 4)
            for k, (src, dst) in enumerate(((w1_hbm, w1b), (w2_hbm, w2b)))
            for n, (lo, hi) in enumerate(((0, 512), (512, 1024), (1024, MAIN), (MAIN, F))) if k or n}
    w_cp[0, 0] = [copy(w1_hbm.at[0:512, L(t)], w1b.at[0:512, L(t)], 0 if k < 8 else 3) for k, t in enumerate(order)]

    def get_v(name, a, q, lo, n):
        return tuple(m[name].get(*((a, 4 * e + q) if name == "va" else (2 * a + e, q)), lo, n) for e in range(2))

    def put_v(name, a, q, lo, val):
        for e in range(2):
            m[name].put(*((a, 4 * e + q) if name == "va" else (2 * a + e, q)), lo, val[e])

    def gather(acc, t, *xs):
        acc[t, 0] = add(acc.get((t, 0)), tree(xs))
        acc[t, 1] = add(acc.get((t, 1)), tree([mul(x, x) for x in xs]))

    def moments(acc, t):
        mean = jnp.sum(acc[t, 0], axis=0, keepdims=True) * (1.0 / D)
        return mean, jnp.maximum(jnp.sum(acc[t, 1], axis=0, keepdims=True) * (1.0 / D) - mean * mean, 0.0)

    def norm_once(acc, t):
        mean, var = moments(acc, t)
        small[MEAN + t:MEAN + t + 1, :] = mean
        small[SCALE + t:SCALE + t + 1, :] = lax.rsqrt(var + EPS)

    def load_x(t):
        eye = (lax.broadcasted_iota(jnp.int32, (128, 128), 0) == lax.broadcasted_iota(jnp.int32, (128, 128), 1)).astype(bf16)
        xt = _nt(paced(eye), jnp.concatenate([w2b[L(t // 3), L(5 * (t % 3) + j)] for j in range(5)], axis=0))
        acc = {}
        for c in range(16):
            x = [lax.slice(xt, (8 * c, 128 * j), (8 * c + 8, 128 * j + 128)) for j in range(5)]
            for j in range(5):
                m["x0"].put(t % 4, t // 4, 128 * j + 8 * c, x[j])
            gather(acc, t, *x)
        norm_once(acc, t)

    def fwd10(t, c):
        halves = []
        m10, r = mul(row(MEAN + t, 8), 10.0), row(SCALE + t, 8)
        for h in range(2):
            x = [m["x0"].get(t % 4, t // 4, 64 * i + 16 * c + 8 * h, 8) for i in range(10)]
            e = _radix5(*[add(x[i], x[i + 5]) for i in range(5)])
            o = _radix5(*[sub(x[i], x[i + 5]) if i % 2 == 0 else sub(x[i + 5], x[i]) for i in range(5)])
            halves.append([mul(v, r) for v in (sub(e[0], m10), o[0], e[1], e[2], e[3], e[4], o[1], o[2], o[3], o[4])])
        for i in range(10):
            m["tb"].put(t % 4, 10 * (t // 4) + i, 16 * c, cat(halves[0][i], halves[1][i]))
        tokens.append(m["tb"].token(t % 4))

    def fwd_d(a, p):
        g = _nn(paced(dm(p)), lax.concatenate([m["tb"].halves(a, 5 * b + p) for b in range(4)], 1))
        for c in range(8):
            v = [(lax.slice(g, (16 * c, 128 * b), (16 * c + 8, 128 * b + 128)),
                  lax.slice(g, (16 * c + 8, 128 * b), (16 * c + 16, 128 * b + 128))) for b in range(4)]
            if p == 0 and c == 0:
                for q, w in enumerate(_radix4([(i, jnp.zeros((8, 128), f32)) for (_, i) in v], -1)):
                    w = _twiddle(w, -q * a)
                    put_v("va", a, q, 320, (cat(w[0], w[0]), cat(w[1], w[1])))
                v = [(r, jnp.where(iota(0) == 0, 0.0, i)) for (r, i) in v]
            for q, w in enumerate(_radix4(v, -1)):
                put_v("va", a, q, 80 * (c % 4) + 16 * p + 8 * (c // 4), _twiddle(w, -q * a))

    def permute_w(get, put):
        cur = [get((-k) % 16) for k in range(16)]
        cur = [pltpu.roll(c, (-k) % 16, 1) if k else c for k, c in enumerate(cur)]
        for bit in (1, 2, 4, 8):
            msk = (iota(1) & bit) != 0
            cur = [lax.select(msk, cur[(k - bit) % 16], cur[k]) for k in range(16)]
        for k in range(16):
            put(k, cur[k])

    def prep_w(src, ri, part, c):
        if c < 20:
            def put(k, v):
                wp[part][ri, k, 8 * (c - 5 * part):8 * (c - 5 * part) + 8, :] = v
            permute_w(lambda t: pltpu.bitcast(src[16 * c:16 * c + 16, L(t)], u32), put)
        else:
            def put(k, v):
                wt[ri, k] = v
            permute_w(lambda t: bcast(cast(src[320:321, L(t)], f32), 8), put)

    def w_rows(ri, k1, c):
        if c == 20:
            v = wt[ri, k1]
            return cat(v, v)
        out = []
        for k in TILE_CLASSES[c % 5]:
            v = wpr[min(c // 5, 2)][ri, k1, pl.ds(k // 2 + 40 * (c // 15), 8, stride=5), :]
            out.append(lax.bitwise_and(v, lax.full(v.shape, 0xFFFF0000, u32)) if k % 2 else lax.shift_left(v, lax.full(v.shape, 16, u32)))
        return pltpu.bitcast(cat(*out), f32)

    def s_in(q, c):
        z = _radix4([get_v("va", a, q, 16 * c, 16) for a in range(4)], -1)
        for p in range(4):
            for j, val in enumerate((add(z[p][0], z[p][1]), z[p][0], z[p][1])):
                m["zb"].put(q, 3 * p + j, 16 * c, val)
        tokens.append(m["zb"].token(q))

    def spectral(extra):
        units = [(h, q) for h in range(2) for q in range(4)]

        def s_dot(h, q, p, j, inverse):
            lo, n = 160 * h, 160 + 16 * h
            lhs = paced(m["yb"].get(2 * q + p % 2, 3 * (p // 2) + j, lo, n) if inverse else m["zb"].get(q, 3 * p + j, lo, n))
            return (_nt if inverse else _nn)(lhs, m["sm"].get(0, 16 * j + q + 4 * p, via=1 + 2 * h + inverse))

        def s_fwd(h, q, ps):
            prod = {(p, j): s_dot(h, q, p, j, 0) for p in ps for j in (1, 2)}
            for k in range(10 + h):
                c = 10 * h + k
                for p in ps:
                    both = m["k1"].get(2 * q, p, 16 * c, 16)
                    x = sub(both, rows(prod[p, 2], 16 * k, 16)), add(both, rows(prod[p, 1], 16 * k, 16))
                    yr, yi = cmul(x, (w_rows(0, q + 4 * p, c), w_rows(1, q + 4 * p, c)))
                    for j, val in enumerate((add(yr, yi), yi, yr)):
                        m["yb"].put(2 * q + p % 2, 3 * (p // 2) + j, 16 * c, val)

        def s_inv(h, q, odd):
            ps = (odd, odd + 2)
            prod = {(p, j): s_dot(h, q, p, j, 1) for p in ps for j in (1, 2)}
            for k in range(20 + h):
                lo, z = 160 * h + 8 * k, []
                for p in ps:
                    both = m["k1"].get(2 * q + 1, p, lo, 8)
                    z.append((add(both, rows(prod[p, 1], 8 * k, 8)), sub(both, rows(prod[p, 2], 8 * k, 8))))
                half = _half4(*z)
                if not odd:
                    for j in range(4):
                        m["hb"].put(q, j, lo, half[j])
                else:
                    for a, w in enumerate(_finish4([m["hb"].get(q, j, lo, 8) for j in range(4)], half, 1)):
                        put_v("vb", 4 * h + a, q, 8 * k, _twiddle(w, q * a))

        for c in range(10):
            s_in(0, c)
        tokens.clear()
        for u in range(9):
            now, before = units[u] if u < 8 else None, units[u - 1] if u else None
            common = ([now + (0,)] if now else []) + ([before + (1,)] if before else [])
            side, more = list(extra[u][0]), extra[u][1]
            if u < 7:
                h, q = units[u + 1]
                side += [(1, s_in, q, 10 * h + k) for k in range(10 + h)]
            early = [(1, inv4, a, p, c) for a in range(4) for p in range(5) for c in range(2)][u - 5::4] if u > 4 else []
            for k, (h, q, inverse) in enumerate(common):
                _merge(side[k * len(side) // len(common):(k + 1) * len(side) // len(common)])
                for p in range(4):
                    m["k1"].put(2 * q + inverse, p, 160 * h, s_dot(h, q, p, 0, inverse))
            for odd in range(2):
                if now:
                    s_fwd(*now, (odd, odd + 2))
                if before:
                    _merge(early[odd::2], more if odd == 0 else [])
                    s_inv(*before, odd)

    def inv4(a, p, c):
        g = _radix4([get_v("vb", 4 * (c // 2) + a, q, 80 * (c % 2) + 16 * p, 16) for q in range(4)], 1)
        if (p, c) == (0, 0):
            for b in range(4):
                m["mean"].put(a, b, 0, cat(*g[b]))
            return
        for b in range(4):
            for j in range(2):
                m["tb"].put(a, 10 * b + 2 * p + j, 16 * c, g[b][j])
        tokens.append(m["tb"].token(a))

    def real_bins(a, first):
        ny = _radix4([get_v("vb", 4 + a, q, 160, 8) for q in range(4)], 1)
        for b in range(4):
            t = a + 4 * b
            g = m["mean"].get(a, b, 0, 32)
            m["tb"].put(a, 10 * b, 0, rows(g, 0, 16))
            m["tb"].put(a, 10 * b + 1, 0, cat(lax.select(iota(0) == 0, ny[b][0], rows(g, 16, 8)), rows(g, 24, 8)))
            mean = small[MEAN + t:MEAN + t + 1, :] + rows(g, 0, 1) * (1.0 / (S * D))
            carried = None if first else small[SHIFT + t:SHIFT + t + 1, :]
            small[SHIFT + t:SHIFT + t + 1, :] = add(small[BIAS2 + t:BIAS2 + t + 1, :] + mean, carried)
            m["mean"].put(a, b, 32, bcast(mean, 8))
        tokens.append(m["mean"].token(a))

    def inv_d0(a):
        for b in range(4):
            m["d0"].put(a % 2, b, 0, _nn(paced(dm(5)), m["tb"].halves(a, 5 * b)))

    def inv_d(a, b):
        t = a + 4 * b
        tt = [_nn(dm(5 + p), m["tb"].halves(a, 5 * b + p)) for p in range(1, 5)]
        mean, sq = m["mean"].get(a, b, 32, 8), None
        for c in range(8):
            v = [rows(tt[i // 2], 16 * c + 8 * (i % 2), 8) for i in range(8)]
            e = _radix5_t(sub(m["d0"].get(a % 2, b, 16 * c, 8), mean), *v[0:4])
            o = _radix5_t(m["d0"].get(a % 2, b, 16 * c + 8, 8), *v[4:8])
            part = []
            for i in range(5):
                for j, sg in ((i, i % 2), (i + 5, 1 - i % 2)):
                    x = add(m["x0"].get(a, b, 64 * j + 8 * c, 8, 2), (sub if sg else add)(e[i], o[i]))
                    m["x1"].put(a, b, 64 * j + 8 * c, x)
                    part.append(mul(x, x))
            sq = add(sq, tree(part))
        var = jnp.sum(sq, axis=0, keepdims=True) * (1.0 / D)
        r = lax.rsqrt(var + EPS)
        small[SCALE + t:SCALE + t + 1, :] = r * lax.rsqrt(var * r * r + EPS) * 0.5

    def split2(load, pick, put, group, gate=None):
        seen = {}

        def blk(i, j):
            if (i, j) not in seen:
                seen[i, j] = load(i, j)
            return seen[i, j]
        for i in group:
            h = {(r, k): pick(i, lambda r1, k1: blk(2 * r1 + r, 2 * k1 + k)) for r in range(2) for k in range(2)}
            for j in range(7):
                put(i, j, pick(j, lambda r, k: h[r, k]))
            if i == group[-1] and len(group) % 2:
                put(i, 7, pick(6, lambda r, k: h[r, k]))
            if gate:
                tokens.append(gate())

    def lhs1(a, v, g):
        def load(r, k):
            t = a + 4 * k
            h = mul(m["x1"].get(a, k, 160 * r + 16 * v, 16, 3 + g), row(SCALE + t, 16))
            if r != k and g == k // 2:
                m["hp"].put(a, plain.setdefault((r, k), len(plain)), 16 * v, h)
            return h

        def put(i, j, val):
            m["a1"].store(a, i, j, 16 * v, val)
        split2(load, _lhs7, put, LHS1[g])
        tokens.append(m["hp"].token(a))
        tokens.append(m["a1"].token(3 * a + g))

    def weights(which, g, lo, t):
        return cast(w_rd[which][g][lo:lo + 16, L(t)], f32)

    def rhs_main(which, n, a, v, g):
        def raw(f, s):
            lo = 128 * (4 * n + f) + 16 * v
            return weights(which, g, lo, a + 4 * s)
        tab = m[("b1", "b2")[which]]
        split2(raw if which else lambda s, f: raw(f, s), _rhs7,
               lambda i, j, val: tab.store(4 * n + a, i, j, 16 * v, val), RHS[g], lambda: tab.token(3 * (4 * n + a) + g))

    def rhs_rest(a, pair, v):
        (p1, p2, p3), (q1, q2, q3) = ([weights(1, 0, MAIN + 64 * k + 16 * v, a + 8 * pair + 4 * e) for k in range(3)] for e in range(2))
        for k, val in enumerate((sub(p1, q1), p2, q2, sub(q3, p3), q1, p3)):
            m["br"].put(a, 6 * pair + k, 16 * v, val)
        tokens.append(m["br"].token(a))

    def rhs_main_tasks(which, ns, as_, gs=range(3)):
        return [(36 * len(RHS[g]), rhs_main, which, n, a, v, g) for g in gs for n in ns for a in as_ for v in range(8)]

    def rhs_rest_tasks():
        return [(22, rhs_rest, a, pair, v) for a in range(4) for pair in range(2) for v in range(4)]

    def gelu_half(u):
        inner = mul(u, add(mul(mul(u, u), 8 * GELU * 0.044715), lax.full(u.shape, 2 * GELU, f32)))
        return add(u, mul(u, lax.tanh(inner)))

    def fold49(ij, flip, prod, done):
        i, j = divmod(ij, 7)
        for v in range(20):
            def slot(bank, par, col):
                return (lambda k, via=1: bank.get(5 * par + k, col, 8 * v, 8, via),
                        lambda k, val: bank.put(5 * par + k, col, 8 * v, val))

            def inner(r, n, h):
                _fold7(i, h, *slot(m["hi"], flip, 2 * r + n), lambda r1, n1, c: done(2 * r1 + r, 2 * n1 + n, v, c))
            _fold7(j, rows(prod, 8 * v, 8), *slot(m["lo"], i % 2, 0), inner)

    def stage_w1(a, k):
        for e in (2 * k, 2 * k + 1):
            m["wt"].put(a, e, 0, cast(w1b[MAIN:F, L(a + 4 * e)], f32))
        tokens.append(m["wt"].token(a))

    def mm1_rest(a, j):
        def h(k):
            return cat(*[m["hp"].get(a, plain[r, k], lo, n) if r != k else m["a1"].load(a, 2 + k // 2, 2 + k % 2, 4, lo, n)
                         for r, lo, n in quarters(j)])
        w = m["wt"].wide(a, range(4), via=1 + j)
        prod = _nt(paced(w), lax.concatenate([h(k) for k in range(4)], 1))
        for lo in range(0, F - MAIN, 8):
            u = add(rows(prod, lo, 8), m["mr1"].get(1 - a % 2, j, lo, 8) if a else m["bt"].get(0, 0, lo, 8, 1 + j))
            m["mr1"].put(a % 2, j, lo, gelu_half(u) if a == 3 else u)

    def mm1_early(lo, hi, ij):
        prod = _nt(paced(m["a1"].tiles(ij, range(lo, hi), 5)), m["b1"].tiles(ij, range(lo, hi), 2))
        m["part"].put(ij // 8, ij % 8, 0, add(prod, m["part"].get(ij // 8, ij % 8, via=2) if lo else None))

    def mm1_main(n, ij):
        def done(r, f, v, u):
            m["vb"].put(4 * (n % 2) + r, f, 8 * v, gelu_half(add(u, row(BIAS1 + 4 * n + f, 8))))
        k = DONE.get(ij, 0) if n == 0 else 0
        prod = _nt(paced(m["a1"].tiles(ij, range(k, 4), 1 + n)), m["b1"].tiles(ij, range(4 * n + k, 4 * n + 4), 1))
        if k:
            prod = add(prod, m["part"].get(ij // 8, ij % 8, 0, 160))
        fold49(ij, n % 2, prod, done)

    def lhs_rest(j, k):
        for e in range(2):
            g = cat(*[m["mr1"].get(1, 2 * j + e, 64 * u, 64, 1 + k) if 2 * j + e < 5 else jnp.zeros((64, 128), f32)
                      for u in ((0, 1), (1, 2), (0, 2))[k]])
            m["ar"].put(0, 6 * k + 2 * j + e, 0, g.T)
        tokens.append(m["ar"].token(0))

    def lhs2(n, v, g):
        split2(lambda r, f: m["vb"].get(4 * (n % 2) + r, f, 16 * v, 16, 1 + g), _lhs7,
               lambda i, j, val: m["a2"].store(n, i, j, 16 * v, val), LHS2[g], lambda: m["a2"].token(3 * n + g))

    def lhs2_tasks(n):
        return [(23 * len(LHS2[g]), lhs2, n, v, g) for v in range(10) for g in range(3)]

    def mm2_rest(a, k, r):
        lhs = paced(cat(*[m["ar"].get(0, 6 * k + j, lo - 128 * j, n, 1 + a) for j in range(5)
                          for q, lo, n in ((q, 160 * q + at, n) for q, at, n in quarters(j)) if q == r]))
        prod = _nn(lhs, lax.concatenate([m["br"].halves(a, 3 * e + k, 1 + r) for e in range(2)], 1))
        for e in range(2):
            m["mr2"].put(3 * a + k, e, 160 * r, lax.slice_in_dim(prod, 128 * e, 128 * e + 128, axis=1))

    def write_out(t, j):
        x = m["x0"].get(t % 4, t // 4, 128 * j, 128, 3) if t % 4 < 3 else cat(
            *[m["vb"].get(4 * r + t // 4, 0, lo, n, 4) for r, lo, n in quarters(j)])
        out = x.T
        w1b[L(t // 3), L(5 * (t % 3) + j)] = cast(out, bf16)
        m["mean"].put(0, 0, 0, rows(out, 120, 8))
        tokens.append(m["mean"].token(0))

    def mm2_main(a, ij, first):
        acc = {}
        def done(r, b, v, y):
            rest = [m["mr2"].get(3 * a + k, b // 2, 160 * r + 8 * v, 8, 1 + b % 2) for k in (b % 2, 2)]
            shift = None if first else row(SHIFT + a + 4 * b, 8)
            x = add(add(m["x1"].get(a, b, 160 * r + 8 * v, 8), shift), add(y, add(*rest)))
            if first or a < 3:
                m["x0"].put(a, b, 160 * r + 8 * v, x)
            else:
                m["vb"].put(4 * r + b, 0, 8 * v, x)
            if first:
                gather(acc, 0, x)
                if v == 19:
                    m["sums"].put(a, b, 16 * r, cat(acc[0, 0], acc[0, 1]))

        prod = _nn(paced(m["a2"].tiles(ij, range(3), 1 + a)), m["b2"].tiles(ij, range(a, 12, 4), 1, 0))
        fresh = set()
        fold49(ij, (a + 1) % 2, prod, lambda r, b, v, y: (done(r, b, v, y), fresh.add((r, b))))
        if a == 3 and not first:
            for r, b in sorted(fresh):
                t = a + 4 * b
                ready.add((r, t))
                for j in range(5):
                    need = {(128 * j // 160, t), ((128 * j + 127) // 160, t)}
                    if (r, t) in need and need <= ready:
                        backlog.append((ij, write_out, t, j))
                for part, need in enumerate(({(0, t), (1, t), (2, t)}, {(2, t), (3, t)})):
                    if (r, t) in need and need <= ready:
                        backlog.append((ij, launch, o_cp[t][part]))
            for _ in range(2 if ij < 48 else 99):
                if backlog and (backlog[0][0] + 4 <= ij or ij == 48):
                    _, fn, *args = backlog.pop(0)
                    args[0].start() if fn is launch and ij == 48 else fn(*args)

    def norm_sums(a, b):
        tot = None
        for r in range(4):
            tot = add(tot, m["sums"].get(a, b, 16 * r, 16))
        norm_once({(a + 4 * b, j): rows(tot, 8 * j, 8) for j in range(2)}, a + 4 * b)

    def after_mm2(a, first):
        if not first:
            return ([(30, write_out, a + 4 * b, j) for b in range(4) for j in range(5)] +
                    [(30, launch, *[o_cp[a + 4 * b][0] for b in range(4)])]) if a < 3 else []
        return ([(20, norm_sums, a, b) for b in range(4)] +
                [(115, fwd10, a + 4 * b, c) for b in range(4) for c in range(4)])

    def post_stage(first):
        def inv4_tasks(a):
            return [(20, real_bins, a, first)] + [(40, inv4, a, p, c) for p in range(5) for c in (2, 3)]
        sums = [rhs_main_tasks(0, [0], [a]) if first else [] for a in range(4)]
        plan = [[(hi - lo, mm1_early, lo, hi, ij) for lo, hi, ij in part] for part in EARLY]
        for a in range(4):
            _merge(inv4_tasks(a)[:3])
            inv_d0(a)
            _merge(inv4_tasks(a)[3:])
            tokens.clear()
            side = [[(30 * len(LHS1[g]), lhs1, a, v, g) for v in range(10)] for g in range(3)]
            for b in range(4):
                inv_d(a, b)
                if a == 0 and b == 2:
                    _merge(side.pop(0))
                    tokens.clear()
                if a or b >= 2:
                    n = 4 // plan[a][0][0]
                    _merge(plan[a][:n])
                    del plan[a][:n]
            if first:
                side.append([(40, stage_w1, a, k) for k in range(2)] + (sums[2] if a == 1 else []))
            if a == 0:
                n = 14 - (24 - len(plan[0]))
                _merge(plan[0][:n], (side.pop(0), -0.2, 0.5))
                tokens.clear()
                del plan[0][:n]
            _merge([(4.8, mm1_rest, a - 1, j) for j in range(5 if a else 0)] + plan[a],
                   ([t for part in side for t in part], 0.0, 0.8))
        if first:
            for k in (3, 0, 1, 2):
                w_cp[1, k].start()
            w_cp[0, 1].wait()
            w_cp[0, 2].wait()
        _merge([(1, mm1_rest, 3, j) for j in range(5)], (sums[3][:8], -0.2, 0.8))

    cut = (48, 84, 156, 204, 240, 288)

    def w2_sums():
        return [t for a in range(4) for g in range(3) for t in rhs_main_tasks(1, range(3), [a], (g,))]

    def mm1_stage(first):
        for n in range(3):
            late, sums = [], []
            if first:
                late = rhs_main_tasks(0, [n], range(4) if n else [3], (1, 2))
                sums = rhs_main_tasks(0, [n + 1], range(4), (0,)) if n < 2 else [(0, w_cp[1, k].wait) for k in range(4)] + rhs_rest_tasks() + w2_sums()[:cut[0]]
            _merge([(1, mm1_main, n, ij) for ij in range(49)],
                   (lhs2_tasks(n - 1) if n else [], 0.45, 0.97),
                   ([(1, lhs_rest, j, k) for j in range(3) for k in range(3)] if n == 0 else [], 0.4, 0.95),
                   (late, 0.0, 0.39), (sums, 0.4 if n else 0.0, 0.95))

    def mm2_stage(first):
        sums = w2_sums() if first else []
        _merge([(1, mm2_rest, a, k, r) for a in range(4) for k in range(3) for r in range(4)], (lhs2_tasks(2), 0.0, 0.9), (sums[cut[0]:cut[1]], 0.0, 0.9))
        for a in range(4):
            _merge([(1, mm2_main, a, ij, first) for ij in range(49)],
                   (after_mm2(a - 1, first) if a else [], 0.1 if a < 3 or not first else 0.4, 0.95 if first else 0.45),
                   (sums[cut[a + 1]:cut[a + 2]], 0.0, 0.95 if a < 3 else 0.39))
        _merge([(1, fwd_d, a, p) for a in range(3) for p in range(5)] if first else [], (after_mm2(3, first), 0.0, 0.9))
        tokens.clear()
        if first:
            for p in range(5):
                fwd_d(3, p)
        else:
            for c in nudges + [c for t in order for c in o_cp[t]]:
                c.wait()

    def token_mixing(first):
        tokens.clear()
        post_stage(first)
        mm1_stage(first)
        mm2_stage(first)

    def first_transform():
        cuts = (0, 80, 160, 321)
        dm_cp = copy(dm_hbm.at[:, L(0, 5)], dm_ref.at[:, L(0, 5)], 2)
        small_cp = [copy(dm_hbm.at[:, L(5, 5)], dm_ref.at[:, L(5, 5)], 0), copy(b1_hbm, b1_ref, 0),
                    copy(b2_hbm, b2_ref.at[0:16, :], 0)]
        f_cp = [[copy(src.at[lo:hi, :], dst.at[lo:hi, :], k) for src, dst in ((wr_hbm, wrb), (wi_hbm, wib))]
                for k, (lo, hi) in enumerate(zip(cuts, cuts[1:]))]

        def prep(k):
            return [(1, prep_w, src, ri, k, c) for c in range(cuts[k] // 16, (cuts[k + 1] + 15) // 16)
                    for ri, src in enumerate((wrb, wib))]

        def fly(tiles):
            return [(1, fwd10, t, c) for t in tiles for c in range(4)]

        def start():
            for name in BANKS:
                if m[name].chained:
                    m[name].clear_tokens()
            launch(*[x_cp[t] for t in order[:6]])
            gate = lax.bitcast_convert_type(tokens.pop()[1], jnp.int32)
            s2, lane = (lax.broadcasted_iota(jnp.int32, (16, 128), k) for k in range(2))
            s2, lane = s2 + cat(gate, gate), lane + cat(gate, gate)
            k2 = ((lane & 15) << 3) + (lane >> 4)
            base, hop = (unit(cast(k & 127, f32) * (1.0 / 128)) for k in (s2 * k2, 16 * k2))
            step = unit(cast(s2, f32) * (1.0 / S))
            for c in range(8):
                if c:
                    base, step = cmul(base, hop), cmul(step, (float(np.cos(np.pi / 64)), float(-np.sin(np.pi / 64))))
                re, im = base
                for k1 in range(0, 16, 2):
                    nxt = cmul((re, im), step)
                    two = [[pltpu.roll(x, k, 1) if k else x for x in z] for k, z in enumerate(((re, im), nxt), k1)]
                    for j in range(3):
                        for k, (x, y) in enumerate(two, k1):
                            m["sm"].put(0, 16 * j + k, 16 * c, (x, sub(y, x), add(x, y))[j])
                    re, im = cmul(nxt, step)
            queue = [[x_cp[t] for t in order[k:k + 2]] + [dm_cp] * (k == 6) for k in range(6, 16, 2)] + f_cp[:2] + [[]]
            for before, lo, hi in ((0, 0, 2), (0, 2, 4), (2, 4, 8), (4, 8, 12), (8, 12, 16)):
                for c in queue.pop(0):
                    c.start()
                for c in [x_cp[t] for t in order[lo:hi]] + [dm_cp] * (lo == 4):
                    c.wait()
                _merge([(1, load_x, t) for t in order[lo:hi]] + [(0.8, fwd_d, lo // 4 - 1, p) for p in range(5 * (lo > 3))],
                       (fly(order[before:lo]), -0.2, 0.6 if lo == 2 else 0.3),
                       (fly(order[12:] if hi == 16 else []), 0.5, 0.88),
                       ([(1, launch, *queue.pop(0))] if lo > 3 else [], 0.2, 0.3))
                tokens.clear()
            for c in f_cp[2]:
                c.start()
            for c in f_cp[0]:
                c.wait()
            _merge([(1, fwd_d, 3, p) for p in range(5)], prep(0))

        def prep_bias():
            half = jnp.concatenate([b1_ref[...].astype(f32).reshape(1, F), jnp.zeros((1, 64), f32)], axis=1) * 0.5
            for n in range(14):
                if n < 12:
                    small[BIAS1 + n:BIAS1 + n + 1, :] = half[:, L(n)]
                else:
                    m["bt"].put(0, 0, 128 * (n - 12), bcast(half[:, L(n)], 128).T)
            small[BIAS2:BIAS2 + 16, :] = b2_ref[0:16, :].astype(f32)

        def rest():
            for c in small_cp + w_cp[0, 0][:4]:
                c.start()
            for c in f_cp[1]:
                c.wait()
            _merge(prep(1))
            sums = rhs_main_tasks(0, [0], [0, 1])
            cut = (0, 4, 10, 28, 34, 44, 48)
            sums = [sums[lo:hi] for lo, hi in zip(cut, cut[1:])]
            none = [], []
            spectral([none, none, none,
                      ([(0, c.start) for c in w_cp[0, 0][4:8] + [w_cp[0, 3]]] + [(0, c.wait) for c in f_cp[2]] + prep(2), []),
                      none, none,
                      ([(0, c.start) for c in w_cp[0, 0][8:]] + [(0, c.wait) for c in small_cp + w_cp[0, 0][:8]] +
                       [(0, prep_bias)] + sums[0], sums[1]), sums[2:4], sums[4:6]])
            w_cp[0, 1].start()
            w_cp[0, 2].start()
            for c in [w_cp[0, 3]] + w_cp[0, 0][8:]:
                c.wait()
        start()
        rest()

    first_transform()
    token_mixing(True)
    spectral([([], [])] * 9)
    token_mixing(False)


@jax.jit
def pallas_interleave_layers__spectral_gfnet__mixer_token_mlp__prompt_kernel(A_x, A_w_r, A_w_i, B_x, B_w1, B_b1, B_w2, B_b2):
    hbm = pl.BlockSpec(memory_space=pl.ANY)
    V = pltpu.VMEM
    out = pl.pallas_call(
        _kernel,
        in_specs=[hbm, hbm, hbm, hbm, hbm, hbm, hbm, hbm],
        out_specs=hbm,
        out_shape=jax.ShapeDtypeStruct((S, D), bf16),
        scratch_shapes=[
            V((F,), bf16), V((64, 128), bf16), V((321, S), bf16), V((321, S), bf16), V((F, S), bf16), V((F, S), bf16), V((64, 1280), u32),
            [V((2, 16, n, 128), u32) for n in (40, 40, 80)], V((2, 16, 8, 128), f32), V((96, 128), f32),
            pltpu.SemaphoreType.DMA((6,)),
            {name: spec[0].shapes(*spec[1:]) for name, spec in BANKS.items()},
        ],
        compiler_params=pltpu.CompilerParams(vmem_limit_bytes=127 * 1024 * 1024, internal_scratch_in_bytes=11 * 4096),
    )(A_x.reshape(S, D), A_w_r.T, A_w_i.T, B_w1.T, B_b1, B_w2,
      B_b2.reshape(16, 128), _CHANNEL_MATRICES)
    return out.reshape(1, S, D)
```

```python
import jax
import jax.experimental.pallas as pl
import jax.experimental.pallas.tpu as pltpu
import jax.numpy as jnp
import ml_dtypes
import numpy as np
from jax import lax

S, D, F = 2048, 640, 1728
MAIN = 1536
EPS = 1e-5
BINS = 336
f32, bf16, u32 = jnp.float32, jnp.bfloat16, jnp.uint32

TILE_CLASSES = ((0, 5), (2, 8), (4, 6), (7, 3), (9, 1))
SN1, SN2 = np.sin(2 * np.pi / 5), np.sin(4 * np.pi / 5)
C5 = float(np.sqrt(5) / 4)
R5 = float(SN2 / SN1)
GELU = float(np.sqrt(2 / np.pi))


def _channel_matrices():
    d, j, i = np.arange(64), np.arange(32), np.arange(128)
    out_rows = (i // 8 % 2) * 64 + (i // 16) * 8 + i % 8
    in_rows = (i // 64) * 64 + (i // 8 % 2) * 32 + (i // 16 % 4) * 8 + i % 8
    fwd, inv = [], []
    z = np.zeros((32, 64))
    for p, (ka, kb) in enumerate(TILE_CLASSES):
        ea = np.exp(-2j * np.pi * np.outer(ka + 10 * j, d) / D)
        eb = np.exp(-2j * np.pi * np.outer(kb + 10 * j, d) / D)
        weight = np.full(128, 2.0)
        if p == 0:
            m = np.block([[ea.real, z], [z, eb.real], [ea.imag, z], [z, eb.imag]])
            m[64, :64] = (-1.0) ** d
            weight[0] = weight[64] = 1.0
        else:
            m = np.block([[ea.real, SN1 * ea.imag], [eb.real, -SN1 * eb.imag],
                          [ea.imag, -SN1 * ea.real], [eb.imag, SN1 * eb.real]])
        fwd.append(m[out_rows])
        inv.append(((m * weight[:, None]).T / (S * D))[out_rows][:, in_rows])
    b = np.concatenate(fwd + inv, axis=1).astype(ml_dtypes.bfloat16).view(np.uint16).astype(np.uint32)
    return b[0::2] | (b[1::2] << 16)


_CHANNEL_MATRICES = _channel_matrices()


def L(t, n=1):
    return slice(128 * t, 128 * (t + n))


def add(a, b):
    return b if a is None else a if b is None else lax.add(a, b)


def sub(a, b):
    return lax.sub(a, b)


def mul(a, b):
    if isinstance(b, float):
        return lax.mul(a, lax.full(a.shape, b, f32))
    return lax.mul(a, b)


def tree(xs):
    return xs[0] if len(xs) == 1 else add(tree(xs[:len(xs) // 2]), tree(xs[len(xs) // 2:]))


def cast(a, dt):
    return lax.convert_element_type(a, dt)


def cat(*xs):
    return lax.concatenate(xs, 0)


def rows(x, lo, n):
    return lax.slice_in_dim(x, lo, lo + n, axis=0)


def bcast(x, n):
    return lax.broadcast_in_dim(x, (n, 128), (0, 1))


def iota(axis):
    return lax.broadcasted_iota(jnp.int32, (8, 128), axis)


def cmul(u, v):
    return sub(mul(u[0], v[0]), mul(u[1], v[1])), add(mul(u[0], v[1]), mul(u[1], v[0]))


def unit(turns):
    angle = turns * float(-2 * np.pi)
    return jnp.cos(angle), jnp.sin(angle)


def _radix5(x0, x1, x2, x3, x4):
    s1, d1, s2, d2 = add(x1, x4), sub(x1, x4), add(x2, x3), sub(x2, x3)
    t = add(s1, s2)
    m = sub(x0, mul(t, 0.25))
    q = mul(sub(s1, s2), C5)
    return add(x0, t), add(m, q), add(d1, mul(d2, R5)), sub(m, q), sub(mul(d1, R5), d2)


def _radix5_t(t0, a1, b1, a2, b2):
    m = add(a1, a2)
    q = mul(sub(a1, a2), C5)
    t = sub(t0, mul(m, 0.25))
    s1, s2 = add(t, q), sub(t, q)
    d1, d2 = add(b1, mul(b2, R5)), sub(mul(b1, R5), b2)
    return add(t0, m), add(s1, d1), add(s2, d2), sub(s2, d2), sub(s1, d1)


def _half4(u, v):
    return add(u[0], v[0]), add(u[1], v[1]), sub(u[0], v[0]), sub(u[1], v[1])


def _finish4(e, o, sign):
    pr, pi, mr, mi = e
    sr, si, tr, ti = o
    o0, o2 = (add(pr, sr), add(pi, si)), (sub(pr, sr), sub(pi, si))
    oa, ob = (add(mr, ti), sub(mi, tr)), (sub(mr, ti), add(mi, tr))
    return (o0, oa, o2, ob) if sign < 0 else (o0, ob, o2, oa)


def _radix4(v, sign):
    return _finish4(_half4(v[0], v[2]), _half4(v[1], v[3]), sign)


def _twiddle(v, e):
    r, i = v
    e %= 16
    if e == 0:
        return r, i
    if e == 4:
        return lax.neg(i), r
    if e == 12:
        return i, lax.neg(r)
    c, s = float(np.cos(np.pi * e / 8)), float(np.sin(np.pi * e / 8))
    if e % 4 == 2:
        if c * s > 0:
            return mul(sub(r, i), c), mul(add(r, i), c)
        return mul(add(r, i), c), mul(sub(i, r), c)
    return sub(mul(r, c), mul(i, s)), add(mul(r, s), mul(i, c))


def _lhs7(i, a):
    if i == 0: return add(a(0, 0), a(1, 1))
    if i == 1: return add(a(1, 0), a(1, 1))
    if i == 2: return a(0, 0)
    if i == 3: return a(1, 1)
    if i == 4: return add(a(0, 0), a(0, 1))
    if i == 5: return sub(a(1, 0), a(0, 0))
    return sub(a(0, 1), a(1, 1))


def _rhs7(i, b):
    if i == 0: return add(b(0, 0), b(1, 1))
    if i == 1: return b(0, 0)
    if i == 2: return sub(b(0, 1), b(1, 1))
    if i == 3: return sub(b(1, 0), b(0, 0))
    if i == 4: return b(1, 1)
    if i == 5: return add(b(0, 0), b(0, 1))
    return add(b(1, 0), b(1, 1))


def _fold7(j, m, get, put, done):
    if j < 3:
        put(j, m)
    elif j == 3:
        done(1, 0, add(get(1), m))
        put(3, add(get(0), m))
    elif j == 4:
        done(0, 1, add(get(2), m))
        put(4, sub(get(3), m))
    elif j == 5:
        done(1, 1, add(add(sub(get(0, 2), get(1, 2)), get(2, 2)), m))
    else:
        done(0, 0, add(get(4), m))


LHS1 = ((2, 5), (3, 6), (1, 0, 4))
LHS2 = ((2, 0, 3), (1, 5), (4, 6))
RHS = ((1, 0, 4), (2, 5), (3, 6))
_FIRST = [7 * i + j for group in LHS1 for i in group for j in range(7)]
EARLY = ([(0, 1, ij) for ij in _FIRST[:24]], [(0, 1, ij) for ij in _FIRST[24:40]],
         [(0, 2, ij) for ij in _FIRST[40:48]], [(1, 3, ij) for ij in _FIRST[:12]])
DONE = {ij: hi for part in EARLY for _, hi, ij in part}


def quarters(j):
    cuts = sorted({128 * j, 128 * j + 128} | {c for c in (160, 320, 480) if 128 * j < c < 128 * j + 128})
    return [(lo // 160, lo % 160, hi - lo) for lo, hi in zip(cuts, cuts[1:])]


def _nt(a, b):
    return lax.dot_general(a, b, (((1,), (1,)), ((), ())), preferred_element_type=f32)


def _nn(a, b):
    return lax.dot_general(a, b, (((1,), (0,)), ((), ())), preferred_element_type=f32)


def _merge(*streams):
    order = []
    for si, st in enumerate(streams):
        st, t0, t1 = st if isinstance(st, tuple) else (st, 0.0, 1.0)
        tot, acc = float(sum(t[0] for t in st)) or 1.0, 0.0
        for t in st:
            order.append((t0 + (t1 - t0) * (acc + (0.5 * t[0] if si else 0.0)) / tot, si, len(order), t))
            acc += t[0]
    for _, _, _, t in sorted(order, key=lambda o: o[:3]):
        t[1](*t[2:])


class Bank:
    def __init__(self, refs, offsets, cols, nrows, packed=0, chained=0):
        self.refs, self.offsets, self.nrows, self.packed, self.chained = refs, offsets, nrows, packed, chained
        self.cache, self.count, self.held = {}, 0, None

    @staticmethod
    def shapes(count, cols, nrows, packed=0, chained=0):
        n = ((cols + packed) >> packed) * (nrows >> packed) + 8
        return [pltpu.VMEM(((n + 31) // 32 * 32, 128 << packed), u32 if packed else f32) for _ in range(count)]

    def view(self, k, via):
        if (k, via) not in self.cache:
            r = self.refs[k]
            self.cache[k, via] = r.at[pl.ds(self.offsets[via], r.shape[0])] if via else r
        return self.cache[k, via]

    def get(self, k, col, lo=0, n=None, via=1):
        lo += (col >> self.packed) * self.nrows
        x = self.view(k, via)[lo >> self.packed:(lo + (n or self.nrows)) >> self.packed, L(col & self.packed)]
        return pltpu.bitcast(x, bf16) if self.packed else x

    def wide(self, k, cols, via=1):
        return lax.concatenate([self.get(k, c, via=via) for c in cols], 1)

    def halves(self, k, c, via=1):
        return cat(self.get(k, 2 * c, via=via), self.get(k, 2 * c + 1, via=via))

    def put(self, k, col, lo, x):
        if self.packed and col % 2 == 0:
            self.held = x
            return
        if self.packed:
            x = pltpu.bitcast(cast(lax.concatenate([self.held, x], 1), bf16), u32)
        at = ((col >> self.packed) * self.nrows + lo) >> self.packed
        self.count += 1
        self.view(k, (0, 6 + self.count % 2, 6)[self.chained])[at:at + x.shape[0], :] = x

    def clear_tokens(self):
        for r in self.refs:
            r[r.shape[0] - 8:r.shape[0], L(0)] = jnp.zeros((8, 128), r.dtype)

    def token(self, k):
        n = self.refs[k].shape[0]
        return (id(self), k), self.refs[k][n - 8:n, L(0)]


class Table(Bank):
    def __init__(self, refs, offsets, nrows, groups, chained):
        super().__init__(refs, offsets, None, nrows, 1, chained)
        self.slot = {i: (g, 7 * k) for g, group in enumerate(groups) for k, i in enumerate(group)}

    @staticmethod
    def shapes(tiles, nrows, groups, chained):
        return [s for _ in range(tiles) for g in groups for s in Bank.shapes(1, 7 * len(g), nrows, 1)]

    def load(self, k, i, j, via, lo=0, n=None):
        g, s = self.slot[i]
        return self.get(3 * k + g, s + j, lo, n, via)

    def store(self, k, i, j, lo, val):
        g, s = self.slot[i]
        self.put(3 * k + g, s + j, lo, val)

    def tiles(self, ij, ks, via, axis=1):
        return lax.concatenate([self.load(k, ij // 7, ij % 7, via) for k in ks], axis)


BANKS = dict(
    x0=(Bank, 4, 4, D),
    x1=(Bank, 4, 4, 2 * BINS),
    vb=(Bank, 16, 4, 168),
    mr2=(Bank, 12, 2, 2 * BINS),
    wt=(Bank, 4, 4, F - MAIN, 1, 2), br=(Bank, 4, 12, 64, 1, 1), tb=(Bank, 4, 40, 64, 1, 1),
    a1=(Table, 4, 160, LHS1, 2), hp=(Bank, 4, 12, 160, 1, 2), bt=(Bank, 1, 1, 256),
    a2=(Table, 3, 160, LHS2, 1), ar=(Bank, 1, 18, 128, 1, 2),
    b1=(Table, 12, 128, RHS, 1), b2=(Table, 12, 128, RHS, 1),
    lo=(Bank, 10, 1, 160), hi=(Bank, 10, 4, 160), zb=(Bank, 4, 12, BINS, 1, 1),
    post=(Bank, 1, 1, 240, 1, 2), sm=(Bank, 1, 48, 128, 1), mean=(Bank, 4, 4, 40, 0, 2), sums=(Bank, 4, 4, 64))

BIAS1, BIAS2, MEAN, SCALE, SHIFT = 0, 16, 32, 48, 64


def _kernel(x_hbm, wr_hbm, wi_hbm, w1_hbm, b1_hbm, w2_hbm, b2_hbm, dm_hbm, o_hbm,
            b1_ref, b2_ref, wrb, wib, w1b, w2b, dm_ref, wp, wt, small, sems, kept):
    zero = iota(1)[0, 0]
    zs = [None] + [pl.multiple_of(zero << (4 + k), 16) for k in range(7)]
    m = {name: spec[0](kept[name], zs, *spec[2:]) for name, spec in BANKS.items()}
    pool, a1, a2 = kept["mr2"], kept["a1"], kept["a2"]
    m.update(va=Bank(kept["x1"], zs, 8, BINS), k1=Bank(pool[:8], zs, 4, BINS), hb=Bank(pool[8:12], zs, 4, BINS),
             part=Bank(pool[:6] + pool[8:9], zs, 8, 160),
             mr1=Bank(pool[6:8], zs, 5, F - MAIN), d0=Bank(pool[9:], zs, 4, 128),
             yb=Bank(a1[2::3] + a1[0::3], zs, 6, BINS, 1))

    def dm(p):
        return pltpu.bitcast(dm_ref[:, L(p)], bf16)

    wpr = [r.at[pl.ds(zs[1], 2)] for r in wp]
    w_rd = [[r.at[pl.ds(zs[1 + g], F)] for g in range(3)] for r in (w1b, w2b)]
    tokens, ready, backlog, plain = [], set(), [], {}

    def row(i, n):
        return bcast(small[i:i + 1, :], n)

    def paced(a):
        if not tokens:
            return a
        n, gates = a.shape[0] // 16, {}
        for i, (key, tok) in enumerate(tokens):
            gates.setdefault(max((i + 1) * n // len(tokens) - 1, 0), {})[key] = tok
        tokens.clear()
        parts, lo = [], 0
        for r in sorted(gates):
            if r > lo:
                parts.append(lax.slice(a, (16 * lo, 0), (16 * r, 128)))
            w = pltpu.bitcast(lax.slice(a, (16 * r, 0), (16 * r + 16, 128)), u32)
            for tok in gates[r].values():
                w = lax.bitwise_or(w, lax.bitcast_convert_type(tok, u32))
            parts.append(pltpu.bitcast(w, bf16))
            lo = r + 1
        if lo < n:
            parts.append(lax.slice(a, (16 * lo, 0), (16 * n, 128)))
        left = cat(*parts)
        return left if a.shape[1] == 128 else lax.concatenate([left, lax.slice(a, (0, 128), a.shape)], 1)

    def copy(src, dst, group):
        return pltpu.make_async_copy(src, dst, sems.at[group])

    order = [a + 4 * b for a in range(4) for b in range(4)]
    x_cp = {t: copy(x_hbm.at[L(t), :], w2b.at[L(t // 3), L(5 * (t % 3), 5)], (0, 1, 2, 2, 3, 3, 4, 4)[k // 2])
            for k, t in enumerate(order)}
    o_cp = {t: [copy(w1b.at[L(t // 3), L(5 * (t % 3) + j, n)], o_hbm.at[L(t), L(j, n)], 5)
                for j, n in (((0, 3), (3, 2)) if t % 4 == 3 else ((0, 5),))] for t in order}
    nudges = []

    def launch(*copies):
        k = len(nudges)
        nudges.append(copy(dm_hbm.at[0:8, L(0)], m["post"].view(0, 5).at[8 * k:8 * k + 8, L(0)], 5))
        for c in copies + (nudges[-1],):
            c.start()
        tokens.append(m["post"].token(0))

    w_cp = {(k, n): copy(src.at[lo:hi, :], dst.at[lo:hi, :], 3 if k or n == 3 else 4)
            for k, (src, dst) in enumerate(((w1_hbm, w1b), (w2_hbm, w2b)))
            for n, (lo, hi) in enumerate(((0, 512), (512, 1024), (1024, MAIN), (MAIN, F))) if k or n}
    w_cp[0, 0] = [copy(w1_hbm.at[0:512, L(t)], w1b.at[0:512, L(t)], 0 if k < 8 else 3) for k, t in enumerate(order)]

    def get_v(name, a, q, lo, n):
        return tuple(m[name].get(*((a, 4 * e + q) if name == "va" else (2 * a + e, q)), lo, n) for e in range(2))

    def put_v(name, a, q, lo, val):
        for e in range(2):
            m[name].put(*((a, 4 * e + q) if name == "va" else (2 * a + e, q)), lo, val[e])

    def gather(acc, t, *xs):
        acc[t, 0] = add(acc.get((t, 0)), tree(xs))
        acc[t, 1] = add(acc.get((t, 1)), tree([mul(x, x) for x in xs]))

    def moments(acc, t):
        mean = jnp.sum(acc[t, 0], axis=0, keepdims=True) * (1.0 / D)
        return mean, jnp.maximum(jnp.sum(acc[t, 1], axis=0, keepdims=True) * (1.0 / D) - mean * mean, 0.0)

    def norm_once(acc, t):
        mean, var = moments(acc, t)
        small[MEAN + t:MEAN + t + 1, :] = mean
        small[SCALE + t:SCALE + t + 1, :] = lax.rsqrt(var + EPS)

    def load_x(t):
        eye = (lax.broadcasted_iota(jnp.int32, (128, 128), 0) == lax.broadcasted_iota(jnp.int32, (128, 128), 1)).astype(bf16)
        xt = _nt(paced(eye), jnp.concatenate([w2b[L(t // 3), L(5 * (t % 3) + j)] for j in range(5)], axis=0))
        acc = {}
        for c in range(16):
            x = [lax.slice(xt, (8 * c, 128 * j), (8 * c + 8, 128 * j + 128)) for j in range(5)]
            for j in range(5):
                m["x0"].put(t % 4, t // 4, 128 * j + 8 * c, x[j])
            gather(acc, t, *x)
        norm_once(acc, t)

    def fwd10(t, c):
        halves = []
        m10, r = mul(row(MEAN + t, 8), 10.0), row(SCALE + t, 8)
        for h in range(2):
            x = [m["x0"].get(t % 4, t // 4, 64 * i + 16 * c + 8 * h, 8) for i in range(10)]
            e = _radix5(*[add(x[i], x[i + 5]) for i in range(5)])
            o = _radix5(*[sub(x[i], x[i + 5]) if i % 2 == 0 else sub(x[i + 5], x[i]) for i in range(5)])
            halves.append([mul(v, r) for v in (sub(e[0], m10), o[0], e[1], e[2], e[3], e[4], o[1], o[2], o[3], o[4])])
        for i in range(10):
            m["tb"].put(t % 4, 10 * (t // 4) + i, 16 * c, cat(halves[0][i], halves[1][i]))
        tokens.append(m["tb"].token(t % 4))

    def fwd_d(a, p):
        g = _nn(paced(dm(p)), lax.concatenate([m["tb"].halves(a, 5 * b + p) for b in range(4)], 1))
        for c in range(8):
            v = [(lax.slice(g, (16 * c, 128 * b), (16 * c + 8, 128 * b + 128)),
                  lax.slice(g, (16 * c + 8, 128 * b), (16 * c + 16, 128 * b + 128))) for b in range(4)]
            if p == 0 and c == 0:
                for q, w in enumerate(_radix4([(i, jnp.zeros((8, 128), f32)) for (_, i) in v], -1)):
                    w = _twiddle(w, -q * a)
                    put_v("va", a, q, 320, (cat(w[0], w[0]), cat(w[1], w[1])))
                v = [(r, jnp.where(iota(0) == 0, 0.0, i)) for (r, i) in v]
            for q, w in enumerate(_radix4(v, -1)):
                put_v("va", a, q, 80 * (c % 4) + 16 * p + 8 * (c // 4), _twiddle(w, -q * a))

    def permute_w(get, put):
        cur = [get((-k) % 16) for k in range(16)]
        cur = [pltpu.roll(c, (-k) % 16, 1) if k else c for k, c in enumerate(cur)]
        for bit in (1, 2, 4, 8):
            msk = (iota(1) & bit) != 0
            cur = [lax.select(msk, cur[(k - bit) % 16], cur[k]) for k in range(16)]
        for k in range(16):
            put(k, cur[k])

    def prep_w(src, ri, part, c):
        if c < 20:
            def put(k, v):
                wp[part][ri, k, 8 * (c - 5 * part):8 * (c - 5 * part) + 8, :] = v
            permute_w(lambda t: pltpu.bitcast(src[16 * c:16 * c + 16, L(t)], u32), put)
        else:
            def put(k, v):
                wt[ri, k] = v
            permute_w(lambda t: bcast(cast(src[320:321, L(t)], f32), 8), put)

    def w_rows(ri, k1, c):
        if c == 20:
            v = wt[ri, k1]
            return cat(v, v)
        out = []
        for k in TILE_CLASSES[c % 5]:
            v = wpr[min(c // 5, 2)][ri, k1, pl.ds(k // 2 + 40 * (c // 15), 8, stride=5), :]
            out.append(lax.bitwise_and(v, lax.full(v.shape, 0xFFFF0000, u32)) if k % 2 else lax.shift_left(v, lax.full(v.shape, 16, u32)))
        return pltpu.bitcast(cat(*out), f32)

    def s_in(q, c):
        z = _radix4([get_v("va", a, q, 16 * c, 16) for a in range(4)], -1)
        for p in range(4):
            for j, val in enumerate((add(z[p][0], z[p][1]), z[p][0], z[p][1])):
                m["zb"].put(q, 3 * p + j, 16 * c, val)
        tokens.append(m["zb"].token(q))

    def spectral(extra):
        units = [(h, q) for h in range(2) for q in range(4)]

        def s_dot(h, q, p, j, inverse):
            lo, n = 160 * h, 160 + 16 * h
            lhs = paced(m["yb"].get(2 * q + p % 2, 3 * (p // 2) + j, lo, n) if inverse else m["zb"].get(q, 3 * p + j, lo, n))
            return (_nt if inverse else _nn)(lhs, m["sm"].get(0, 16 * j + q + 4 * p, via=1 + 2 * h + inverse))

        def s_fwd(h, q, ps):
            prod = {(p, j): s_dot(h, q, p, j, 0) for p in ps for j in (1, 2)}
            for k in range(10 + h):
                c = 10 * h + k
                for p in ps:
                    both = m["k1"].get(2 * q, p, 16 * c, 16)
                    x = sub(both, rows(prod[p, 2], 16 * k, 16)), add(both, rows(prod[p, 1], 16 * k, 16))
                    yr, yi = cmul(x, (w_rows(0, q + 4 * p, c), w_rows(1, q + 4 * p, c)))
                    for j, val in enumerate((add(yr, yi), yi, yr)):
                        m["yb"].put(2 * q + p % 2, 3 * (p // 2) + j, 16 * c, val)

        def s_inv(h, q, odd):
            ps = (odd, odd + 2)
            prod = {(p, j): s_dot(h, q, p, j, 1) for p in ps for j in (1, 2)}
            for k in range(20 + h):
                lo, z = 160 * h + 8 * k, []
                for p in ps:
                    both = m["k1"].get(2 * q + 1, p, lo, 8)
                    z.append((add(both, rows(prod[p, 1], 8 * k, 8)), sub(both, rows(prod[p, 2], 8 * k, 8))))
                half = _half4(*z)
                if not odd:
                    for j in range(4):
                        m["hb"].put(q, j, lo, half[j])
                else:
                    for a, w in enumerate(_finish4([m["hb"].get(q, j, lo, 8) for j in range(4)], half, 1)):
                        put_v("vb", 4 * h + a, q, 8 * k, _twiddle(w, q * a))

        for c in range(10):
            s_in(0, c)
        tokens.clear()
        for u in range(9):
            now, before = units[u] if u < 8 else None, units[u - 1] if u else None
            common = ([now + (0,)] if now else []) + ([before + (1,)] if before else [])
            side, more = list(extra[u][0]), extra[u][1]
            if u < 7:
                h, q = units[u + 1]
                side += [(1, s_in, q, 10 * h + k) for k in range(10 + h)]
            early = [(1, inv4, a, p, c) for a in range(4) for p in range(5) for c in range(2)][u - 5::4] if u > 4 else []
            for k, (h, q, inverse) in enumerate(common):
                _merge(side[k * len(side) // len(common):(k + 1) * len(side) // len(common)])
                for p in range(4):
                    m["k1"].put(2 * q + inverse, p, 160 * h, s_dot(h, q, p, 0, inverse))
            for odd in range(2):
                if now:
                    s_fwd(*now, (odd, odd + 2))
                if before:
                    _merge(early[odd::2], more if odd == 0 else [])
                    s_inv(*before, odd)

    def inv4(a, p, c):
        g = _radix4([get_v("vb", 4 * (c // 2) + a, q, 80 * (c % 2) + 16 * p, 16) for q in range(4)], 1)
        if (p, c) == (0, 0):
            for b in range(4):
                m["mean"].put(a, b, 0, cat(*g[b]))
            return
        for b in range(4):
            for j in range(2):
                m["tb"].put(a, 10 * b + 2 * p + j, 16 * c, g[b][j])
        tokens.append(m["tb"].token(a))

    def real_bins(a, first):
        ny = _radix4([get_v("vb", 4 + a, q, 160, 8) for q in range(4)], 1)
        for b in range(4):
            t = a + 4 * b
            g = m["mean"].get(a, b, 0, 32)
            m["tb"].put(a, 10 * b, 0, rows(g, 0, 16))
            m["tb"].put(a, 10 * b + 1, 0, cat(lax.select(iota(0) == 0, ny[b][0], rows(g, 16, 8)), rows(g, 24, 8)))
            mean = small[MEAN + t:MEAN + t + 1, :] + rows(g, 0, 1) * (1.0 / (S * D))
            carried = None if first else small[SHIFT + t:SHIFT + t + 1, :]
            small[SHIFT + t:SHIFT + t + 1, :] = add(small[BIAS2 + t:BIAS2 + t + 1, :] + mean, carried)
            m["mean"].put(a, b, 32, bcast(mean, 8))
        tokens.append(m["mean"].token(a))

    def inv_d0(a):
        for b in range(4):
            m["d0"].put(a % 2, b, 0, _nn(paced(dm(5)), m["tb"].halves(a, 5 * b)))

    def inv_d(a, b):
        t = a + 4 * b
        tt = [_nn(dm(5 + p), m["tb"].halves(a, 5 * b + p)) for p in range(1, 5)]
        mean, sq = m["mean"].get(a, b, 32, 8), None
        for c in range(8):
            v = [rows(tt[i // 2], 16 * c + 8 * (i % 2), 8) for i in range(8)]
            e = _radix5_t(sub(m["d0"].get(a % 2, b, 16 * c, 8), mean), *v[0:4])
            o = _radix5_t(m["d0"].get(a % 2, b, 16 * c + 8, 8), *v[4:8])
            part = []
            for i in range(5):
                for j, sg in ((i, i % 2), (i + 5, 1 - i % 2)):
                    x = add(m["x0"].get(a, b, 64 * j + 8 * c, 8, 2), (sub if sg else add)(e[i], o[i]))
                    m["x1"].put(a, b, 64 * j + 8 * c, x)
                    part.append(mul(x, x))
            sq = add(sq, tree(part))
        var = jnp.sum(sq, axis=0, keepdims=True) * (1.0 / D)
        r = lax.rsqrt(var + EPS)
        small[SCALE + t:SCALE + t + 1, :] = r * lax.rsqrt(var * r * r + EPS) * 0.5

    def split2(load, pick, put, group, gate=None):
        seen = {}

        def blk(i, j):
            if (i, j) not in seen:
                seen[i, j] = load(i, j)
            return seen[i, j]
        for i in group:
            h = {(r, k): pick(i, lambda r1, k1: blk(2 * r1 + r, 2 * k1 + k)) for r in range(2) for k in range(2)}
            for j in range(7):
                put(i, j, pick(j, lambda r, k: h[r, k]))
            if i == group[-1] and len(group) % 2:
                put(i, 7, pick(6, lambda r, k: h[r, k]))
            if gate:
                tokens.append(gate())

    def lhs1(a, v, g):
        def load(r, k):
            t = a + 4 * k
            h = mul(m["x1"].get(a, k, 160 * r + 16 * v, 16, 3 + g), row(SCALE + t, 16))
            if r != k and g == k // 2:
                m["hp"].put(a, plain.setdefault((r, k), len(plain)), 16 * v, h)
            return h

        def put(i, j, val):
            m["a1"].store(a, i, j, 16 * v, val)
        split2(load, _lhs7, put, LHS1[g])
        tokens.append(m["hp"].token(a))
        tokens.append(m["a1"].token(3 * a + g))

    def weights(which, g, lo, t):
        return cast(w_rd[which][g][lo:lo + 16, L(t)], f32)

    def rhs_main(which, n, a, v, g):
        def raw(f, s):
            lo = 128 * (4 * n + f) + 16 * v
            return weights(which, g, lo, a + 4 * s)
        tab = m[("b1", "b2")[which]]
        split2(raw if which else lambda s, f: raw(f, s), _rhs7,
               lambda i, j, val: tab.store(4 * n + a, i, j, 16 * v, val), RHS[g], lambda: tab.token(3 * (4 * n + a) + g))

    def rhs_rest(a, pair, v):
        (p1, p2, p3), (q1, q2, q3) = ([weights(1, 0, MAIN + 64 * k + 16 * v, a + 8 * pair + 4 * e) for k in range(3)] for e in range(2))
        for k, val in enumerate((sub(p1, q1), p2, q2, sub(q3, p3), q1, p3)):
            m["br"].put(a, 6 * pair + k, 16 * v, val)
        tokens.append(m["br"].token(a))

    def rhs_main_tasks(which, ns, as_, gs=range(3)):
        return [(36 * len(RHS[g]), rhs_main, which, n, a, v, g) for g in gs for n in ns for a in as_ for v in range(8)]

    def rhs_rest_tasks():
        return [(22, rhs_rest, a, pair, v) for a in range(4) for pair in range(2) for v in range(4)]

    def gelu_half(u):
        inner = mul(u, add(mul(mul(u, u), 8 * GELU * 0.044715), lax.full(u.shape, 2 * GELU, f32)))
        return add(u, mul(u, lax.tanh(inner)))

    def fold49(ij, flip, prod, done):
        i, j = divmod(ij, 7)
        for v in range(20):
            def slot(bank, par, col):
                return (lambda k, via=1: bank.get(5 * par + k, col, 8 * v, 8, via),
                        lambda k, val: bank.put(5 * par + k, col, 8 * v, val))

            def inner(r, n, h):
                _fold7(i, h, *slot(m["hi"], flip, 2 * r + n), lambda r1, n1, c: done(2 * r1 + r, 2 * n1 + n, v, c))
            _fold7(j, rows(prod, 8 * v, 8), *slot(m["lo"], i % 2, 0), inner)

    def stage_w1(a, k):
        for e in (2 * k, 2 * k + 1):
            m["wt"].put(a, e, 0, cast(w1b[MAIN:F, L(a + 4 * e)], f32))
        tokens.append(m["wt"].token(a))

    def mm1_rest(a, j):
        def h(k):
            return cat(*[m["hp"].get(a, plain[r, k], lo, n) if r != k else m["a1"].load(a, 2 + k // 2, 2 + k % 2, 4, lo, n)
                         for r, lo, n in quarters(j)])
        w = m["wt"].wide(a, range(4), via=1 + j)
        prod = _nt(paced(w), lax.concatenate([h(k) for k in range(4)], 1))
        for lo in range(0, F - MAIN, 8):
            u = add(rows(prod, lo, 8), m["mr1"].get(1 - a % 2, j, lo, 8) if a else m["bt"].get(0, 0, lo, 8, 1 + j))
            m["mr1"].put(a % 2, j, lo, gelu_half(u) if a == 3 else u)

    def mm1_early(lo, hi, ij):
        prod = _nt(paced(m["a1"].tiles(ij, range(lo, hi), 5)), m["b1"].tiles(ij, range(lo, hi), 2))
        m["part"].put(ij // 8, ij % 8, 0, add(prod, m["part"].get(ij // 8, ij % 8, via=2) if lo else None))

    def mm1_main(n, ij):
        def done(r, f, v, u):
            m["vb"].put(4 * (n % 2) + r, f, 8 * v, gelu_half(add(u, row(BIAS1 + 4 * n + f, 8))))
        k = DONE.get(ij, 0) if n == 0 else 0
        prod = _nt(paced(m["a1"].tiles(ij, range(k, 4), 1 + n)), m["b1"].tiles(ij, range(4 * n + k, 4 * n + 4), 1))
        if k:
            prod = add(prod, m["part"].get(ij // 8, ij % 8, 0, 160))
        fold49(ij, n % 2, prod, done)

    def lhs_rest(j, k):
        for e in range(2):
            g = cat(*[m["mr1"].get(1, 2 * j + e, 64 * u, 64, 1 + k) if 2 * j + e < 5 else jnp.zeros((64, 128), f32)
                      for u in ((0, 1), (1, 2), (0, 2))[k]])
            m["ar"].put(0, 6 * k + 2 * j + e, 0, g.T)
        tokens.append(m["ar"].token(0))

    def lhs2(n, v, g):
        split2(lambda r, f: m["vb"].get(4 * (n % 2) + r, f, 16 * v, 16, 1 + g), _lhs7,
               lambda i, j, val: m["a2"].store(n, i, j, 16 * v, val), LHS2[g], lambda: m["a2"].token(3 * n + g))

    def lhs2_tasks(n):
        return [(23 * len(LHS2[g]), lhs2, n, v, g) for v in range(10) for g in range(3)]

    def mm2_rest(a, k, r):
        lhs = paced(cat(*[m["ar"].get(0, 6 * k + j, lo - 128 * j, n, 1 + a) for j in range(5)
                          for q, lo, n in ((q, 160 * q + at, n) for q, at, n in quarters(j)) if q == r]))
        prod = _nn(lhs, lax.concatenate([m["br"].halves(a, 3 * e + k, 1 + r) for e in range(2)], 1))
        for e in range(2):
            m["mr2"].put(3 * a + k, e, 160 * r, lax.slice_in_dim(prod, 128 * e, 128 * e + 128, axis=1))

    def write_out(t, j):
        x = m["x0"].get(t % 4, t // 4, 128 * j, 128, 3) if t % 4 < 3 else cat(
            *[m["vb"].get(4 * r + t // 4, 0, lo, n, 4) for r, lo, n in quarters(j)])
        out = x.T
        w1b[L(t // 3), L(5 * (t % 3) + j)] = cast(out, bf16)
        m["mean"].put(0, 0, 0, rows(out, 120, 8))
        tokens.append(m["mean"].token(0))

    def mm2_main(a, ij, first):
        acc = {}
        def done(r, b, v, y):
            rest = [m["mr2"].get(3 * a + k, b // 2, 160 * r + 8 * v, 8, 1 + b % 2) for k in (b % 2, 2)]
            shift = None if first else row(SHIFT + a + 4 * b, 8)
            x = add(add(m["x1"].get(a, b, 160 * r + 8 * v, 8), shift), add(y, add(*rest)))
            if first or a < 3:
                m["x0"].put(a, b, 160 * r + 8 * v, x)
            else:
                m["vb"].put(4 * r + b, 0, 8 * v, x)
            if first:
                gather(acc, 0, x)
                if v == 19:
                    m["sums"].put(a, b, 16 * r, cat(acc[0, 0], acc[0, 1]))

        prod = _nn(paced(m["a2"].tiles(ij, range(3), 1 + a)), m["b2"].tiles(ij, range(a, 12, 4), 1, 0))
        fresh = set()
        fold49(ij, (a + 1) % 2, prod, lambda r, b, v, y: (done(r, b, v, y), fresh.add((r, b))))
        if a == 3 and not first:
            for r, b in sorted(fresh):
                t = a + 4 * b
                ready.add((r, t))
                for j in range(5):
                    need = {(128 * j // 160, t), ((128 * j + 127) // 160, t)}
                    if (r, t) in need and need <= ready:
                        backlog.append((ij, write_out, t, j))
                for part, need in enumerate(({(0, t), (1, t), (2, t)}, {(2, t), (3, t)})):
                    if (r, t) in need and need <= ready:
                        backlog.append((ij, launch, o_cp[t][part]))
            for _ in range(2 if ij < 48 else 99):
                if backlog and (backlog[0][0] + 4 <= ij or ij == 48):
                    _, fn, *args = backlog.pop(0)
                    args[0].start() if fn is launch and ij == 48 else fn(*args)

    def norm_sums(a, b):
        tot = None
        for r in range(4):
            tot = add(tot, m["sums"].get(a, b, 16 * r, 16))
        norm_once({(a + 4 * b, j): rows(tot, 8 * j, 8) for j in range(2)}, a + 4 * b)

    def after_mm2(a, first):
        if not first:
            return ([(30, write_out, a + 4 * b, j) for b in range(4) for j in range(5)] +
                    [(30, launch, *[o_cp[a + 4 * b][0] for b in range(4)])]) if a < 3 else []
        return ([(20, norm_sums, a, b) for b in range(4)] +
                [(115, fwd10, a + 4 * b, c) for b in range(4) for c in range(4)])

    def post_stage(first):
        def inv4_tasks(a):
            return [(20, real_bins, a, first)] + [(40, inv4, a, p, c) for p in range(5) for c in (2, 3)]
        sums = [rhs_main_tasks(0, [0], [a]) if first else [] for a in range(4)]
        plan = [[(hi - lo, mm1_early, lo, hi, ij) for lo, hi, ij in part] for part in EARLY]
        for a in range(4):
            _merge(inv4_tasks(a)[:3])
            inv_d0(a)
            _merge(inv4_tasks(a)[3:])
            tokens.clear()
            side = [[(30 * len(LHS1[g]), lhs1, a, v, g) for v in range(10)] for g in range(3)]
            for b in range(4):
                inv_d(a, b)
                if a == 0 and b == 2:
                    _merge(side.pop(0))
                    tokens.clear()
                if a or b >= 2:
                    n = 4 // plan[a][0][0]
                    _merge(plan[a][:n])
                    del plan[a][:n]
            if first:
                side.append([(40, stage_w1, a, k) for k in range(2)] + (sums[2] if a == 1 else []))
            if a == 0:
                n = 14 - (24 - len(plan[0]))
                _merge(plan[0][:n], (side.pop(0), -0.2, 0.5))
                tokens.clear()
                del plan[0][:n]
            _merge([(4.8, mm1_rest, a - 1, j) for j in range(5 if a else 0)] + plan[a],
                   ([t for part in side for t in part], 0.0, 0.8))
        if first:
            for k in (3, 0, 1, 2):
                w_cp[1, k].start()
            w_cp[0, 1].wait()
            w_cp[0, 2].wait()
        _merge([(1, mm1_rest, 3, j) for j in range(5)], (sums[3][:8], -0.2, 0.8))

    cut = (48, 84, 156, 204, 240, 288)

    def w2_sums():
        return [t for a in range(4) for g in range(3) for t in rhs_main_tasks(1, range(3), [a], (g,))]

    def mm1_stage(first):
        for n in range(3):
            late, sums = [], []
            if first:
                late = rhs_main_tasks(0, [n], range(4) if n else [3], (1, 2))
                sums = rhs_main_tasks(0, [n + 1], range(4), (0,)) if n < 2 else [(0, w_cp[1, k].wait) for k in range(4)] + rhs_rest_tasks() + w2_sums()[:cut[0]]
            _merge([(1, mm1_main, n, ij) for ij in range(49)],
                   (lhs2_tasks(n - 1) if n else [], 0.45, 0.97),
                   ([(1, lhs_rest, j, k) for j in range(3) for k in range(3)] if n == 0 else [], 0.4, 0.95),
                   (late, 0.0, 0.39), (sums, 0.4 if n else 0.0, 0.95))

    def mm2_stage(first):
        sums = w2_sums() if first else []
        _merge([(1, mm2_rest, a, k, r) for a in range(4) for k in range(3) for r in range(4)], (lhs2_tasks(2), 0.0, 0.9), (sums[cut[0]:cut[1]], 0.0, 0.9))
        for a in range(4):
            _merge([(1, mm2_main, a, ij, first) for ij in range(49)],
                   (after_mm2(a - 1, first) if a else [], 0.1 if a < 3 or not first else 0.4, 0.95 if first else 0.45),
                   (sums[cut[a + 1]:cut[a + 2]], 0.0, 0.95 if a < 3 else 0.39))
        _merge([(1, fwd_d, a, p) for a in range(3) for p in range(5)] if first else [], (after_mm2(3, first), 0.0, 0.9))
        tokens.clear()
        if first:
            for p in range(5):
                fwd_d(3, p)
        else:
            for c in nudges + [c for t in order for c in o_cp[t]]:
                c.wait()

    def token_mixing(first):
        tokens.clear()
        post_stage(first)
        mm1_stage(first)
        mm2_stage(first)

    def first_transform():
        cuts = (0, 80, 160, 321)
        dm_cp = copy(dm_hbm.at[:, L(0, 5)], dm_ref.at[:, L(0, 5)], 2)
        small_cp = [copy(dm_hbm.at[:, L(5, 5)], dm_ref.at[:, L(5, 5)], 0), copy(b1_hbm, b1_ref, 0),
                    copy(b2_hbm, b2_ref.at[0:16, :], 0)]
        f_cp = [[copy(src.at[lo:hi, :], dst.at[lo:hi, :], k) for src, dst in ((wr_hbm, wrb), (wi_hbm, wib))]
                for k, (lo, hi) in enumerate(zip(cuts, cuts[1:]))]

        def prep(k):
            return [(1, prep_w, src, ri, k, c) for c in range(cuts[k] // 16, (cuts[k + 1] + 15) // 16)
                    for ri, src in enumerate((wrb, wib))]

        def fly(tiles):
            return [(1, fwd10, t, c) for t in tiles for c in range(4)]

        def start():
            for name in BANKS:
                if m[name].chained:
                    m[name].clear_tokens()
            launch(*[x_cp[t] for t in order[:6]])
            gate = lax.bitcast_convert_type(tokens.pop()[1], jnp.int32)
            s2, lane = (lax.broadcasted_iota(jnp.int32, (16, 128), k) for k in range(2))
            s2, lane = s2 + cat(gate, gate), lane + cat(gate, gate)
            k2 = ((lane & 15) << 3) + (lane >> 4)
            base, hop = (unit(cast(k & 127, f32) * (1.0 / 128)) for k in (s2 * k2, 16 * k2))
            step = unit(cast(s2, f32) * (1.0 / S))
            for c in range(8):
                if c:
                    base, step = cmul(base, hop), cmul(step, (float(np.cos(np.pi / 64)), float(-np.sin(np.pi / 64))))
                re, im = base
                for k1 in range(0, 16, 2):
                    nxt = cmul((re, im), step)
                    two = [[pltpu.roll(x, k, 1) if k else x for x in z] for k, z in enumerate(((re, im), nxt), k1)]
                    for j in range(3):
                        for k, (x, y) in enumerate(two, k1):
                            m["sm"].put(0, 16 * j + k, 16 * c, (x, sub(y, x), add(x, y))[j])
                    re, im = cmul(nxt, step)
            queue = [[x_cp[t] for t in order[k:k + 2]] + [dm_cp] * (k == 6) for k in range(6, 16, 2)] + f_cp[:2] + [[]]
            for before, lo, hi in ((0, 0, 2), (0, 2, 4), (2, 4, 8), (4, 8, 12), (8, 12, 16)):
                for c in queue.pop(0):
                    c.start()
                for c in [x_cp[t] for t in order[lo:hi]] + [dm_cp] * (lo == 4):
                    c.wait()
                _merge([(1, load_x, t) for t in order[lo:hi]] + [(0.8, fwd_d, lo // 4 - 1, p) for p in range(5 * (lo > 3))],
                       (fly(order[before:lo]), -0.2, 0.6 if lo == 2 else 0.3),
                       (fly(order[12:] if hi == 16 else []), 0.7, 0.95),
                       ([(1, launch, *queue.pop(0))] if lo > 3 else [], 0.2, 0.3))
                tokens.clear()
            for c in f_cp[2]:
                c.start()
            for c in f_cp[0]:
                c.wait()
            _merge([(1, fwd_d, 3, p) for p in range(5)], prep(0))

        def prep_bias():
            half = jnp.concatenate([b1_ref[...].astype(f32).reshape(1, F), jnp.zeros((1, 64), f32)], axis=1) * 0.5
            for n in range(14):
                if n < 12:
                    small[BIAS1 + n:BIAS1 + n + 1, :] = half[:, L(n)]
                else:
                    m["bt"].put(0, 0, 128 * (n - 12), bcast(half[:, L(n)], 128).T)
            small[BIAS2:BIAS2 + 16, :] = b2_ref[0:16, :].astype(f32)

        def rest():
            for c in small_cp + w_cp[0, 0][:4]:
                c.start()
            for c in f_cp[1]:
                c.wait()
            _merge(prep(1))
            sums = rhs_main_tasks(0, [0], [0, 1])
            cut = (0, 4, 10, 28, 34, 44, 48)
            sums = [sums[lo:hi] for lo, hi in zip(cut, cut[1:])]
            none = [], []
            spectral([none, none, none,
                      ([(0, c.start) for c in w_cp[0, 0][4:8] + [w_cp[0, 3]]] + [(0, c.wait) for c in f_cp[2]] + prep(2), []),
                      none, none,
                      ([(0, c.start) for c in w_cp[0, 0][8:]] + [(0, c.wait) for c in small_cp + w_cp[0, 0][:8]] +
                       [(0, prep_bias)] + sums[0], sums[1]), sums[2:4], sums[4:6]])
            w_cp[0, 1].start()
            w_cp[0, 2].start()
            for c in [w_cp[0, 3]] + w_cp[0, 0][8:]:
                c.wait()
        start()
        rest()

    first_transform()
    token_mixing(True)
    spectral([([], [])] * 9)
    token_mixing(False)


@jax.jit
def pallas_interleave_layers__spectral_gfnet__mixer_token_mlp__prompt_kernel(A_x, A_w_r, A_w_i, B_x, B_w1, B_b1, B_w2, B_b2):
    hbm = pl.BlockSpec(memory_space=pl.ANY)
    V = pltpu.VMEM
    out = pl.pallas_call(
        _kernel,
        in_specs=[hbm, hbm, hbm, hbm, hbm, hbm, hbm, hbm],
        out_specs=hbm,
        out_shape=jax.ShapeDtypeStruct((S, D), bf16),
        scratch_shapes=[
            V((F,), bf16), V((64, 128), bf16), V((321, S), bf16), V((321, S), bf16), V((F, S), bf16), V((F, S), bf16), V((64, 1280), u32),
            [V((2, 16, n, 128), u32) for n in (40, 40, 80)], V((2, 16, 8, 128), f32), V((96, 128), f32),
            pltpu.SemaphoreType.DMA((6,)),
            {name: spec[0].shapes(*spec[1:]) for name, spec in BANKS.items()},
        ],
        compiler_params=pltpu.CompilerParams(vmem_limit_bytes=127 * 1024 * 1024, internal_scratch_in_bytes=11 * 4096),
    )(A_x.reshape(S, D), A_w_r.T, A_w_i.T, B_w1.T, B_b1, B_w2,
      B_b2.reshape(16, 128), _CHANNEL_MATRICES)
    return out.reshape(1, S, D)
```
